```python
import jax
import jax.numpy as jnp

def _softmax(x, axis=-1):
    return jax.nn.softmax(x, axis=axis)

def _gelu(x):
    return jax.nn.gelu(x, approximate=True)

def _silu(x):
    return jax.nn.silu(x)

def _sigmoid(x):
    return jax.nn.sigmoid(x)

def _layernorm(x, axis=-1, eps=1e-05):
    m = jnp.mean(x, axis=axis, keepdims=True)
    v = jnp.var(x, axis=axis, keepdims=True)
    return (x - m) / jnp.sqrt(v + eps)

def _scatter_add(tgt, idx, src, axis=0):
    return tgt.at[idx].add(src)

def _segment_sum(src, seg, n):
    return jax.ops.segment_sum(src, seg, n)

class _Rng:

    def __init__(self, key):
        self._k = key

    def _next(self):
        self._k, sub = jax.random.split(self._k)
        return sub

    def normal(self, shape):
        return jax.random.normal(self._next(), shape, dtype=jnp.bfloat16)

    def randint(self, lo, hi, shape):
        return jax.random.randint(self._next(), shape, lo, hi, dtype=jnp.int32)

    def uniform(self, shape, lo=0.0, hi=1.0):
        return jax.random.uniform(self._next(), shape, jnp.bfloat16, lo, hi)

    def permutation(self, n):
        return jax.random.permutation(self._next(), n)
kernel_name = 'adaLN_cond__memory_aug_recurrent_mem_tr__glu_gated_swiglu__prompt'

def setup_inputs():
    _rng = _Rng(jax.random.key(int.from_bytes(__import__("os").urandom(4), "little")))
    _w = lambda a: (lambda t: t.astype(jnp.bfloat16) if jnp.issubdtype(t.dtype, jnp.floating) else t)(jnp.asarray(a))

    def _A_setup():
        B, S, Dm = (1, 2048, 1024)
        H, Dh = (32, 128)
        M, seg = (8, 32)
        seg = min(seg, S)
        S = S // seg * seg
        return {'x': _w((lambda *s: _rng.normal(s) * 0.05)(B, S, Dm)), 'mem0': _w((lambda *s: _rng.normal(s) * 0.05)(B, M, Dm)), 'Wq': _w((lambda *s: _rng.normal(s) * 0.05)(Dm, H, Dh) * Dm ** (-0.5)), 'Wk': _w((lambda *s: _rng.normal(s) * 0.05)(Dm, H, Dh) * Dm ** (-0.5)), 'Wv': _w((lambda *s: _rng.normal(s) * 0.05)(Dm, H, Dh) * Dm ** (-0.5)), 'Wo': _w((lambda *s: _rng.normal(s) * 0.05)(H, Dh, Dm) * (H * Dh) ** (-0.5)), 'seg_len': seg}
    _A_in = _A_setup()

    def _B_setup():
        B, S, D, F = (1, 2048, 1024, 3584)
        return {'x': _w((lambda *s: _rng.normal(s) * 0.05)(B, S, D)), 'w1': _w((lambda *s: _rng.normal(s) * 0.05)(D, F) * (2.0 / D) ** 0.5), 'w3': _w((lambda *s: _rng.normal(s) * 0.05)(D, F) * (2.0 / D) ** 0.5), 'w2': _w((lambda *s: _rng.normal(s) * 0.05)(F, D) * (2.0 / F) ** 0.5)}
    _B_in = _B_setup()
    return {'A_x': _A_in['x'], 'A_mem0': _A_in['mem0'], 'A_Wq': _A_in['Wq'], 'A_Wk': _A_in['Wk'], 'A_Wv': _A_in['Wv'], 'A_Wo': _A_in['Wo'], 'A_seg_len': _A_in['seg_len'], 'B_x': _B_in['x'], 'B_w1': _B_in['w1'], 'B_w3': _B_in['w3'], 'B_w2': _B_in['w2'], 'c': _w((lambda *s: _rng.normal(s) * 0.05)(1, 1024)), 'w_mod': _w((lambda *s: _rng.normal(s) * 0.05)(1024, 6 * 1024) * 1024 ** (-0.5))}

def reference(A_x, A_mem0, A_Wq, A_Wk, A_Wv, A_Wo, A_seg_len, B_x, B_w1, B_w3, B_w2, c, w_mod):

    def _A_ref(x, mem0, Wq, Wk, Wv, Wo, seg_len):
        B, S, Dm = x.shape
        H, Dh = (Wq.shape[1], Wq.shape[2])
        M = mem0.shape[1]
        scale = Dh ** (-0.5)
        n_seg = S // seg_len
        L = M + seg_len
        idx = jnp.arange(L)
        mask = (idx[:, None] < M) | (idx[:, None] >= idx[None, :])
        mem = mem0
        outs = []
        for s in range(n_seg):
            xs = x[:, s * seg_len:(s + 1) * seg_len, :].copy()
            h = jnp.concatenate([mem, xs], axis=1)
            q = jnp.einsum('btd,dhe->bhte', h, Wq)
            k = jnp.einsum('btd,dhe->bhte', h, Wk)
            v = jnp.einsum('btd,dhe->bhte', h, Wv)
            scores = jnp.einsum('bhqe,bhke->bhqk', q, k) * scale
            scores = jnp.where(mask[None, None], scores, -1000000000.0)
            p = _softmax(scores, axis=-1)
            o = jnp.einsum('bhqk,bhke->bhqe', p, v)
            o = jnp.einsum('bhte,hed->btd', o, Wo)
            mem = o[:, :M, :].copy()
            outs.append(o[:, M:, :])
        return jnp.concatenate(outs, axis=1)

    def _B_ref(x, w1, w3, w2):
        gate = jnp.einsum('bsd,df->bsf', x, w1)
        up = jnp.einsum('bsd,df->bsf', x, w3)
        h = _silu(gate) * up
        out = jnp.einsum('bsf,fd->bsd', h, w2)
        return out
    x = A_x
    mod = (_silu(c) @ w_mod).reshape(c.shape[0], 6, 1, -1)
    sa, ca, ga, sb, cb, gb = (mod[:, 0].copy(), mod[:, 1].copy(), mod[:, 2].copy(), mod[:, 3].copy(), mod[:, 4].copy(), mod[:, 5].copy())
    h = _layernorm(x, axis=-1) * (1 + ca) + sa
    x = x + ga * _A_ref(h, A_mem0, A_Wq, A_Wk, A_Wv, A_Wo, A_seg_len)
    h = _layernorm(x, axis=-1) * (1 + cb) + sb
    x = x + gb * _B_ref(h, B_w1, B_w3, B_w2)
    return x
```

```python
import functools

import jax
import jax.numpy as jnp
from jax import lax
import jax.experimental.pallas as pl
import jax.experimental.pallas.tpu as pltpu

F32 = jnp.float32
BF16 = jnp.bfloat16
U32 = jnp.uint32
LANE = 128
HG = 4
KCH = 256
RP = 32
NSTG = 4
FM = 256
FC = 512


def _mm(a, b):
    return lax.dot_general(a, b, (((1,), (0,)), ((), ())), preferred_element_type=F32)


def _mm_nt(a, b):
    return lax.dot_general(a, b, (((1,), (1,)), ((), ())), preferred_element_type=F32)


def _rnd(v):
    return v.astype(BF16).astype(F32)


def _norm(x):
    m = jnp.mean(x, axis=-1, keepdims=True)
    xc = x - m
    v = jnp.mean(xc * xc, axis=-1, keepdims=True)
    return xc * lax.rsqrt(v + 1e-5)


def _kernel(c_ref, mem0_ref, x_hbm, wq_hbm, wk_hbm, wv_hbm, wo_hbm, w1_hbm, w3_hbm, w2_hbm,
            wmod_hbm, out_hbm,
            xb, h2b, wqkv, wo, w1, w3, w2, wmod, stg, mod, hin, oprev, ob,
            sem_x, sem_mod, sem_stg, sem_wo, sem_ffn, sem_out, *, seg, n_heads):
    S, D = xb.shape
    M = mem0_ref.shape[0]
    L = M + seg
    H = n_heads
    F = w1.shape[1]
    n_seg = S // seg
    n_grp = H // HG
    n_ct = D // LANE
    n_kch = D // KCH
    scale = float(LANE) ** -0.5

    mod_cp = [pltpu.make_async_copy(wmod_hbm.at[:, pl.ds(0, 2 * D)], wmod.at[:, pl.ds(0, 2 * D)],
                                    sem_mod.at[0]),
              pltpu.make_async_copy(wmod_hbm.at[:, pl.ds(2 * D, 4 * D)],
                                    wmod.at[:, pl.ds(2 * D, 4 * D)], sem_mod.at[1])]
    x_cp = pltpu.make_async_copy(x_hbm, xb, sem_x.at[0])
    chunks = [(t, kc) for t in range(3) for kc in range(n_kch)]

    def stg_cp(i):
        t, kc = chunks[i]
        src = (wq_hbm, wk_hbm, wv_hbm)[t]
        return pltpu.make_async_copy(src.at[pl.ds(kc * KCH * H, KCH * H), :], stg.at[i % NSTG],
                                     sem_stg.at[i % NSTG])

    wo_cp = [pltpu.make_async_copy(wo_hbm.at[:, pl.ds(j * LANE, LANE)], wo.at[j], sem_wo.at[j])
             for j in range(n_ct)]
    ffn_cp = [pltpu.make_async_copy(a, b, sem_ffn.at[i])
              for i, (a, b) in enumerate(((w1_hbm, w1), (w3_hbm, w3), (w2_hbm, w2)))]

    for i in range(NSTG):
        stg_cp(i).start()
    mod_cp[0].start()
    x_cp.start()

    stg32 = stg.bitcast(U32)
    for i, (t, kc) in enumerate(chunks):
        stg_cp(i).wait()

        def repack(r, carry, i=i, t=t, kc=kc):
            nw = RP * (H // 2)
            src = stg32.at[i % NSTG, pl.ds(pl.multiple_of(r * nw, nw), nw), :]
            rows = pl.ds(pl.multiple_of(kc * (KCH // 2) + r * (RP // 2), RP // 2), RP // 2)
            for hp in range(H // 2):
                a = src[pl.ds(hp, RP // 2, stride=H), :]
                b = src[pl.ds(hp + H // 2, RP // 2, stride=H), :]
                wqkv[t, 2 * hp, rows, :] = (a & jnp.uint32(0xFFFF)) | (b << 16)
                wqkv[t, 2 * hp + 1, rows, :] = (a >> 16) | (b & jnp.uint32(0xFFFF0000))
            return carry

        lax.fori_loop(0, KCH // RP, repack, 0)
        if i + NSTG < len(chunks):
            stg_cp(i + NSTG).start()
        if i + NSTG == len(chunks) - 1:
            for cp in wo_cp:
                cp.start()
            mod_cp[1].start()

    cv = c_ref[...].astype(F32)
    sc = jnp.broadcast_to(_rnd(cv * jax.nn.sigmoid(cv)), (8, D))
    mod_cp[0].wait()
    for j in range(2):
        mod[j] = _mm(sc, wmod[:, j * D:(j + 1) * D])
    x_cp.wait()
    mod_cp[1].wait()
    for cp in ffn_cp:
        cp.start()
    for j in range(2, 6):
        mod[j] = _mm(sc, wmod[:, j * D:(j + 1) * D])
    for cp in wo_cp:
        cp.wait()

    def mrow(j):
        return mod[j, 0:1, :]

    def pre_attn(s):
        xs = xb[pl.ds(pl.multiple_of(s * seg, seg), seg), :].astype(F32)
        return _rnd(_norm(xs) * (1.0 + mrow(1)) + mrow(0))

    def post_attn(s):
        rows = pl.ds(pl.multiple_of(s * seg, seg), seg)
        x1 = (xb[rows, :].astype(F32) + mrow(2) * oprev[...]).astype(BF16)
        xb[rows, :] = x1
        h2b[rows, :] = (_norm(x1.astype(F32)) * (1.0 + mrow(4)) + mrow(3)).astype(BF16)

    hin[0:M, :] = mem0_ref[...].astype(F32)
    hin[M:L, :] = pre_attn(0)
    oprev[...] = jnp.zeros(oprev.shape, F32)

    def step(s, carry):
        h = hin[...]
        ri = lax.broadcasted_iota(jnp.int32, (L, L), 0)
        ci = lax.broadcasted_iota(jnp.int32, (L, L), 1)
        mask = (ri < M) | (ri >= ci)
        qkv, prob, att = {}, {}, {}

        def proj(g):
            w = jnp.concatenate([pltpu.bitcast(wqkv[t, g * HG + j], BF16)
                                 for t in range(3) for j in range(HG)], axis=1)
            qkv[g] = _mm(h, w)

        def part(g, t, j):
            o = (t * HG + j) * LANE
            return qkv[g][:, o:o + LANE]

        def scores(g):
            prob[g] = []
            for j in range(HG):
                sv = _mm_nt(_rnd(part(g, 0, j)), part(g, 1, j).astype(BF16)) * scale
                sv = jnp.where(mask, sv, -1e9)
                e = jnp.exp(sv - jnp.max(sv, axis=-1, keepdims=True))
                prob[g].append(_rnd(e / jnp.sum(e, axis=-1, keepdims=True)))

        def values(g):
            att[g] = [_rnd(_mm(prob[g][j], part(g, 2, j).astype(BF16))) for j in range(HG)]

        def outp(g0, g1):
            a = jnp.concatenate([v for g in range(g0, g1) for v in att[g]], axis=1)
            rows = pl.ds(g0 * HG * LANE, (g1 - g0) * HG * LANE)
            return _mm(a, jnp.concatenate([wo[j, rows, :] for j in range(n_ct)], axis=1))

        for g in range(n_grp):
            proj(g)
            if g == 0:
                post_attn(jnp.maximum(s - 1, 0))
            if g == 1:
                nxt = pre_attn(jnp.minimum(s + 1, n_seg - 1))
            if g >= 1:
                scores(g - 1)
            if g >= 2:
                values(g - 2)
        acc = outp(0, 1)
        scores(n_grp - 1)
        values(n_grp - 2)
        acc = acc + outp(1, 3)
        values(n_grp - 1)
        acc = acc + outp(3, n_grp)
        hin[0:M, :] = _rnd(acc[0:M])
        hin[M:L, :] = nxt
        oprev[...] = acc[M:L]
        return carry

    lax.fori_loop(0, n_seg, step, 0)
    post_attn(n_seg - 1)

    for cp in ffn_cp:
        cp.wait()
    n_blk = S // FM

    def out_cp(b):
        return pltpu.make_async_copy(ob.at[b % 2], out_hbm.at[pl.ds(b * FM, FM), :],
                                     sem_out.at[b % 2])

    def ffn(b, carry):
        rows = pl.ds(pl.multiple_of(b * FM, FM), FM)

        @pl.when(b >= 2)
        def _():
            out_cp(b - 2).wait()

        hh = h2b[rows, :]
        acts = []
        for f in range(F // FC):
            cols = slice(f * FC, (f + 1) * FC)
            gt = _mm(hh, w1[:, cols])
            up = _mm(hh, w3[:, cols])
            acts.append((gt * jax.nn.sigmoid(gt) * up).astype(BF16))
        y = _mm(jnp.concatenate(acts, axis=1), w2[...])
        ob[b % 2] = (xb[rows, :].astype(F32) + mrow(5) * y).astype(ob.dtype)
        out_cp(b).start()
        return carry

    lax.fori_loop(0, n_blk, ffn, 0)
    for b in range(max(n_blk - 2, 0), n_blk):
        out_cp(b).wait()


@functools.partial(jax.jit, static_argnames=("A_seg_len",))
def pallas_adaLN_cond__memory_aug_recurrent_mem_tr__glu_gated_swiglu__prompt_kernel(
    A_x, A_mem0, A_Wq, A_Wk, A_Wv, A_Wo, A_seg_len, B_x, B_w1, B_w3, B_w2, c, w_mod,
):
    del B_x
    B, S, D = A_x.shape
    H, Dh = A_Wq.shape[1], A_Wq.shape[2]
    M = A_mem0.shape[1]
    F = B_w1.shape[1]
    seg = int(A_seg_len)
    assert B == 1 and Dh == LANE and S % seg == 0 and S % FM == 0 and F % FC == 0
    hbm = pl.BlockSpec(memory_space=pl.ANY)
    vmem = pl.BlockSpec(memory_space=pltpu.VMEM)
    dma = pltpu.SemaphoreType.DMA
    out = pl.pallas_call(
        functools.partial(_kernel, seg=seg, n_heads=H),
        out_shape=jax.ShapeDtypeStruct((S, D), A_x.dtype),
        in_specs=[vmem, vmem] + [hbm] * 9,
        out_specs=hbm,
        scratch_shapes=[
            pltpu.VMEM((S, D), BF16),
            pltpu.VMEM((S, D), BF16),
            pltpu.VMEM((3, H, D // 2, LANE), U32),
            pltpu.VMEM((D // LANE, H * Dh, LANE), BF16),
            pltpu.VMEM((D, F), BF16),
            pltpu.VMEM((D, F), BF16),
            pltpu.VMEM((F, D), BF16),
            pltpu.VMEM((D, 6 * D), BF16),
            pltpu.VMEM((NSTG, KCH * H, LANE), BF16),
            pltpu.VMEM((6, 8, D), F32),
            pltpu.VMEM((M + seg, D), F32),
            pltpu.VMEM((seg, D), F32),
            pltpu.VMEM((2, FM, D), A_x.dtype),
            dma((1,)), dma((2,)), dma((NSTG,)), dma((D // LANE,)), dma((3,)), dma((2,)),
        ],
        compiler_params=pltpu.CompilerParams(vmem_limit_bytes=120 * 2**20),
    )(c, A_mem0.reshape(M, D), A_x.reshape(S, D), A_Wq.reshape(D * H, Dh),
      A_Wk.reshape(D * H, Dh), A_Wv.reshape(D * H, Dh), A_Wo.reshape(H * Dh, D),
      B_w1, B_w3, B_w2, w_mod)
    return out.reshape(B, S, D)
```

```python
import functools

import jax
import jax.numpy as jnp
from jax import lax
import jax.experimental.pallas as pl
import jax.experimental.pallas.tpu as pltpu

F32 = jnp.float32
BF16 = jnp.bfloat16
U32 = jnp.uint32
LANE = 128
HG = 4
HC = 8
RP = 64
NSTG = 4
PRE = 8
FM = 256
FC = 512


def _mm(a, b):
    return lax.dot_general(a, b, (((1,), (0,)), ((), ())), preferred_element_type=F32)


def _mm_nt(a, b):
    return lax.dot_general(a, b, (((1,), (1,)), ((), ())), preferred_element_type=F32)


def _rnd(v):
    return v.astype(BF16).astype(F32)


def _norm(x):
    m = jnp.mean(x, axis=-1, keepdims=True)
    xc = x - m
    v = jnp.mean(xc * xc, axis=-1, keepdims=True)
    return xc * lax.rsqrt(v + 1e-5)


def _kernel(c_ref, mem0_ref, x_hbm, wq_hbm, wk_hbm, wv_hbm, wo_hbm, w1_hbm, w3_hbm, w2_hbm,
            wmod_hbm, out_hbm,
            xb, xp, ab, wqkv, pre, wo, w1, w3, w2, wmod, stg, tmp, mod, hp, hin, h2b, x1b, ob,
            sem_x, sem_mod, sem_stg, sem_wo, sem_ffn, sem_out):
    n_seg, seg, D = xb.shape
    S = n_seg * seg
    M = mem0_ref.shape[0]
    L = M + seg
    LR = L - PRE
    H = wq_hbm.shape[1]
    F = w1.shape[1]
    n_grp = H // HG
    n_ct = D // LANE
    n_hc = H // HC
    n_chunk = 3 * n_hc
    scale = float(LANE) ** -0.5

    mod_cp = [pltpu.make_async_copy(wmod_hbm.at[:, pl.ds(a * D, n * D)],
                                    wmod.at[:, pl.ds(a * D, n * D)], sem_mod.at[i])
              for i, (a, n) in enumerate(((0, 1), (1, 1), (2, 4)))]
    xp_cp = pltpu.make_async_copy(x_hbm.at[:, pl.ds(seg - PRE, PRE), :], xp, sem_x.at[0])
    x_cp = pltpu.make_async_copy(x_hbm, xb, sem_x.at[1])

    def stg_cp(t, hc, slot):
        src = (wq_hbm, wk_hbm, wv_hbm)[t]
        return pltpu.make_async_copy(src.at[:, pl.ds(pl.multiple_of(hc * HC, HC), HC), :],
                                     stg.at[slot], sem_stg.at[slot])

    wo_cp = [pltpu.make_async_copy(wo_hbm.at[:, pl.ds(j * LANE, LANE)], wo.at[j], sem_wo.at[j])
             for j in range(n_ct)]
    ffn_cp = [pltpu.make_async_copy(a, b, sem_ffn.at[i])
              for i, (a, b) in enumerate(((w1_hbm, w1), (w3_hbm, w3), (w2_hbm, w2)))]

    stg_cp(0, 0, 0).start()
    xp_cp.start()
    mod_cp[0].start()
    mod_cp[1].start()

    def repack(i):
        hw = HC // 2
        for r in range(D // RP):
            v = pltpu.bitcast(stg[i % NSTG, pl.ds(r * RP, RP)].reshape(RP * HC, LANE), U32)
            tmp[pl.ds(r * RP * hw, RP * hw), :] = v
        for r in range(D // RP):
            rows = pl.ds(r * (RP // 2), RP // 2)
            for j in range(hw):
                a = tmp[pl.ds(r * RP * hw + j, RP // 2, stride=2 * hw), :]
                b = tmp[pl.ds(r * RP * hw + hw + j, RP // 2, stride=2 * hw), :]
                wqkv[i * HC + 2 * j, rows, :] = (a & jnp.uint32(0xFFFF)) | (b << 16)
                wqkv[i * HC + 2 * j + 1, rows, :] = (a >> 16) | (b & jnp.uint32(0xFFFF0000))

    def pre_proj(i):
        w = jnp.concatenate([pltpu.bitcast(wqkv[i * HC + j], BF16) for j in range(HC)], axis=1)
        r = _mm(hp[...], w)
        for j in range(HC):
            pre[i * HC + j] = r[:, j * LANE:(j + 1) * LANE]

    def mrow(j):
        return mod[j, 0:1, :]

    cv = c_ref[...].astype(F32)
    sc = jnp.broadcast_to(_rnd(cv * jax.nn.sigmoid(cv)), (8, D))
    stg_cp(0, 0, 0).wait()
    repack(0)
    xp_cp.wait()
    xn = _norm(xp[...].astype(F32).reshape(n_seg * PRE, D))
    mod_cp[0].wait()
    stg_cp(0, 1, 1).start()
    mod[0] = _mm(sc, wmod[:, 0:D])
    mod_cp[1].wait()
    for i in range(2, NSTG):
        stg_cp(i // n_hc, i % n_hc, i).start()
    mod[1] = _mm(sc, wmod[:, D:2 * D])
    hp[...] = (xn * (1.0 + mrow(1)) + mrow(0)).astype(BF16)

    def warm(i, carry):
        nx = i + NSTG
        for t in range(3):
            @pl.when(nx // n_hc == t)
            def _(t=t):
                stg_cp(t, nx % n_hc, nx % NSTG).start()

        @pl.when(i == 1)
        def _():
            x_cp.start()

        @pl.when(i == 3)
        def _():
            for cp in wo_cp:
                cp.start()

        stg_cp(0, 0, (i + 1) % NSTG).wait()
        pre_proj(i)
        repack(i + 1)
        return carry

    lax.fori_loop(0, n_chunk - 1, warm, 0)
    mod_cp[2].start()
    for cp in ffn_cp:
        cp.start()
    x_cp.wait()
    for cp in wo_cp:
        cp.wait()
    pre_proj(n_chunk - 1)

    def pre_attn(s):
        xs = xb[s].astype(F32)[0:seg - PRE]
        return _norm(xs) * (1.0 + mrow(1)) + mrow(0)

    hin[...] = jnp.concatenate([mem0_ref[...].astype(F32), pre_attn(0)], axis=0).astype(BF16)

    def step(s, carry):
        h = hin[...]
        ri = lax.broadcasted_iota(jnp.int32, (L, L), 0)
        ci = lax.broadcasted_iota(jnp.int32, (L, L), 1)
        mask = (ri < M) | (ri >= ci)
        prow = pl.ds(pl.multiple_of(s * PRE, PRE), PRE)
        qkv, prob, att = {}, {}, {}

        def proj(g):
            w = jnp.concatenate([pltpu.bitcast(wqkv[t * H + g * HG + j], BF16)
                                 for t in range(3) for j in range(HG)], axis=1)
            qkv[g] = _mm(h, w)

        def part(g, t, j):
            o = (t * HG + j) * LANE
            return jnp.concatenate([qkv[g][:, o:o + LANE], pre[t * H + g * HG + j, prow, :]], axis=0)

        def scores(g):
            prob[g] = []
            for j in range(HG):
                sv = _mm_nt(_rnd(part(g, 0, j)), part(g, 1, j).astype(BF16)) * scale
                sv = jnp.where(mask, sv, -1e9)
                e = jnp.exp(sv - jnp.max(sv, axis=-1, keepdims=True))
                prob[g].append(_rnd(e / jnp.sum(e, axis=-1, keepdims=True)))

        def values(g):
            att[g] = [_rnd(_mm(prob[g][j], part(g, 2, j).astype(BF16))) for j in range(HG)]

        def outp(g0, g1):
            a = jnp.concatenate([v for g in range(g0, g1) for v in att[g]], axis=1)
            rows = pl.ds(g0 * HG * LANE, (g1 - g0) * HG * LANE)
            return _mm(a, jnp.concatenate([wo[j, rows, :] for j in range(n_ct)], axis=1))

        for g in range(n_grp):
            proj(g)
            if g == 1:
                nxt = pre_attn(jnp.minimum(s + 1, n_seg - 1))
            if g >= 1:
                scores(g - 1)
            if g >= 2:
                values(g - 2)
        acc = outp(0, 1)
        scores(n_grp - 1)
        values(n_grp - 2)
        acc = acc + outp(1, 3)
        values(n_grp - 1)
        acc = acc + outp(3, n_grp)
        hin[...] = jnp.concatenate([acc[0:M], nxt], axis=0).astype(BF16)
        ab[s] = acc[M:L].astype(BF16)
        return carry

    lax.fori_loop(0, n_seg, step, 0)

    mod_cp[2].wait()
    for cp in ffn_cp:
        cp.wait()
    for j in range(2, 6):
        mod[j] = _mm(sc, wmod[:, j * D:(j + 1) * D])
    n_blk = S // FM
    spb = FM // seg

    def post_attn(b, slot):
        segs = pl.ds(b * spb, spb)
        x1 = xb[segs].astype(F32).reshape(FM, D) + mrow(2) * ab[segs].astype(F32).reshape(FM, D)
        x1b[slot] = x1
        h2b[slot] = (_norm(x1) * (1.0 + mrow(4)) + mrow(3)).astype(BF16)

    def out_cp(b):
        return pltpu.make_async_copy(ob.at[b % 2], out_hbm.at[pl.ds(b * FM, FM), :],
                                     sem_out.at[b % 2])

    post_attn(0, 0)

    def ffn(b, carry):
        @pl.when(b >= 2)
        def _():
            out_cp(b - 2).wait()

        hh = h2b[b % 2]
        acts = []
        for f in range(F // FC):
            cols = slice(f * FC, (f + 1) * FC)
            gt = _mm(hh, w1[:, cols])
            up = _mm(hh, w3[:, cols])
            acts.append((gt * jax.nn.sigmoid(gt) * up).astype(BF16))
        post_attn(jnp.minimum(b + 1, n_blk - 1), (b + 1) % 2)
        y = _mm(jnp.concatenate(acts, axis=1), w2[...])
        ob[b % 2] = (x1b[b % 2] + mrow(5) * y).astype(ob.dtype)
        out_cp(b).start()
        return carry

    lax.fori_loop(0, n_blk, ffn, 0)
    for b in range(max(n_blk - 2, 0), n_blk):
        out_cp(b).wait()


@functools.partial(jax.jit, static_argnames=("A_seg_len",))
def pallas_adaLN_cond__memory_aug_recurrent_mem_tr__glu_gated_swiglu__prompt_kernel(
    A_x, A_mem0, A_Wq, A_Wk, A_Wv, A_Wo, A_seg_len, B_x, B_w1, B_w3, B_w2, c, w_mod,
):
    del B_x
    B, S, D = A_x.shape
    H, Dh = A_Wq.shape[1], A_Wq.shape[2]
    M = A_mem0.shape[1]
    F = B_w1.shape[1]
    seg = int(A_seg_len)
    n_seg = S // seg
    assert B == 1 and Dh == LANE and S % seg == 0 and S % FM == 0 and F % FC == 0
    hbm = pl.BlockSpec(memory_space=pl.ANY)
    vmem = pl.BlockSpec(memory_space=pltpu.VMEM)
    dma = pltpu.SemaphoreType.DMA
    out = pl.pallas_call(
        _kernel,
        out_shape=jax.ShapeDtypeStruct((S, D), A_x.dtype),
        in_specs=[vmem, vmem] + [hbm] * 9,
        out_specs=hbm,
        scratch_shapes=[
            pltpu.VMEM((n_seg, seg, D), BF16),
            pltpu.VMEM((n_seg, PRE, D), BF16),
            pltpu.VMEM((n_seg, seg, D), BF16),
            pltpu.VMEM((3 * H, D // 2, LANE), U32),
            pltpu.VMEM((3 * H, n_seg * PRE, LANE), F32),
            pltpu.VMEM((D // LANE, H * Dh, LANE), BF16),
            pltpu.VMEM((D, F), BF16),
            pltpu.VMEM((D, F), BF16),
            pltpu.VMEM((F, D), BF16),
            pltpu.VMEM((D, 6 * D), BF16),
            pltpu.VMEM((NSTG, D, HC, LANE), BF16),
            pltpu.VMEM((D * HC // 2, LANE), U32),
            pltpu.VMEM((6, 8, D), F32),
            pltpu.VMEM((n_seg * PRE, D), BF16),
            pltpu.VMEM((M + seg - PRE, D), BF16),
            pltpu.VMEM((2, FM, D), BF16),
            pltpu.VMEM((2, FM, D), F32),
            pltpu.VMEM((2, FM, D), A_x.dtype),
            dma((2,)), dma((3,)), dma((NSTG,)), dma((D // LANE,)), dma((3,)), dma((2,)),
        ],
        compiler_params=pltpu.CompilerParams(vmem_limit_bytes=126 * 2**20),
    )(c, A_mem0.reshape(M, D), A_x.reshape(n_seg, seg, D), A_Wq, A_Wk, A_Wv,
      A_Wo.reshape(H * Dh, D), B_w1, B_w3, B_w2, w_mod)
    return out.reshape(B, S, D)
```

```python
import functools

import jax
import jax.numpy as jnp
from jax import lax
import jax.experimental.pallas as pl
import jax.experimental.pallas.tpu as pltpu

F32 = jnp.float32
BF16 = jnp.bfloat16
U32 = jnp.uint32
LANE = 128
HG = 4
HC = 8
RP = 64
VLAG = 3
NSTG = 4
PRE = 8
FM = 256
FC = 512


def _mm(a, b):
    return lax.dot_general(a, b, (((1,), (0,)), ((), ())), preferred_element_type=F32)


def _mm_nt(a, b):
    return lax.dot_general(a, b, (((1,), (1,)), ((), ())), preferred_element_type=F32)


def _rnd(v):
    return v.astype(BF16).astype(F32)


def _pack(v):
    return pltpu.bitcast(v.astype(BF16), U32)


def _unpack(v):
    return pltpu.bitcast(v, BF16)


def _norm(x):
    m = jnp.mean(x, axis=-1, keepdims=True)
    xc = x - m
    v = jnp.mean(xc * xc, axis=-1, keepdims=True)
    return xc * lax.rsqrt(v + 1e-5)


def _kernel(c_ref, mem0_ref, x_hbm, wq_hbm, wk_hbm, wv_hbm, wo_hbm, w1_hbm, w3_hbm, w2_hbm,
            wmod_hbm, out_hbm,
            xb, xp, ab, wqkv, pre, wo, w1, w3, w2, wmod, stg, tmp, mod, hp, hin, h2b, x1b, ob,
            sem_x, sem_mod, sem_stg, sem_wo, sem_ffn, sem_out):
    n_seg, seg, D = xb.shape
    S = n_seg * seg
    M = mem0_ref.shape[0]
    L = M + seg
    LR = L - PRE
    H = wq_hbm.shape[1]
    F = w1.shape[1]
    n_grp = H // HG
    n_ct = D // LANE
    n_hc = H // HC
    n_chunk = 3 * n_hc
    scale = float(LANE) ** -0.5

    mod_cp = [pltpu.make_async_copy(wmod_hbm.at[:, pl.ds(a * D, n * D)],
                                    wmod.at[:, pl.ds(a * D, n * D)], sem_mod.at[i])
              for i, (a, n) in enumerate(((0, 1), (1, 1), (2, 4)))]
    xp_cp = pltpu.make_async_copy(x_hbm.at[:, pl.ds(seg - PRE, PRE), :], xp, sem_x.at[0])
    x_cp = pltpu.make_async_copy(x_hbm, xb, sem_x.at[1])

    def stg_cp(t, hc, slot):
        src = (wq_hbm, wk_hbm, wv_hbm)[t]
        return pltpu.make_async_copy(src.at[:, pl.ds(pl.multiple_of(hc * HC, HC), HC), :],
                                     stg.at[slot], sem_stg.at[slot])

    wo_cp = [pltpu.make_async_copy(wo_hbm.at[:, pl.ds(j * LANE, LANE)], wo.at[j], sem_wo.at[j])
             for j in range(n_ct)]
    ffn_cp = [pltpu.make_async_copy(a, b, sem_ffn.at[i])
              for i, (a, b) in enumerate(((w1_hbm, w1), (w3_hbm, w3), (w2_hbm, w2)))]

    xp_cp.start()
    mod_cp[0].start()
    mod_cp[1].start()

    hw = HC // 2

    def flatten(slot):
        for r in range(D // RP):
            v = stg[slot, pl.ds(r * RP, RP)].reshape(RP * HC, LANE)
            tmp[pl.ds(r * RP * hw, RP * hw), :] = pltpu.bitcast(v, U32)

    def pre_proj(i):
        for j0 in range(0, hw, 2):
            ws = []
            for j in range(j0, j0 + 2):
                a = tmp[pl.ds(j, D, stride=hw), :]
                for k, half in enumerate((a << 16, a & jnp.uint32(0xFFFF0000))):
                    ws.append(_pack(pltpu.bitcast(half, F32)))
                    wqkv[i * HC + 2 * j + k] = ws[-1]
            r = _mm(_unpack(hp[...]), jnp.concatenate([_unpack(w) for w in ws], axis=1))
            for k in range(4):
                pre[i * HC + 2 * j0 + k] = r[:, k * LANE:(k + 1) * LANE]

    def mrow(j):
        return mod[j, 0:1, :]

    cv = c_ref[...].astype(F32)
    sc = jnp.broadcast_to(_rnd(cv * jax.nn.sigmoid(cv)), (8, D))
    xp_cp.wait()
    xn = _norm(xp[...].astype(F32).reshape(n_seg * PRE, D))
    mod_cp[0].wait()
    stg_cp(0, 0, 0).start()
    mod[0] = _mm(sc, wmod[:, 0:D])
    mod_cp[1].wait()
    for i in range(1, NSTG - 1):
        stg_cp(i // n_hc, i % n_hc, i).start()
    mod[1] = _mm(sc, wmod[:, D:2 * D])
    hp[...] = _pack(xn * (1.0 + mrow(1)) + mrow(0))

    def warm(i, carry):
        nx = i + NSTG - 1
        for t in range(3):
            @pl.when(nx // n_hc == t)
            def _(t=t):
                stg_cp(t, nx % n_hc, nx % NSTG).start()

        @pl.when(i == 1)
        def _():
            x_cp.start()

        @pl.when(i == 3)
        def _():
            for cp in wo_cp:
                cp.start()

        stg_cp(0, 0, i % NSTG).wait()
        flatten(i % NSTG)
        pre_proj(i)
        return carry

    lax.fori_loop(0, n_chunk, warm, 0)
    mod_cp[2].start()
    for cp in ffn_cp:
        cp.start()
    x_cp.wait()
    for cp in wo_cp:
        cp.wait()

    def pre_attn(s):
        xs = xb[s].astype(F32)[0:seg - PRE]
        return _norm(xs) * (1.0 + mrow(1)) + mrow(0)

    hin[...] = _pack(jnp.concatenate([mem0_ref[...].astype(F32), pre_attn(0)], axis=0))

    def step(s, carry):
        h = _unpack(hin[...])
        ri = lax.broadcasted_iota(jnp.int32, (L, L), 0)
        ci = lax.broadcasted_iota(jnp.int32, (L, L), 1)
        mask = (ri < M) | (ri >= ci)
        prow = pl.ds(pl.multiple_of(s * PRE, PRE), PRE)
        qkv, prob, att = {}, {}, {}

        def proj(g, ts):
            w = jnp.concatenate([_unpack(wqkv[t * H + g * HG + j])
                                 for t in ts for j in range(HG)], axis=1)
            r = _mm(h, w)
            for i, t in enumerate(ts):
                for j in range(HG):
                    o = (i * HG + j) * LANE
                    qkv[g, t, j] = r[:, o:o + LANE]

        def part(g, t, j):
            return jnp.concatenate([qkv[g, t, j], pre[t * H + g * HG + j, prow, :]], axis=0)

        def scores(g):
            prob[g] = []
            for j in range(HG):
                sv = _mm_nt(_rnd(part(g, 0, j)), part(g, 1, j).astype(BF16)) * scale
                sv = jnp.where(mask, sv, -1e9)
                e = jnp.exp(sv - jnp.max(sv, axis=-1, keepdims=True))
                prob[g].append(_rnd(e / jnp.sum(e, axis=-1, keepdims=True)))

        def values(g):
            att[g] = [_rnd(_mm(prob[g][j], part(g, 2, j).astype(BF16))) for j in range(HG)]

        def outp(g0, g1):
            a = jnp.concatenate([v for g in range(g0, g1) for v in att[g]], axis=1)
            rows = pl.ds(g0 * HG * LANE, (g1 - g0) * HG * LANE)
            return _mm(a, jnp.concatenate([wo[j, rows, :] for j in range(n_ct)], axis=1))

        for g in range(n_grp):
            proj(g, (0, 1))
            if g == 1:
                nxt = pre_attn(jnp.minimum(s + 1, n_seg - 1))
            if g >= 1:
                scores(g - 1)
        for g in range(n_grp):
            proj(g, (2,))
            if g == 0:
                scores(n_grp - 1)
            if g >= VLAG:
                values(g - VLAG)
        for g in range(n_grp - VLAG, n_grp):
            values(g)
        acc = outp(0, n_grp)
        hin[...] = _pack(jnp.concatenate([acc[0:M], nxt], axis=0))
        ab[s] = acc[M:L].astype(BF16)
        return carry

    lax.fori_loop(0, n_seg, step, 0)

    mod_cp[2].wait()
    for cp in ffn_cp:
        cp.wait()
    for j in range(2, 6):
        mod[j] = _mm(sc, wmod[:, j * D:(j + 1) * D])
    n_blk = S // FM
    spb = FM // seg

    def post_attn(b, slot):
        segs = pl.ds(b * spb, spb)
        x1 = xb[segs].astype(F32).reshape(FM, D) + mrow(2) * ab[segs].astype(F32).reshape(FM, D)
        x1b[slot] = x1
        h2b[slot] = (_norm(x1) * (1.0 + mrow(4)) + mrow(3)).astype(BF16)

    def out_cp(b):
        return pltpu.make_async_copy(ob.at[b % 2], out_hbm.at[pl.ds(b * FM, FM), :],
                                     sem_out.at[b % 2])

    post_attn(0, 0)

    def ffn(b, carry):
        @pl.when(b >= 2)
        def _():
            out_cp(b - 2).wait()

        hh = h2b[b % 2]
        acts = []
        for f in range(F // FC):
            cols = slice(f * FC, (f + 1) * FC)
            gt = _mm(hh, w1[:, cols])
            up = _mm(hh, w3[:, cols])
            acts.append((gt * jax.nn.sigmoid(gt) * up).astype(BF16))
        post_attn(jnp.minimum(b + 1, n_blk - 1), (b + 1) % 2)
        y = _mm(jnp.concatenate(acts, axis=1), w2[...])
        ob[b % 2] = (x1b[b % 2] + mrow(5) * y).astype(ob.dtype)
        out_cp(b).start()
        return carry

    lax.fori_loop(0, n_blk, ffn, 0)
    for b in range(max(n_blk - 2, 0), n_blk):
        out_cp(b).wait()


@functools.partial(jax.jit, static_argnames=("A_seg_len",))
def pallas_adaLN_cond__memory_aug_recurrent_mem_tr__glu_gated_swiglu__prompt_kernel(
    A_x, A_mem0, A_Wq, A_Wk, A_Wv, A_Wo, A_seg_len, B_x, B_w1, B_w3, B_w2, c, w_mod,
):
    del B_x
    B, S, D = A_x.shape
    H, Dh = A_Wq.shape[1], A_Wq.shape[2]
    M = A_mem0.shape[1]
    F = B_w1.shape[1]
    seg = int(A_seg_len)
    n_seg = S // seg
    assert B == 1 and Dh == LANE and S % seg == 0 and S % FM == 0 and F % FC == 0
    hbm = pl.BlockSpec(memory_space=pl.ANY)
    vmem = pl.BlockSpec(memory_space=pltpu.VMEM)
    dma = pltpu.SemaphoreType.DMA
    out = pl.pallas_call(
        _kernel,
        out_shape=jax.ShapeDtypeStruct((S, D), A_x.dtype),
        in_specs=[vmem, vmem] + [hbm] * 9,
        out_specs=hbm,
        scratch_shapes=[
            pltpu.VMEM((n_seg, seg, D), BF16),
            pltpu.VMEM((n_seg, PRE, D), BF16),
            pltpu.VMEM((n_seg, seg, D), BF16),
            pltpu.VMEM((3 * H, D // 2, LANE), U32),
            pltpu.VMEM((3 * H, n_seg * PRE, LANE), F32),
            pltpu.VMEM((D // LANE, H * Dh, LANE), BF16),
            pltpu.VMEM((D, F), BF16),
            pltpu.VMEM((D, F), BF16),
            pltpu.VMEM((F, D), BF16),
            pltpu.VMEM((D, 6 * D), BF16),
            pltpu.VMEM((NSTG, D, HC, LANE), BF16),
            pltpu.VMEM((D * HC // 2, LANE), U32),
            pltpu.VMEM((6, 8, D), F32),
            pltpu.VMEM((n_seg * PRE // 2, D), U32),
            pltpu.VMEM(((M + seg - PRE) // 2, D), U32),
            pltpu.VMEM((2, FM, D), BF16),
            pltpu.VMEM((2, FM, D), F32),
            pltpu.VMEM((2, FM, D), A_x.dtype),
            dma((2,)), dma((3,)), dma((NSTG,)), dma((D // LANE,)), dma((3,)), dma((2,)),
        ],
        compiler_params=pltpu.CompilerParams(vmem_limit_bytes=126 * 2**20),
    )(c, A_mem0.reshape(M, D), A_x.reshape(n_seg, seg, D), A_Wq, A_Wk, A_Wv,
      A_Wo.reshape(H * Dh, D), B_w1, B_w3, B_w2, w_mod)
    return out.reshape(B, S, D)
```

```python
import functools

import jax
import jax.numpy as jnp
from jax import lax
import jax.experimental.pallas as pl
import jax.experimental.pallas.tpu as pltpu

F32 = jnp.float32
BF16 = jnp.bfloat16
U32 = jnp.uint32
LANE = 128
HG = 4
HC = 8
RP = 64
VLAG = 3
LATE = 1
UNR = 2
NSTG = 4
PRE = 8
FM = 128
FC = 256


def _mm(a, b):
    return lax.dot_general(a, b, (((1,), (0,)), ((), ())), preferred_element_type=F32)


def _mm_nt(a, b):
    return lax.dot_general(a, b, (((1,), (1,)), ((), ())), preferred_element_type=F32)


def _rnd(v):
    return v.astype(BF16).astype(F32)


def _pack(v):
    return pltpu.bitcast(v.astype(BF16), U32)


def _unpack(v):
    return pltpu.bitcast(v, BF16)


def _lhs7(a11, a12, a21, a22):
    return (a11 + a22, a21 + a22, a11, a22, a11 + a12, a21 - a11, a12 - a22)


def _rhs7(b11, b12, b21, b22):
    return (b11 + b22, b11, b12 - b22, b21 - b11, b22, b11 + b12, b21 + b22)


def _out4(m):
    return (m[0] + m[3] - m[4] + m[6], m[2] + m[4], m[1] + m[3], m[0] - m[1] + m[2] + m[5])


def _norm(x):
    m = jnp.mean(x, axis=-1, keepdims=True)
    xc = x - m
    v = jnp.mean(xc * xc, axis=-1, keepdims=True)
    return xc * lax.rsqrt(v + 1e-5)


def _kernel(c_ref, mem0_ref, x_hbm, wq_hbm, wk_hbm, wv_hbm, wo_hbm, w1_hbm, w3_hbm, w2_hbm,
            wmod_hbm, out_hbm,
            xb, ab, w1, w3, w2, wmod, mod, h2b, x1b, ob,
            sem_x, sem_mod, sem_stg, sem_wo, sem_ffn, sem_out):
    n_seg, seg, D = xb.shape
    S = n_seg * seg
    M = mem0_ref.shape[0]
    L = M + seg
    LR = L - PRE
    H = wq_hbm.shape[1]
    F = w1.shape[1]
    n_grp = H // HG
    n_ct = D // LANE
    n_hc = H // HC
    n_chunk = 3 * n_hc
    scale = float(LANE) ** -0.5

    mod_cp = [pltpu.make_async_copy(wmod_hbm.at[:, pl.ds(a * D, n * D)],
                                    wmod.at[:, pl.ds(a * D, n * D)], sem_mod.at[i])
              for i, (a, n) in enumerate(((0, 1), (1, 1), (2, 4)))]
    ffn_cp = [pltpu.make_async_copy(a, b, sem_ffn.at[i])
              for i, (a, b) in enumerate(((w1_hbm, w1), (w3_hbm, w3), (w2_hbm, w2)))]

    def mrow(j):
        return mod[j, 0:1, :]

    cv = c_ref[...].astype(F32)
    sc = jnp.broadcast_to(_rnd(cv * jax.nn.sigmoid(cv)), (8, D))

    def attention(xp, wqkv, pre, wo, stg, tmp, hp, hin):
        xp_cp = pltpu.make_async_copy(x_hbm.at[:, pl.ds(seg - PRE, PRE), :], xp, sem_x.at[0])
        x_cp = pltpu.make_async_copy(x_hbm, xb, sem_x.at[1])

        def stg_cp(t, hc, slot):
            src = (wq_hbm, wk_hbm, wv_hbm)[t]
            return pltpu.make_async_copy(src.at[:, pl.ds(pl.multiple_of(hc * HC, HC), HC), :],
                                         stg.at[slot], sem_stg.at[slot])

        wo_cp = [pltpu.make_async_copy(wo_hbm.at[:, pl.ds(j * LANE, LANE)], wo.at[j], sem_wo.at[j])
                 for j in range(n_ct)]


        xp_cp.start()
        mod_cp[0].start()
        mod_cp[1].start()

        hw = HC // 2

        def flatten(slot):
            for r in range(D // RP):
                v = stg[slot, pl.ds(r * RP, RP)].reshape(RP * HC, LANE)
                tmp[pl.ds(r * RP * hw, RP * hw), :] = pltpu.bitcast(v, U32)

        def pre_proj(i):
            for j0 in range(0, hw, 2):
                ws = []
                for j in range(j0, j0 + 2):
                    a = tmp[pl.ds(j, D, stride=hw), :]
                    for k, half in enumerate((a << 16, a & jnp.uint32(0xFFFF0000))):
                        ws.append(_pack(pltpu.bitcast(half, F32)))
                        wqkv[i * HC + 2 * j + k] = ws[-1]
                r = _mm(_unpack(hp[...]), jnp.concatenate([_unpack(w) for w in ws], axis=1))
                for k in range(4):
                    pre[i * HC + 2 * j0 + k] = r[:, k * LANE:(k + 1) * LANE]


        xp_cp.wait()
        xn = _norm(xp[...].astype(F32).reshape(n_seg * PRE, D))
        mod_cp[0].wait()
        stg_cp(0, 0, 0).start()
        mod[0] = _mm(sc, wmod[:, 0:D])
        mod_cp[1].wait()
        for i in range(1, NSTG):
            stg_cp(i // n_hc, i % n_hc, i).start()
        mod[1] = _mm(sc, wmod[:, D:2 * D])
        hp[...] = _pack(xn * (1.0 + mrow(1)) + mrow(0))

        def warm(i, carry):
            slot = lax.rem(i, NSTG)
            stg_cp(0, 0, slot).wait()
            flatten(slot)
            pre_proj(i)
            nx = i + NSTG
            for t in range(3):
                @pl.when(lax.div(nx, n_hc) == t)
                def _(t=t):
                    stg_cp(t, lax.rem(nx, n_hc), slot).start()

            @pl.when(i == 0)
            def _():
                x_cp.start()

            @pl.when(i == 2)
            def _():
                for cp in wo_cp:
                    cp.start()

            return carry

        lax.fori_loop(0, n_chunk, warm, 0)
        x_cp.wait()
        for cp in wo_cp:
            cp.wait()

        def pre_attn(s):
            xs = xb[s].astype(F32)[0:seg - PRE]
            return _norm(xs) * (1.0 + mrow(1)) + mrow(0)

        hin[...] = _pack(jnp.concatenate([mem0_ref[...].astype(F32), pre_attn(0)], axis=0))

        def step(s, carry):
            h = _unpack(hin[...])
            ri = lax.broadcasted_iota(jnp.int32, (L, L), 0)
            ci = lax.broadcasted_iota(jnp.int32, (L, L), 1)
            mask = (ri < M) | (ri >= ci)
            prow = pl.ds(pl.multiple_of(s * PRE, PRE), PRE)
            qkv, prob, att = {}, {}, {}

            def proj(g, ts):
                w = jnp.concatenate([_unpack(wqkv[t * H + g * HG + j])
                                     for t in ts for j in range(HG)], axis=1)
                r = _mm(h, w)
                for i, t in enumerate(ts):
                    for j in range(HG):
                        o = (i * HG + j) * LANE
                        qkv[g, t, j] = r[:, o:o + LANE]

            def part(g, t, j):
                return jnp.concatenate([qkv[g, t, j], pre[t * H + g * HG + j, prow, :]], axis=0)

            def scores(g):
                prob[g] = []
                for j in range(HG):
                    sv = _mm_nt(_rnd(part(g, 0, j)), part(g, 1, j).astype(BF16)) * scale
                    sv = jnp.where(mask, sv, -1e9)
                    e = jnp.exp(sv - jnp.max(sv, axis=-1, keepdims=True))
                    prob[g].append(_rnd(e / jnp.sum(e, axis=-1, keepdims=True)))

            def values(g):
                att[g] = [_rnd(_mm(prob[g][j], part(g, 2, j).astype(BF16))) for j in range(HG)]

            def outp(g0, g1):
                a = jnp.concatenate([v for g in range(g0, g1) for v in att[g]], axis=1)
                rows = pl.ds(g0 * HG * LANE, (g1 - g0) * HG * LANE)
                return _mm(a, jnp.concatenate([wo[j, rows, :] for j in range(n_ct)], axis=1))

            for g in range(n_grp):
                proj(g, (0, 1))
                if g == 1:
                    nxt = pre_attn(jnp.minimum(s + 1, n_seg - 1))
                if g >= 1:
                    scores(g - 1)
            for g in range(n_grp):
                proj(g, (2,))
                if g == 0:
                    scores(n_grp - 1)
                if g >= VLAG:
                    values(g - VLAG)
            for g in range(n_grp - VLAG, n_grp):
                values(g)
            acc = outp(0, n_grp)
            hin[...] = _pack(jnp.concatenate([acc[0:M], nxt], axis=0))
            ab[s] = acc[M:L].astype(BF16)
            return carry

        def steps(k, carry):
            @pl.when(k == LATE)
            def _():
                mod_cp[2].start()
                for cp in ffn_cp:
                    cp.start()

            for u in range(UNR):
                step(k * UNR + u, carry)
            return carry

        lax.fori_loop(0, n_seg // UNR, steps, 0)

    pl.run_scoped(
        attention,
        pltpu.VMEM((n_seg, PRE, D), BF16),
        pltpu.VMEM((3 * H, D // 2, LANE), U32),
        pltpu.VMEM((3 * H, n_seg * PRE, LANE), F32),
        pltpu.VMEM((n_ct, H * LANE, LANE), BF16),
        pltpu.VMEM((NSTG, D, HC, LANE), BF16),
        pltpu.VMEM((D * HC // 2, LANE), U32),
        pltpu.VMEM((n_seg * PRE // 2, D), U32),
        pltpu.VMEM((LR // 2, D), U32))

    def swiglu(wu, wd):
        mod_cp[2].wait()
        for cp in ffn_cp:
            cp.wait()
        for j in range(2, 6):
            mod[j] = _mm(sc, wmod[:, j * D:(j + 1) * D])
        n_blk = S // FM
        spb = FM // seg

        hm, hd, hf = FM // 2, D // 2, F // 2
        nft = F // LANE

        def up_ops(r, carry):
            top = pl.ds(pl.multiple_of(r * 16, 16), 16)
            bot = pl.ds(pl.multiple_of(hd + r * 16, 16), 16)
            ops = _rhs7(*(w[rows, :].astype(F32) for rows in (top, bot) for w in (w1, w3)))
            for i, o in enumerate(ops):
                wu[i, pl.ds(pl.multiple_of(r * 8, 8), 8), :] = _pack(o)
            return carry

        def down_ops(r, carry):
            top = pl.ds(pl.multiple_of(r * 64, 64), 64)
            bot = pl.ds(pl.multiple_of(hf + r * 64, 64), 64)
            ops = _rhs7(*(w2[rows, cols].astype(F32) for rows in (top, bot)
                          for cols in (slice(0, hd), slice(hd, D))))
            for i, o in enumerate(ops):
                wd[i, pl.ds(pl.multiple_of(r * 32, 32), 32), :] = _pack(o)
            return carry

        lax.fori_loop(0, hd // 16, up_ops, 0)
        lax.fori_loop(0, hf // 64, down_ops, 0)

        def post_attn(b, slot):
            segs = pl.ds(b * spb, spb)
            x1 = xb[segs].astype(F32).reshape(FM, D) + mrow(2) * ab[segs].astype(F32).reshape(FM, D)
            x1b[slot] = x1
            h2 = _norm(x1) * (1.0 + mrow(4)) + mrow(3)
            for i, o in enumerate(_lhs7(h2[:hm, :hd], h2[:hm, hd:], h2[hm:, :hd], h2[hm:, hd:])):
                h2b[slot, i] = _pack(o)

        def out_cp(b):
            return pltpu.make_async_copy(ob.at[b % 2], out_hbm.at[pl.ds(b * FM, FM), :],
                                         sem_out.at[b % 2])

        post_attn(0, 0)

        def ffn(b, carry):
            @pl.when(b >= 2)
            def _():
                out_cp(b - 2).wait()

            slot = lax.rem(b, 2)
            hh = [_unpack(h2b[slot, i]) for i in range(7)]

            def act(cols):
                g1, u1, g2, u2 = _out4([
                    _mm(hh[i], jnp.concatenate([_unpack(wu[i, :, c]) for c in cols], axis=1))
                    for i in range(7)])
                return g1 * jax.nn.sigmoid(g1) * u1, g2 * jax.nn.sigmoid(g2) * u2

            lhs = []
            for f in range(hf // FC):
                a1, a2 = act((pl.ds(f * FC, FC), pl.ds(hf + f * FC, FC)))
                lhs.append([o.astype(BF16) for o in
                            _lhs7(a1[:, :FC], a1[:, FC:], a2[:, :FC], a2[:, FC:])])
            post_attn(jnp.minimum(b + 1, n_blk - 1), 1 - slot)
            y = _out4([_mm(jnp.concatenate([l[i] for l in lhs], axis=1), _unpack(wd[i]))
                       for i in range(7)])
            y = jnp.concatenate([jnp.concatenate(y[:2], axis=1), jnp.concatenate(y[2:], axis=1)],
                                axis=0)
            ob[slot] = (x1b[slot] + mrow(5) * y).astype(ob.dtype)
            out_cp(b).start()
            return carry

        lax.fori_loop(0, n_blk, ffn, 0)
        for b in range(max(n_blk - 2, 0), n_blk):
            out_cp(b).wait()

    pl.run_scoped(swiglu, pltpu.VMEM((7, D // 4, F), U32), pltpu.VMEM((7, F // 4, D // 2), U32))


@functools.partial(jax.jit, static_argnames=("A_seg_len",))
def pallas_adaLN_cond__memory_aug_recurrent_mem_tr__glu_gated_swiglu__prompt_kernel(
    A_x, A_mem0, A_Wq, A_Wk, A_Wv, A_Wo, A_seg_len, B_x, B_w1, B_w3, B_w2, c, w_mod,
):
    del B_x
    B, S, D = A_x.shape
    H, Dh = A_Wq.shape[1], A_Wq.shape[2]
    M = A_mem0.shape[1]
    F = B_w1.shape[1]
    seg = int(A_seg_len)
    n_seg = S // seg
    assert B == 1 and Dh == LANE and S % seg == 0 and S % FM == 0 and F % FC == 0
    hbm = pl.BlockSpec(memory_space=pl.ANY)
    vmem = pl.BlockSpec(memory_space=pltpu.VMEM)
    dma = pltpu.SemaphoreType.DMA
    out = pl.pallas_call(
        _kernel,
        out_shape=jax.ShapeDtypeStruct((S, D), A_x.dtype),
        in_specs=[vmem, vmem] + [hbm] * 9,
        out_specs=hbm,
        scratch_shapes=[
            pltpu.VMEM((n_seg, seg, D), BF16),
            pltpu.VMEM((n_seg, seg, D), BF16),
            pltpu.VMEM((D, F), BF16),
            pltpu.VMEM((D, F), BF16),
            pltpu.VMEM((F, D), BF16),
            pltpu.VMEM((D, 6 * D), BF16),
            pltpu.VMEM((6, 8, D), F32),
            pltpu.VMEM((2, 7, FM // 4, D // 2), U32),
            pltpu.VMEM((2, FM, D), F32),
            pltpu.VMEM((2, FM, D), A_x.dtype),
            dma((2,)), dma((3,)), dma((NSTG,)), dma((D // LANE,)), dma((3,)), dma((2,)),
        ],
        compiler_params=pltpu.CompilerParams(vmem_limit_bytes=126 * 2**20),
    )(c, A_mem0.reshape(M, D), A_x.reshape(n_seg, seg, D), A_Wq, A_Wk, A_Wv,
      A_Wo.reshape(H * Dh, D), B_w1, B_w3, B_w2, w_mod)
    return out.reshape(B, S, D)
```

```python
import functools

import jax
import jax.numpy as jnp
from jax import lax
import jax.experimental.pallas as pl
import jax.experimental.pallas.tpu as pltpu

F32 = jnp.float32
BF16 = jnp.bfloat16
U32 = jnp.uint32
LANE = 128
HG = 4
HC = 8
RP = 64
VLAG = 3
DR = 64
UNR = 2
TIE = 3
NSTG = 4
PRE = 8
FM = 128
FC = 256


def _mm(a, b):
    return lax.dot_general(a, b, (((1,), (0,)), ((), ())), preferred_element_type=F32)


def _mm_nt(a, b):
    return lax.dot_general(a, b, (((1,), (1,)), ((), ())), preferred_element_type=F32)


def _rnd(v):
    return v.astype(BF16).astype(F32)


def _pack(v):
    return pltpu.bitcast(v.astype(BF16), U32)


def _unpack(v):
    return pltpu.bitcast(v, BF16)


def _lhs7(a11, a12, a21, a22):
    return (a11 + a22, a21 + a22, a11, a22, a11 + a12, a21 - a11, a12 - a22)


def _rhs7(b11, b12, b21, b22):
    return (b11 + b22, b11, b12 - b22, b21 - b11, b22, b11 + b12, b21 + b22)


def _out4(m):
    return (m[0] + m[3] - m[4] + m[6], m[2] + m[4], m[1] + m[3], m[0] - m[1] + m[2] + m[5])


def _after(v, token, i):
    return jnp.where(i < 0, pltpu.bitcast(token, v.dtype), v)


def _norm(x):
    m = jnp.mean(x, axis=-1, keepdims=True)
    xc = x - m
    v = jnp.mean(xc * xc, axis=-1, keepdims=True)
    return xc * lax.rsqrt(v + 1e-5)


def _kernel(c_ref, mem0_ref, x_hbm, wq_hbm, wk_hbm, wv_hbm, wo_hbm, w1_hbm, w3_hbm, w2_hbm,
            wmod_hbm, out_hbm,
            xb, ab, wqkv, pre, wo, mod, hin, ru, rd, h2b, ob,
            sem_x, sem_mod, sem_stg, sem_wo, sem_raw, sem_out):
    n_seg, seg, D = xb.shape
    M = mem0_ref.shape[0]
    L = M + seg
    H = wq_hbm.shape[1]
    F = w1_hbm.shape[1]
    n_grp, n_ct, n_hc = H // HG, D // LANE, H // HC
    n_it = n_seg // UNR
    n_blk, spb = n_seg * seg // FM, FM // seg
    hd, hf = D // 2, F // 2
    ur, dr = ru.shape[2], rd.shape[2]
    n_dr = hf // dr
    scale = float(LANE) ** -0.5

    def mrow(j):
        return mod[j, 0:1, :]

    x_cp = pltpu.make_async_copy(x_hbm, xb, sem_x.at[1])
    wo_cp = [pltpu.make_async_copy(wo_hbm.at[:, pl.ds(j * LANE, LANE)], wo.at[j], sem_wo.at[j])
             for j in range(n_ct)]

    def raw_cp(k, slot):
        kd = jnp.minimum(k, n_dr - 1)
        cps = [pltpu.make_async_copy(w.at[pl.ds(pl.multiple_of(o + k * ur, ur), ur), :],
                                     ru.at[slot, 2 * i + j], sem_raw.at[slot, 2 * i + j])
               for i, o in enumerate((0, hd)) for j, w in enumerate((w1_hbm, w3_hbm))]
        return cps + [
            pltpu.make_async_copy(w2_hbm.at[pl.ds(pl.multiple_of(o + kd * dr, dr), dr), :],
                                  rd.at[slot, i], sem_raw.at[slot, 4 + i])
            for i, o in enumerate((0, hf))]

    def warmup(xp, wmod, stg, tmp, hp):
        hw, hr = HC // 2, n_seg * PRE // 2
        mod_cp = [pltpu.make_async_copy(wmod_hbm.at[:, pl.ds(a * D, n * D)],
                                        wmod.at[:, pl.ds(a * D, n * D)], sem_mod.at[i])
                  for i, (a, n) in enumerate(((0, 1), (1, 1), (2, 4)))]
        xp_cp = pltpu.make_async_copy(x_hbm.at[:, pl.ds(seg - PRE, PRE), :], xp, sem_x.at[0])

        def stg_cp(t, hc, slot):
            src = (wq_hbm, wk_hbm, wv_hbm)[t]
            return pltpu.make_async_copy(src.at[:, pl.ds(pl.multiple_of(hc * HC, HC), HC), :],
                                         stg.at[slot], sem_stg.at[slot])

        xp_cp.start()
        mod_cp[0].start()
        mod_cp[1].start()
        cv = c_ref[...].astype(F32)
        sc = jnp.broadcast_to(_rnd(cv * jax.nn.sigmoid(cv)), (8, D))
        xp_cp.wait()
        xn = _norm(xp[...].astype(F32).reshape(2 * hr, D))
        mod_cp[0].wait()
        stg_cp(0, 0, 0).start()
        mod[0] = _mm(sc, wmod[:, 0:D])
        mod_cp[1].wait()
        for i in range(1, NSTG):
            stg_cp(i // n_hc, i % n_hc, i).start()
        mod[1] = _mm(sc, wmod[:, D:2 * D])
        h = xn * (1.0 + mrow(1)) + mrow(0)
        for i, o in enumerate(_lhs7(h[:hr, :hd], h[:hr, hd:], h[hr:, :hd], h[hr:, hd:])):
            hp[i] = _pack(o)

        def warm(i, carry):
            slot = lax.rem(i, NSTG)
            stg_cp(0, 0, slot).wait()
            for r in range(D // RP):
                v = stg[slot, pl.ds(r * RP, RP)].reshape(RP * HC, LANE)
                tmp[pl.ds(r * RP * hw, RP * hw), :] = pltpu.bitcast(v, U32)
            ops = []
            for j in range(hw):
                quad = []
                for half in range(2):
                    a = tmp[pl.ds(half * hd * hw + j, hd, stride=hw), :]
                    for k, w in enumerate((a << 16, a & jnp.uint32(0xFFFF0000))):
                        quad.append(pltpu.bitcast(w, F32))
                        wqkv[i * HC + 2 * j + k, pl.ds(half * hd // 2, hd // 2), :] = (
                            _pack(quad[-1]))
                ops.append([o.astype(BF16) for o in _rhs7(*quad)])
            prod = {n: _mm(_unpack(hp[n]), jnp.concatenate([o[n] for o in ops], axis=1))
                    for n in (1, 5, 0, 2, 3, 4, 6)}
            c4 = _out4(prod)
            for n, cq in enumerate(c4):
                for j in range(hw):
                    pre[i * HC + 2 * j + n % 2, pl.ds((n // 2) * hr, hr), :] = (
                        cq[:, j * LANE:(j + 1) * LANE])
            nx = i + NSTG
            for t in range(3):
                @pl.when(lax.div(nx, n_hc) == t)
                def _(t=t):
                    stg_cp(t, lax.rem(nx, n_hc), slot).start()

            for at, cps in ((0, [x_cp]), (2, wo_cp[:n_ct // 2]), (4, wo_cp[n_ct // 2:]),
                            (6, [mod_cp[2]] + raw_cp(0, 0))):
                @pl.when(i == at)
                def _(cps=cps):
                    for cp in cps:
                        cp.start()

            return carry

        lax.fori_loop(0, 3 * n_hc, warm, 0)
        mod_cp[2].wait()

        def mod_rest(j, carry):
            mod[j] = _mm(sc, wmod[:, pl.ds(pl.multiple_of(j * D, D), D)])
            return carry

        lax.fori_loop(2, 6, mod_rest, 0)

    pl.run_scoped(warmup,
                  pltpu.VMEM((n_seg, PRE, D), BF16),
                  pltpu.VMEM((D, 6 * D), BF16),
                  pltpu.VMEM((NSTG, D, HC, LANE), BF16),
                  pltpu.VMEM((D * HC // 2, LANE), U32),
                  pltpu.VMEM((7, n_seg * PRE // 4, hd), U32))
    x_cp.wait()
    for cp in wo_cp:
        cp.wait()

    def pre_attn(s):
        xs = xb[s].astype(F32)[0:seg - PRE]
        return _norm(xs) * (1.0 + mrow(1)) + mrow(0)

    def step(s, side):
        h = _unpack(hin[...])
        ri = lax.broadcasted_iota(jnp.int32, (L, L), 0)
        ci = lax.broadcasted_iota(jnp.int32, (L, L), 1)
        mask = (ri < M) | (ri >= ci)
        prow = pl.ds(pl.multiple_of(s * PRE, PRE), PRE)
        qkv, prob, att = {}, {}, {}

        def proj(g, ts):
            heads = [(t, g * HG + j) for t in ts for j in range(HG)]
            r = _mm(h, jnp.concatenate([_unpack(wqkv[t * H + n]) for t, n in heads], axis=1))
            for i, (t, n) in enumerate(heads):
                early = pre[t * H + n, prow, :]
                if (t, n) in side:
                    early = side[t, n](early)
                qkv[t, n] = jnp.concatenate([r[:, i * LANE:(i + 1) * LANE], early], axis=0)

        def scores(g):
            for n in range(g * HG, (g + 1) * HG):
                sv = _mm_nt(_rnd(qkv[0, n]), qkv[1, n].astype(BF16)) * scale
                sv = jnp.where(mask, sv, -1e9)
                e = jnp.exp(sv - jnp.max(sv, axis=-1, keepdims=True))
                prob[n] = _rnd(e / jnp.sum(e, axis=-1, keepdims=True))

        def values(g):
            for n in range(g * HG, (g + 1) * HG):
                att[n] = _rnd(_mm(prob[n], qkv[2, n].astype(BF16)))

        nxt = pre_attn(jnp.minimum(s + 1, n_seg - 1))
        for g in range(n_grp):
            proj(g, (0, 1))
            if g >= 1:
                scores(g - 1)
        for g in range(n_grp):
            proj(g, (2,))
            if g == 0:
                scores(n_grp - 1)
            if g >= VLAG:
                values(g - VLAG)
        for g in range(n_grp - VLAG, n_grp):
            values(g)
        acc = _mm(jnp.concatenate([att[n] for n in range(H)], axis=1),
                  jnp.concatenate([wo[j] for j in range(n_ct)], axis=1))
        hin[...] = _pack(jnp.concatenate([acc[0:M], nxt], axis=0))
        ab[s] = acc[M:L].astype(BF16)

    def main(wu, wd):
        def steps(k, carry):
            slot = lax.rem(k, 2)
            for cp in raw_cp(k, slot):
                cp.wait()

            @pl.when(k + 1 < n_it)
            def _():
                for cp in raw_cp(k + 1, 1 - slot):
                    cp.start()

            kd = jnp.minimum(k, n_dr - 1)

            def up_piece(c, v):
                cols = pl.ds(c * LANE, LANE)
                for i, o in enumerate(_rhs7(*(ru[slot, j, :, cols].astype(F32)
                                              for j in range(4)))):
                    wu[k, i, :, cols] = _pack(o)
                return _after(v, wu[jnp.minimum(k, n_it), 0, 0:8, cols], k)

            def down_piece(r, c, v):
                rows, cols = pl.ds(r * 8, 8), pl.ds(c * LANE, LANE)
                for i, o in enumerate(_rhs7(*(
                        rd[slot, j, pl.ds(r * 16, 16), pl.ds(o + c * LANE, LANE)].astype(F32)
                        for j in range(2) for o in (0, hd)))):
                    wd[kd, i, rows, cols] = _pack(o)
                return _after(v, wd[jnp.minimum(kd, n_it), 0, rows, cols], k)

            pieces = [functools.partial(up_piece, c) for c in range(F // LANE)]
            pieces += [functools.partial(down_piece, r, c)
                       for r in range(dr // 16) for c in range(hd // LANE)]
            spots = [(u, t, n) for u in range(UNR) for t, m in ((1, 2), (2, 4))
                     for n in range(0, H, m)]
            assert len(pieces) <= len(spots)
            for u in range(UNR):
                step(k * UNR + u, {sp[1:]: f for sp, f in zip(spots, pieces) if sp[0] == u})
            return carry

        hin[...] = _pack(jnp.concatenate([mem0_ref[...].astype(F32), pre_attn(0)], axis=0))
        lax.fori_loop(0, n_it, steps, 0)

        hm = FM // 2

        def resid(b):
            segs = pl.ds(b * spb, spb)
            return (xb[segs].astype(F32).reshape(FM, D)
                    + mrow(2) * ab[segs].astype(F32).reshape(FM, D))

        def ffn_in(b, slot):
            h2 = _norm(resid(b)) * (1.0 + mrow(4)) + mrow(3)
            for i, o in enumerate(_lhs7(h2[:hm, :hd], h2[:hm, hd:], h2[hm:, :hd], h2[hm:, hd:])):
                h2b[slot, i] = _pack(o)

        def out_cp(b):
            return pltpu.make_async_copy(ob.at[b % 2], out_hbm.at[pl.ds(b * FM, FM), :],
                                         sem_out.at[b % 2])

        def ffn(b, carry):
            @pl.when(b >= 2)
            def _():
                out_cp(b - 2).wait()

            slot = lax.rem(b, 2)
            hh = [_unpack(h2b[slot, i]) for i in range(7)]
            lhs = []
            for f in range(hf // FC):
                cols = (pl.ds(f * FC, FC), pl.ds(hf + f * FC, FC))
                g1, u1, g2, u2 = _out4([
                    _mm(hh[i], jnp.concatenate([_unpack(wu[:, i, :, c].reshape(hd // 2, FC)) for c in cols], axis=1))
                    for i in range(7)])
                a1, a2 = g1 * jax.nn.sigmoid(g1) * u1, g2 * jax.nn.sigmoid(g2) * u2
                lhs.append([o.astype(BF16) for o in
                            _lhs7(a1[:, :FC], a1[:, FC:], a2[:, :FC], a2[:, FC:])])
            ffn_in(jnp.minimum(b + 1, n_blk - 1), 1 - slot)
            token = h2b[jnp.minimum(1 - slot, 1), 0, :, 0:FC]
            lhs[-1][TIE] = _unpack(_after(pltpu.bitcast(lhs[-1][TIE], U32), token, b))
            y = _out4([_mm(jnp.concatenate([l[i] for l in lhs], axis=1),
                           _unpack(wd[:, i].reshape(hf // 2, hd)))
                       for i in range(7)])
            y = jnp.concatenate([jnp.concatenate(y[:2], axis=1),
                                 jnp.concatenate(y[2:], axis=1)], axis=0)
            ob[slot] = (resid(b) + mrow(5) * y).astype(ob.dtype)
            out_cp(b).start()
            return carry

        ffn_in(0, 0)
        lax.fori_loop(0, n_blk, ffn, 0)
        for b in range(n_blk - 2, n_blk):
            out_cp(b).wait()

    pl.run_scoped(main, pltpu.VMEM((n_it, 7, ur // 2, F), U32),
                  pltpu.VMEM((n_dr, 7, dr // 2, hd), U32))


@functools.partial(jax.jit, static_argnames=("A_seg_len",))
def pallas_adaLN_cond__memory_aug_recurrent_mem_tr__glu_gated_swiglu__prompt_kernel(
    A_x, A_mem0, A_Wq, A_Wk, A_Wv, A_Wo, A_seg_len, B_x, B_w1, B_w3, B_w2, c, w_mod,
):
    del B_x
    B, S, D = A_x.shape
    H, Dh = A_Wq.shape[1], A_Wq.shape[2]
    M = A_mem0.shape[1]
    F = B_w1.shape[1]
    seg = int(A_seg_len)
    n_seg = S // seg
    assert B == 1 and Dh == LANE and S % seg == 0 and S % FM == 0 and F % FC == 0
    hbm = pl.BlockSpec(memory_space=pl.ANY)
    vmem = pl.BlockSpec(memory_space=pltpu.VMEM)
    dma = pltpu.SemaphoreType.DMA
    out = pl.pallas_call(
        _kernel,
        out_shape=jax.ShapeDtypeStruct((S, D), A_x.dtype),
        in_specs=[vmem, vmem] + [hbm] * 9,
        out_specs=hbm,
        scratch_shapes=[
            pltpu.VMEM((n_seg, seg, D), BF16),
            pltpu.VMEM((n_seg, seg, D), BF16),
            pltpu.VMEM((3 * H, D // 2, LANE), U32),
            pltpu.VMEM((3 * H, n_seg * PRE, LANE), F32),
            pltpu.VMEM((D // LANE, H * Dh, LANE), BF16),
            pltpu.VMEM((6, 8, D), F32),
            pltpu.VMEM(((M + seg - PRE) // 2, D), U32),
            pltpu.VMEM((2, 4, D // 2 // (n_seg // UNR), F), BF16),
            pltpu.VMEM((2, 2, DR, D), BF16),
            pltpu.VMEM((2, 7, FM // 4, D // 2), U32),
            pltpu.VMEM((2, FM, D), A_x.dtype),
            dma((2,)), dma((3,)), dma((NSTG,)), dma((D // LANE,)), dma((2, 6)), dma((2,)),
        ],
        compiler_params=pltpu.CompilerParams(vmem_limit_bytes=124 * 2**20),
    )(c, A_mem0.reshape(M, D), A_x.reshape(n_seg, seg, D), A_Wq, A_Wk, A_Wv,
      A_Wo.reshape(H * Dh, D), B_w1, B_w3, B_w2, w_mod)
    return out.reshape(B, S, D)
```

```python
import functools

import jax
import jax.numpy as jnp
from jax import lax
import jax.experimental.pallas as pl
import jax.experimental.pallas.tpu as pltpu

F32 = jnp.float32
BF16 = jnp.bfloat16
U32 = jnp.uint32
LANE = 128
HG = 4
HC = 8
RP = 64
VLAG = 3
DR = 64
UNR = 2
NSTG = 4
PRE = 8
FM = 128
FC = 256


def _mm(a, b):
    return lax.dot_general(a, b, (((1,), (0,)), ((), ())), preferred_element_type=F32)


def _mm_nt(a, b):
    return lax.dot_general(a, b, (((1,), (1,)), ((), ())), preferred_element_type=F32)


def _rnd(v):
    return v.astype(BF16).astype(F32)


def _pack(v):
    return pltpu.bitcast(v.astype(BF16), U32)


def _unpack(v):
    return pltpu.bitcast(v, BF16)


def _lhs7(a11, a12, a21, a22):
    return (a11 + a22, a21 + a22, a11, a22, a11 + a12, a21 - a11, a12 - a22)


def _rhs7(b11, b12, b21, b22):
    return (b11 + b22, b11, b12 - b22, b21 - b11, b22, b11 + b12, b21 + b22)


def _out4(m):
    return (m[0] + m[3] - m[4] + m[6], m[2] + m[4], m[1] + m[3], m[0] - m[1] + m[2] + m[5])


def _after(v, token, i):
    return jnp.where(i < 0, pltpu.bitcast(token, v.dtype), v)


def _norm(x):
    m = jnp.mean(x, axis=-1, keepdims=True)
    xc = x - m
    v = jnp.mean(xc * xc, axis=-1, keepdims=True)
    return xc * lax.rsqrt(v + 1e-5)


def _kernel(c_ref, mem0_ref, x_hbm, wq_hbm, wk_hbm, wv_hbm, wo_hbm, w1_hbm, w3_hbm, w2_hbm,
            wmod_hbm, out_hbm,
            xb, ab, wqkv, pre, wo, mod, hin, ru, rd, h2b, ob,
            sem_x, sem_mod, sem_stg, sem_wo, sem_raw, sem_out):
    n_seg, seg, D = xb.shape
    M = mem0_ref.shape[0]
    L = M + seg
    H = wq_hbm.shape[1]
    F = w1_hbm.shape[1]
    n_grp, n_ct, n_hc = H // HG, D // LANE, H // HC
    n_it = n_seg // UNR
    n_blk, spb = n_seg * seg // FM, FM // seg
    hd, hf = D // 2, F // 2
    ur, dr = ru.shape[2], rd.shape[2]
    n_dr = hf // dr
    scale = float(LANE) ** -0.5

    def mrow(j):
        return mod[j, 0:1, :]

    x_cp = pltpu.make_async_copy(x_hbm, xb, sem_x.at[1])
    wo_cp = [pltpu.make_async_copy(wo_hbm.at[:, pl.ds(j * LANE, LANE)], wo.at[j], sem_wo.at[j])
             for j in range(n_ct)]

    def raw_cp(k, slot):
        kd = jnp.minimum(k, n_dr - 1)
        cps = [pltpu.make_async_copy(w.at[pl.ds(pl.multiple_of(o + k * ur, ur), ur), :],
                                     ru.at[slot, 2 * i + j], sem_raw.at[slot, 2 * i + j])
               for i, o in enumerate((0, hd)) for j, w in enumerate((w1_hbm, w3_hbm))]
        return cps + [
            pltpu.make_async_copy(w2_hbm.at[pl.ds(pl.multiple_of(o + kd * dr, dr), dr), :],
                                  rd.at[slot, i], sem_raw.at[slot, 4 + i])
            for i, o in enumerate((0, hf))]

    def warmup(xp, wmod, stg, tmp, hp):
        hw, hr = HC // 2, n_seg * PRE // 2
        mod_cp = [pltpu.make_async_copy(wmod_hbm.at[:, pl.ds(a * D, n * D)],
                                        wmod.at[:, pl.ds(a * D, n * D)], sem_mod.at[i])
                  for i, (a, n) in enumerate(((0, 1), (1, 1), (2, 4)))]
        xp_cp = pltpu.make_async_copy(x_hbm.at[:, pl.ds(seg - PRE, PRE), :], xp, sem_x.at[0])

        def stg_cp(t, hc, slot):
            src = (wq_hbm, wk_hbm, wv_hbm)[t]
            return pltpu.make_async_copy(src.at[:, pl.ds(pl.multiple_of(hc * HC, HC), HC), :],
                                         stg.at[slot], sem_stg.at[slot])

        xp_cp.start()
        mod_cp[0].start()
        mod_cp[1].start()
        cv = c_ref[...].astype(F32)
        sc = jnp.broadcast_to(_rnd(cv * jax.nn.sigmoid(cv)), (8, D))
        xp_cp.wait()
        xn = _norm(xp[...].astype(F32).reshape(2 * hr, D))
        mod_cp[0].wait()
        stg_cp(0, 0, 0).start()
        mod[0] = _mm(sc, wmod[:, 0:D])
        mod_cp[1].wait()
        for i in range(1, NSTG):
            stg_cp(i // n_hc, i % n_hc, i).start()
        mod[1] = _mm(sc, wmod[:, D:2 * D])
        h = xn * (1.0 + mrow(1)) + mrow(0)
        for i, o in enumerate(_lhs7(h[:hr, :hd], h[:hr, hd:], h[hr:, :hd], h[hr:, hd:])):
            hp[i] = _pack(o)

        def warm(i, carry):
            slot = lax.rem(i, NSTG)
            stg_cp(0, 0, slot).wait()
            for r in range(D // RP):
                v = stg[slot, pl.ds(r * RP, RP)].reshape(RP * HC, LANE)
                tmp[pl.ds(r * RP * hw, RP * hw), :] = pltpu.bitcast(v, U32)
            ops = []
            for j in range(hw):
                quad = []
                for half in range(2):
                    a = tmp[pl.ds(half * hd * hw + j, hd, stride=hw), :]
                    for k, w in enumerate((a << 16, a & jnp.uint32(0xFFFF0000))):
                        quad.append(pltpu.bitcast(w, F32))
                        wqkv[i * HC + 2 * j + k, pl.ds(half * hd // 2, hd // 2), :] = (
                            _pack(quad[-1]))
                ops.append([o.astype(BF16) for o in _rhs7(*quad)])
            prod = {n: _mm(_unpack(hp[n]), jnp.concatenate([o[n] for o in ops], axis=1))
                    for n in (1, 5, 0, 2, 3, 4, 6)}
            c4 = _out4(prod)
            for n, cq in enumerate(c4):
                for j in range(hw):
                    pre[i * HC + 2 * j + n % 2, pl.ds((n // 2) * hr, hr), :] = (
                        cq[:, j * LANE:(j + 1) * LANE])
            nx = i + NSTG
            for t in range(3):
                @pl.when(lax.div(nx, n_hc) == t)
                def _(t=t):
                    stg_cp(t, lax.rem(nx, n_hc), slot).start()

            for at, cps in ((0, [x_cp]), (2, wo_cp[:n_ct // 2]), (4, wo_cp[n_ct // 2:]),
                            (6, [mod_cp[2]] + raw_cp(0, 0))):
                @pl.when(i == at)
                def _(cps=cps):
                    for cp in cps:
                        cp.start()

            return carry

        lax.fori_loop(0, 3 * n_hc, warm, 0)
        mod_cp[2].wait()

        def mod_rest(j, carry):
            mod[j] = _mm(sc, wmod[:, pl.ds(pl.multiple_of(j * D, D), D)])
            return carry

        lax.fori_loop(2, 6, mod_rest, 0)

    pl.run_scoped(warmup,
                  pltpu.VMEM((n_seg, PRE, D), BF16),
                  pltpu.VMEM((D, 6 * D), BF16),
                  pltpu.VMEM((NSTG, D, HC, LANE), BF16),
                  pltpu.VMEM((D * HC // 2, LANE), U32),
                  pltpu.VMEM((7, n_seg * PRE // 4, hd), U32))
    x_cp.wait()
    for cp in wo_cp:
        cp.wait()

    def pre_attn(s):
        xs = xb[s].astype(F32)[0:seg - PRE]
        return _norm(xs) * (1.0 + mrow(1)) + mrow(0)

    def step(s, side):
        h = _unpack(hin[...])
        ri = lax.broadcasted_iota(jnp.int32, (L, L), 0)
        ci = lax.broadcasted_iota(jnp.int32, (L, L), 1)
        mask = (ri < M) | (ri >= ci)
        prow = pl.ds(pl.multiple_of(s * PRE, PRE), PRE)
        qkv, prob, att = {}, {}, {}

        def proj(g, ts):
            heads = [(t, g * HG + j) for t in ts for j in range(HG)]
            r = _mm(h, jnp.concatenate([_unpack(wqkv[t * H + n]) for t, n in heads], axis=1))
            for i, (t, n) in enumerate(heads):
                early = pre[t * H + n, prow, :]
                if (t, n) in side:
                    early = side[t, n](early)
                qkv[t, n] = jnp.concatenate([r[:, i * LANE:(i + 1) * LANE], early], axis=0)

        def scores(g):
            for n in range(g * HG, (g + 1) * HG):
                sv = _mm_nt(_rnd(qkv[0, n]), qkv[1, n].astype(BF16)) * scale
                sv = jnp.where(mask, sv, -1e9)
                e = jnp.exp(sv - jnp.max(sv, axis=-1, keepdims=True))
                prob[n] = _rnd(e / jnp.sum(e, axis=-1, keepdims=True))

        def values(g):
            for n in range(g * HG, (g + 1) * HG):
                att[n] = _rnd(_mm(prob[n], qkv[2, n].astype(BF16)))

        nxt = pre_attn(jnp.minimum(s + 1, n_seg - 1))
        for g in range(n_grp):
            proj(g, (0, 1))
            if g >= 1:
                scores(g - 1)
        for g in range(n_grp):
            proj(g, (2,))
            if g == 0:
                scores(n_grp - 1)
            if g >= VLAG:
                values(g - VLAG)
        for g in range(n_grp - VLAG, n_grp):
            values(g)
        acc = _mm(jnp.concatenate([att[n] for n in range(H)], axis=1),
                  jnp.concatenate([wo[j] for j in range(n_ct)], axis=1))
        hin[...] = _pack(jnp.concatenate([acc[0:M], nxt], axis=0))
        ab[s] = acc[M:L].astype(BF16)

    def main(wu, wd):
        def steps(k, carry):
            slot = lax.rem(k, 2)
            for cp in raw_cp(k, slot):
                cp.wait()

            @pl.when(k + 1 < n_it)
            def _():
                for cp in raw_cp(k + 1, 1 - slot):
                    cp.start()

            kd = jnp.minimum(k, n_dr - 1)

            def up_piece(c, v):
                cols = pl.ds(c * LANE, LANE)
                for i, o in enumerate(_rhs7(*(ru[slot, j, :, cols].astype(F32)
                                              for j in range(4)))):
                    wu[k, i, :, cols] = _pack(o)
                return _after(v, wu[jnp.minimum(k, n_it), 0, 0:8, cols], k)

            def down_piece(r, c, v):
                rows, cols = pl.ds(r * 8, 8), pl.ds(c * LANE, LANE)
                for i, o in enumerate(_rhs7(*(
                        rd[slot, j, pl.ds(r * 16, 16), pl.ds(o + c * LANE, LANE)].astype(F32)
                        for j in range(2) for o in (0, hd)))):
                    wd[kd, i, rows, cols] = _pack(o)
                return _after(v, wd[jnp.minimum(kd, n_it), 0, rows, cols], k)

            pieces = [functools.partial(up_piece, c) for c in range(F // LANE)]
            pieces += [functools.partial(down_piece, r, c)
                       for r in range(dr // 16) for c in range(hd // LANE)]
            spots = [(u, t, n) for u in range(UNR) for t, m in ((1, 2), (2, 4))
                     for n in range(0, H, m)]
            assert len(pieces) <= len(spots)
            for u in range(UNR):
                step(k * UNR + u, {sp[1:]: f for sp, f in zip(spots, pieces) if sp[0] == u})
            return carry

        hin[...] = _pack(jnp.concatenate([mem0_ref[...].astype(F32), pre_attn(0)], axis=0))
        lax.fori_loop(0, n_it, steps, 0)

        hm = FM // 2

        def resid(b):
            segs = pl.ds(b * spb, spb)
            return (xb[segs].astype(F32).reshape(FM, D)
                    + mrow(2) * ab[segs].astype(F32).reshape(FM, D))

        def ffn_in(b, slot, r):
            h2 = []
            for o in (r * 16, hm + r * 16):
                sg, rows = b * spb + o // seg, pl.ds(o % seg, 16)
                x1 = xb[sg, rows, :].astype(F32) + mrow(2) * ab[sg, rows, :].astype(F32)
                h2.append(_norm(x1) * (1.0 + mrow(4)) + mrow(3))
            for i, o in enumerate(_lhs7(h2[0][:, :hd], h2[0][:, hd:], h2[1][:, :hd], h2[1][:, hd:])):
                h2b[slot, i, pl.ds(r * 8, 8), :] = _pack(o)

        def out_cp(b):
            return pltpu.make_async_copy(ob.at[b % 2], out_hbm.at[pl.ds(b * FM, FM), :],
                                         sem_out.at[b % 2])

        def ffn(b, carry):
            @pl.when(b >= 2)
            def _():
                out_cp(b - 2).wait()

            slot = lax.rem(b, 2)
            hh = [_unpack(h2b[slot, i]) for i in range(7)]
            lhs = []
            for f in range(hf // FC):
                cols = (pl.ds(f * FC, FC), pl.ds(hf + f * FC, FC))
                g1, u1, g2, u2 = _out4([
                    _mm(hh[i], jnp.concatenate([_unpack(wu[:, i, :, c].reshape(hd // 2, FC)) for c in cols], axis=1))
                    for i in range(7)])
                a1, a2 = g1 * jax.nn.sigmoid(g1) * u1, g2 * jax.nn.sigmoid(g2) * u2
                lhs.append([o.astype(BF16) for o in
                            _lhs7(a1[:, :FC], a1[:, FC:], a2[:, :FC], a2[:, FC:])])
            prod = []
            for i in range(7):
                w = wd[:, i].reshape(hf // 2, hd)
                if 1 <= i <= hm // 16:
                    ffn_in(jnp.minimum(b + 1, n_blk - 1), 1 - slot, i - 1)
                    token = h2b[jnp.minimum(1 - slot, 1), 0, pl.ds((i - 1) * 8, 8), :]
                    w = jnp.concatenate([_after(w[:8], token, b), w[8:]], axis=0)
                prod.append(_mm(jnp.concatenate([l[i] for l in lhs], axis=1), _unpack(w)))
            y = _out4(prod)
            y = jnp.concatenate([jnp.concatenate(y[:2], axis=1),
                                 jnp.concatenate(y[2:], axis=1)], axis=0)
            ob[slot] = (resid(b) + mrow(5) * y).astype(ob.dtype)
            out_cp(b).start()
            return carry

        for r in range(hm // 16):
            ffn_in(0, 0, r)
        lax.fori_loop(0, n_blk, ffn, 0)
        for b in range(n_blk - 2, n_blk):
            out_cp(b).wait()

    pl.run_scoped(main, pltpu.VMEM((n_it, 7, ur // 2, F), U32),
                  pltpu.VMEM((n_dr, 7, dr // 2, hd), U32))


@functools.partial(jax.jit, static_argnames=("A_seg_len",))
def pallas_adaLN_cond__memory_aug_recurrent_mem_tr__glu_gated_swiglu__prompt_kernel(
    A_x, A_mem0, A_Wq, A_Wk, A_Wv, A_Wo, A_seg_len, B_x, B_w1, B_w3, B_w2, c, w_mod,
):
    del B_x
    B, S, D = A_x.shape
    H, Dh = A_Wq.shape[1], A_Wq.shape[2]
    M = A_mem0.shape[1]
    F = B_w1.shape[1]
    seg = int(A_seg_len)
    n_seg = S // seg
    assert B == 1 and Dh == LANE and S % seg == 0 and S % FM == 0 and F % FC == 0
    hbm = pl.BlockSpec(memory_space=pl.ANY)
    vmem = pl.BlockSpec(memory_space=pltpu.VMEM)
    dma = pltpu.SemaphoreType.DMA
    out = pl.pallas_call(
        _kernel,
        out_shape=jax.ShapeDtypeStruct((S, D), A_x.dtype),
        in_specs=[vmem, vmem] + [hbm] * 9,
        out_specs=hbm,
        scratch_shapes=[
            pltpu.VMEM((n_seg, seg, D), BF16),
            pltpu.VMEM((n_seg, seg, D), BF16),
            pltpu.VMEM((3 * H, D // 2, LANE), U32),
            pltpu.VMEM((3 * H, n_seg * PRE, LANE), F32),
            pltpu.VMEM((D // LANE, H * Dh, LANE), BF16),
            pltpu.VMEM((6, 8, D), F32),
            pltpu.VMEM(((M + seg - PRE) // 2, D), U32),
            pltpu.VMEM((2, 4, D // 2 // (n_seg // UNR), F), BF16),
            pltpu.VMEM((2, 2, DR, D), BF16),
            pltpu.VMEM((2, 7, FM // 4, D // 2), U32),
            pltpu.VMEM((2, FM, D), A_x.dtype),
            dma((2,)), dma((3,)), dma((NSTG,)), dma((D // LANE,)), dma((2, 6)), dma((2,)),
        ],
        compiler_params=pltpu.CompilerParams(vmem_limit_bytes=124 * 2**20),
    )(c, A_mem0.reshape(M, D), A_x.reshape(n_seg, seg, D), A_Wq, A_Wk, A_Wv,
      A_Wo.reshape(H * Dh, D), B_w1, B_w3, B_w2, w_mod)
    return out.reshape(B, S, D)
```

```python
import functools

import jax
import jax.numpy as jnp
from jax import lax
import jax.experimental.pallas as pl
import jax.experimental.pallas.tpu as pltpu

F32 = jnp.float32
BF16 = jnp.bfloat16
U32 = jnp.uint32
LANE = 128
HG = 4
HC = 8
RP = 64
VLAG = 3
SPOT = ((1, 3), (2, 2))
DR = 32
UNR = 2
NSTG = 4
PRE = 8
FM = 128
FC = 256


def _mm(a, b):
    return lax.dot_general(a, b, (((1,), (0,)), ((), ())), preferred_element_type=F32)


def _mm_nt(a, b):
    return lax.dot_general(a, b, (((1,), (1,)), ((), ())), preferred_element_type=F32)


def _rnd(v):
    return v.astype(BF16).astype(F32)


def _pack(v):
    return pltpu.bitcast(v.astype(BF16), U32)


def _unpack(v):
    return pltpu.bitcast(v, BF16)


_LHS = (((1, 0), (1, 3)), ((1, 2), (1, 3)), ((1, 0),), ((1, 3),), ((1, 0), (1, 1)),
        ((1, 2), (-1, 0)), ((1, 1), (-1, 3)))
_RHS = (((1, 0), (1, 3)), ((1, 0),), ((1, 1), (-1, 3)), ((1, 2), (-1, 0)), ((1, 3),),
        ((1, 0), (1, 1)), ((1, 2), (1, 3)))


def _comb(terms, quad):
    v = quad(terms[0][1])
    for sign, q in terms[1:]:
        v = v + quad(q) if sign > 0 else v - quad(q)
    return v


def _ops7(table, quads):
    return [_comb(t, quads.__getitem__) for t in table]


def _ops49(table, i, block):
    return _ops7(table, [
        _comb(table[i], lambda q: block(2 * (q // 2) + r, 2 * (q % 2) + c))
        for r in range(2) for c in range(2)])


def _out4(m):
    return (m[0] + m[3] - m[4] + m[6], m[2] + m[4], m[1] + m[3], m[0] - m[1] + m[2] + m[5])


def _out16(m):
    inner = [_out4(m[7 * i:7 * i + 7]) for i in range(7)]
    return {(2 * (q // 2) + p // 2, 2 * (q % 2) + p % 2): v
            for p in range(4) for q, v in enumerate(_out4([c[p] for c in inner]))}


def _after(v, token, i):
    return jnp.where(i < 0, pltpu.bitcast(token, v.dtype), v)


def _norm(x):
    m = jnp.mean(x, axis=-1, keepdims=True)
    xc = x - m
    v = jnp.mean(xc * xc, axis=-1, keepdims=True)
    return xc * lax.rsqrt(v + 1e-5)


def _kernel(c_ref, mem0_ref, x_hbm, wq_hbm, wk_hbm, wv_hbm, wo_hbm, w1_hbm, w3_hbm, w2_hbm,
            wmod_hbm, out_hbm,
            xb, ab, wqkv, pre, wo, mod, hin, ru, rd, h2f, h2b, ob,
            sem_x, sem_mod, sem_stg, sem_wo, sem_raw, sem_out):
    n_seg, seg, D = xb.shape
    M = mem0_ref.shape[0]
    L = M + seg
    H = wq_hbm.shape[1]
    F = w1_hbm.shape[2]
    n_grp, n_ct, n_hc = H // HG, D // LANE, H // HC
    n_it = n_seg // UNR
    n_blk, spb = n_seg * seg // FM, FM // seg
    hd, qd, qf = D // 2, D // 4, F // 4
    n_dr = qf // DR
    scale = float(LANE) ** -0.5

    def mrow(j):
        return mod[j, 0:1, :]

    x_cp = pltpu.make_async_copy(x_hbm, xb, sem_x.at[1])
    wo_cp = [pltpu.make_async_copy(wo_hbm.at[:, pl.ds(j * LANE, LANE)], wo.at[j], sem_wo.at[j])
             for j in range(n_ct)]

    def raw_cp(k, slot):
        rows = pl.ds(pl.multiple_of(lax.div(k, 2) * 16, 16), 16)
        cps = [pltpu.make_async_copy(
            w.at[:, rows, pl.ds(pl.multiple_of((2 * c + lax.rem(k, 2)) * qf, LANE), qf)],
            ru.at[slot, 2 * j + c], sem_raw.at[slot, 2 * j + c])
            for j, w in enumerate((w1_hbm, w3_hbm)) for c in range(2)]
        rows = pl.ds(pl.multiple_of(jnp.minimum(k, n_dr - 1) * DR, DR), DR)
        return cps + [pltpu.make_async_copy(w2_hbm.at[:, rows, :], rd.at[slot],
                                            sem_raw.at[slot, 4])]

    def warmup(xp, wmod, stg, tmp, hp):
        hw, hr = HC // 2, n_seg * PRE // 2
        mod_cp = [pltpu.make_async_copy(wmod_hbm.at[:, pl.ds(a * D, n * D)],
                                        wmod.at[:, pl.ds(a * D, n * D)], sem_mod.at[i])
                  for i, (a, n) in enumerate(((0, 1), (1, 1), (2, 4)))]
        xp_cp = pltpu.make_async_copy(x_hbm.at[:, pl.ds(seg - PRE, PRE), :], xp, sem_x.at[0])

        def stg_cp(t, hc, slot):
            src = (wq_hbm, wk_hbm, wv_hbm)[t]
            return pltpu.make_async_copy(src.at[:, pl.ds(pl.multiple_of(hc * HC, HC), HC), :],
                                         stg.at[slot], sem_stg.at[slot])

        xp_cp.start()
        mod_cp[0].start()
        mod_cp[1].start()
        cv = c_ref[...].astype(F32)
        sc = jnp.broadcast_to(_rnd(cv * jax.nn.sigmoid(cv)), (8, D))
        xp_cp.wait()
        xn = _norm(xp[...].astype(F32).reshape(2 * hr, D))
        mod_cp[0].wait()
        stg_cp(0, 0, 0).start()
        mod[0] = _mm(sc, wmod[:, 0:D])
        mod_cp[1].wait()
        for i in range(1, NSTG):
            stg_cp(i // n_hc, i % n_hc, i).start()
        mod[1] = _mm(sc, wmod[:, D:2 * D])
        h = xn * (1.0 + mrow(1)) + mrow(0)
        for i, o in enumerate(_ops7(_LHS, (h[:hr, :hd], h[:hr, hd:], h[hr:, :hd], h[hr:, hd:]))):
            hp[i] = _pack(o)

        def warm(i, carry):
            slot = lax.rem(i, NSTG)
            stg_cp(0, 0, slot).wait()
            for r in range(D // RP):
                v = stg[slot, pl.ds(r * RP, RP)].reshape(RP * HC, LANE)
                tmp[pl.ds(r * RP * hw, RP * hw), :] = pltpu.bitcast(v, U32)
            ops = []
            for j in range(hw):
                quad = []
                for half in range(2):
                    a = tmp[pl.ds(half * hd * hw + j, hd, stride=hw), :]
                    for k, w in enumerate((a << 16, a & jnp.uint32(0xFFFF0000))):
                        quad.append(pltpu.bitcast(w, F32))
                        wqkv[i * HC + 2 * j + k, pl.ds(half * hd // 2, hd // 2), :] = (
                            _pack(quad[-1]))
                ops.append([o.astype(BF16) for o in _ops7(_RHS, quad)])
            prod = {n: _mm(_unpack(hp[n]), jnp.concatenate([o[n] for o in ops], axis=1))
                    for n in (1, 5, 0, 2, 3, 4, 6)}
            c4 = _out4(prod)
            for n, cq in enumerate(c4):
                for j in range(hw):
                    pre[i * HC + 2 * j + n % 2, pl.ds((n // 2) * hr // 2, hr // 2), :] = (
                        _pack(cq[:, j * LANE:(j + 1) * LANE]))
            nx = i + NSTG
            for t in range(3):
                @pl.when(lax.div(nx, n_hc) == t)
                def _(t=t):
                    stg_cp(t, lax.rem(nx, n_hc), slot).start()

            for at, cps in ((0, [x_cp]), (2, wo_cp[:n_ct // 2]), (4, wo_cp[n_ct // 2:]),
                            (6, [mod_cp[2]] + raw_cp(0, 0))):
                @pl.when(i == at)
                def _(cps=cps):
                    for cp in cps:
                        cp.start()

            return carry

        lax.fori_loop(0, 3 * n_hc, warm, 0)
        mod_cp[2].wait()

        def mod_rest(j, carry):
            mod[j] = _mm(sc, wmod[:, pl.ds(pl.multiple_of(j * D, D), D)])
            return carry

        lax.fori_loop(2, 6, mod_rest, 0)

    pl.run_scoped(warmup,
                  pltpu.VMEM((n_seg, PRE, D), BF16),
                  pltpu.VMEM((D, 6 * D), BF16),
                  pltpu.VMEM((NSTG, D, HC, LANE), BF16),
                  pltpu.VMEM((D * HC // 2, LANE), U32),
                  pltpu.VMEM((7, n_seg * PRE // 4, hd), U32))
    x_cp.wait()
    for cp in wo_cp:
        cp.wait()

    def pre_attn(s):
        xs = xb[s].astype(F32)[0:seg - PRE]
        return _norm(xs) * (1.0 + mrow(1)) + mrow(0)

    def step(k, u, side):
        s = k * UNR + u
        h = _unpack(hin[...])
        ri = lax.broadcasted_iota(jnp.int32, (L, L), 0)
        ci = lax.broadcasted_iota(jnp.int32, (L, L), 1)
        mask = (ri < M) | (ri >= ci)
        prow = pl.ds(pl.multiple_of(k * PRE, PRE), PRE)
        qkv, prob, att = {}, {}, {}

        def proj(g, ts):
            heads = [(t, g * HG + j) for t in ts for j in range(HG)]
            r = _mm(h, jnp.concatenate([_unpack(wqkv[t * H + n]) for t, n in heads], axis=1))
            for i, (t, n) in enumerate(heads):
                early = pre[t * H + n, prow, :]
                if (t, n) in side:
                    early = side[t, n](early)
                early = _unpack(early).astype(F32)[u * PRE:(u + 1) * PRE]
                qkv[t, n] = jnp.concatenate([r[:, i * LANE:(i + 1) * LANE], early], axis=0)

        def scores(g):
            for n in range(g * HG, (g + 1) * HG):
                sv = _mm_nt(_rnd(qkv[0, n]), qkv[1, n].astype(BF16)) * scale
                sv = jnp.where(mask, sv, -1e9)
                e = jnp.exp(sv - jnp.max(sv, axis=-1, keepdims=True))
                prob[n] = _rnd(e / jnp.sum(e, axis=-1, keepdims=True))

        def values(g):
            for n in range(g * HG, (g + 1) * HG):
                att[n] = _rnd(_mm(prob[n], qkv[2, n].astype(BF16)))

        nxt = pre_attn(jnp.minimum(s + 1, n_seg - 1))
        for g in range(n_grp):
            proj(g, (0, 1))
            if g >= 1:
                scores(g - 1)
        for g in range(n_grp):
            proj(g, (2,))
            if g == 0:
                scores(n_grp - 1)
            if g >= VLAG:
                values(g - VLAG)
        for g in range(n_grp - VLAG, n_grp):
            values(g)
        acc = _mm(jnp.concatenate([att[n] for n in range(H)], axis=1),
                  jnp.concatenate([wo[j] for j in range(n_ct)], axis=1))
        hin[...] = _pack(jnp.concatenate([acc[0:M], nxt], axis=0))
        ab[s] = acc[M:L].astype(BF16)

    def main(wu, wd):
        def steps(k, carry):
            slot = lax.rem(k, 2)
            for cp in raw_cp(k, slot):
                cp.wait()

            @pl.when(k + 1 < n_it)
            def _():
                for cp in raw_cp(k + 1, 1 - slot):
                    cp.start()

            kd = jnp.minimum(k, n_dr - 1)

            def up_piece(t, i, v):
                cols = pl.ds(t * LANE, LANE)
                ops = _ops49(_RHS, i, lambda r, c: ru[slot, c, r, :, cols].astype(F32))
                for j, o in enumerate(ops):
                    wu[lax.div(k, 2), slot, 7 * i + j, :, cols] = _pack(o)
                return _after(v, wu[lax.div(k, 2), jnp.minimum(slot, 1), 7 * i, :, cols], k)

            def down_piece(a, t, i, v):
                rows, cols = pl.ds(a * 8, 8), pl.ds(t * LANE, LANE)
                ops = _ops49(_RHS, i, lambda r, c: rd[
                    slot, r, pl.ds(a * 16, 16), pl.ds(c * qd + t * LANE, LANE)].astype(F32))
                for j, o in enumerate(ops):
                    wd[kd, 7 * i + j, rows, cols] = _pack(o)
                return _after(v, wd[jnp.minimum(kd, n_it), 7 * i, rows, cols], k)

            pieces = [functools.partial(up_piece, t, i)
                      for t in range(qf // LANE) for i in range(7)]
            pieces += [functools.partial(down_piece, a, t, i) for a in range(DR // 16)
                       for t in range(qd // LANE) for i in range(7)]
            spots = [(u, t, n) for u in range(UNR) for t, m in SPOT for n in range(H) if n % 4 < m]
            assert len(pieces) <= len(spots)
            for u in range(UNR):
                step(k, u, {sp[1:]: f for sp, f in zip(spots, pieces) if sp[0] == u})
            return carry

        hin[...] = _pack(jnp.concatenate([mem0_ref[...].astype(F32), pre_attn(0)], axis=0))
        lax.fori_loop(0, n_it, steps, 0)

        def resid(sg, rows):
            return xb[sg, rows, :].astype(F32) + mrow(2) * ab[sg, rows, :].astype(F32)

        def norm_piece(b, r, a):
            rows = pl.ds(a * 16, 16)
            h2f[r, rows, :] = _norm(resid(b * 4 + r, rows)) * (1.0 + mrow(4)) + mrow(3)
            return h2f[jnp.minimum(b, 0) + r, pl.ds(a * 16, 8), 0:qd]

        def lhs_piece(b, a, i):
            ops = _ops49(_LHS, i, lambda r, c: h2f[r, pl.ds(a * 16, 16), pl.ds(c * qd, qd)])
            for j, o in enumerate(ops):
                h2b[7 * i + j, pl.ds(a * 8, 8), :] = _pack(o)
            return h2b[jnp.minimum(b, 0) + 7 * i, pl.ds(a * 8, 8), :]

        ffn_in = [functools.partial(norm_piece, r=r, a=a)
                  for r in range(4) for a in range(seg // 16)]
        ffn_in += [functools.partial(lhs_piece, a=a, i=i)
                   for a in range(seg // 16) for i in range(7)]

        def out_cp(b):
            return pltpu.make_async_copy(ob.at[b % 2], out_hbm.at[pl.ds(b * FM, FM), :],
                                         sem_out.at[b % 2])

        def ffn(b, carry):
            @pl.when(b >= 2)
            def _():
                out_cp(b - 2).wait()

            slot = lax.rem(b, 2)
            lhs = []
            for f in range(qf // LANE):
                cols = pl.ds(f * LANE, LANE)
                gu = _out16([_mm(_unpack(h2b[n]), jnp.concatenate(
                    [_unpack(wu[:, c, n, :, cols].reshape(qd // 2, LANE)) for c in range(2)],
                    axis=1)) for n in range(49)])
                act = {}
                for r in range(4):
                    for c in range(2):
                        g = gu[r, c]
                        v = g * jax.nn.sigmoid(g) * gu[r, 2 + c]
                        act[r, 2 * c], act[r, 2 * c + 1] = v[:, :LANE], v[:, LANE:]
                lhs.append([o.astype(BF16) for i in range(7)
                            for o in _ops49(_LHS, i, lambda r, c: act[r, c])])
            prod = []
            for n in range(49):
                w = wd[:, n].reshape(qf // 2, qd)
                if n % 2 == 1 and n // 2 < len(ffn_in):
                    token = ffn_in[n // 2](jnp.minimum(b + 1, n_blk - 1))
                    w = jnp.concatenate([_after(w[:8], token, b), w[8:]], axis=0)
                prod.append(_mm(jnp.concatenate([l[n] for l in lhs], axis=1), _unpack(w)))
            y = _out16(prod)
            for r in range(4):
                yr = jnp.concatenate([y[r, c] for c in range(4)], axis=1)
                ob[slot, pl.ds(r * seg, seg), :] = (
                    resid(b * 4 + r, slice(None)) + mrow(5) * yr).astype(ob.dtype)
            out_cp(b).start()
            return carry

        for piece in ffn_in:
            piece(0)
        lax.fori_loop(0, n_blk, ffn, 0)
        for b in range(n_blk - 2, n_blk):
            out_cp(b).wait()

    pl.run_scoped(main, pltpu.VMEM((n_it // 2, 2, 49, 8, qf), U32),
                  pltpu.VMEM((n_dr, 49, DR // 2, qd), U32))


@functools.partial(jax.jit, static_argnames=("A_seg_len",))
def pallas_adaLN_cond__memory_aug_recurrent_mem_tr__glu_gated_swiglu__prompt_kernel(
    A_x, A_mem0, A_Wq, A_Wk, A_Wv, A_Wo, A_seg_len, B_x, B_w1, B_w3, B_w2, c, w_mod,
):
    del B_x
    B, S, D = A_x.shape
    H, Dh = A_Wq.shape[1], A_Wq.shape[2]
    M = A_mem0.shape[1]
    F = B_w1.shape[1]
    seg = int(A_seg_len)
    n_seg = S // seg
    assert B == 1 and Dh == LANE and S % seg == 0 and S % FM == 0 and F % FC == 0
    hbm = pl.BlockSpec(memory_space=pl.ANY)
    vmem = pl.BlockSpec(memory_space=pltpu.VMEM)
    dma = pltpu.SemaphoreType.DMA
    out = pl.pallas_call(
        _kernel,
        out_shape=jax.ShapeDtypeStruct((S, D), A_x.dtype),
        in_specs=[vmem, vmem] + [hbm] * 9,
        out_specs=hbm,
        scratch_shapes=[
            pltpu.VMEM((n_seg, seg, D), BF16),
            pltpu.VMEM((n_seg, seg, D), BF16),
            pltpu.VMEM((3 * H, D // 2, LANE), U32),
            pltpu.VMEM((3 * H, n_seg * PRE // 2, LANE), U32),
            pltpu.VMEM((D // LANE, H * Dh, LANE), BF16),
            pltpu.VMEM((6, 8, D), F32),
            pltpu.VMEM(((M + seg - PRE) // 2, D), U32),
            pltpu.VMEM((2, 4, 4, 16, F // 4), BF16),
            pltpu.VMEM((2, 4, DR, D), BF16),
            pltpu.VMEM((4, seg, D), F32),
            pltpu.VMEM((49, seg // 2, D // 4), U32),
            pltpu.VMEM((2, FM, D), A_x.dtype),
            dma((2,)), dma((3,)), dma((NSTG,)), dma((D // LANE,)), dma((2, 5)), dma((2,)),
        ],
        compiler_params=pltpu.CompilerParams(vmem_limit_bytes=127 * 2**20),
    )(c, A_mem0.reshape(M, D), A_x.reshape(n_seg, seg, D), A_Wq, A_Wk, A_Wv,
      A_Wo.reshape(H * Dh, D), B_w1.reshape(4, D // 4, F), B_w3.reshape(4, D // 4, F),
      B_w2.reshape(4, F // 4, D), w_mod)
    return out.reshape(B, S, D)
```

```python
import functools

import jax
import jax.numpy as jnp
from jax import lax
import jax.experimental.pallas as pl
import jax.experimental.pallas.tpu as pltpu

F32 = jnp.float32
BF16 = jnp.bfloat16
U32 = jnp.uint32
LANE = 128
HG = 4
HC = 8
RP = 64
VLAG = 3
SPOT = ((1, 3), (2, 2))
DR = 32
UNR = 2
NSPLIT = 6
NSTG = 4
PRE = 8
FM = 128
FC = 256


def _mm(a, b):
    return lax.dot_general(a, b, (((1,), (0,)), ((), ())), preferred_element_type=F32)


def _mm_nt(a, b):
    return lax.dot_general(a, b, (((1,), (1,)), ((), ())), preferred_element_type=F32)


def _rnd(v):
    return v.astype(BF16).astype(F32)


def _pack(v):
    return pltpu.bitcast(v.astype(BF16), U32)


def _pack_all(vs):
    n = vs[0].shape[1]
    w = _pack(jnp.concatenate(vs, axis=1))
    return [w[:, i * n:(i + 1) * n] for i in range(len(vs))]


def _unpack(v):
    return pltpu.bitcast(v, BF16)


_LHS = (((1, 0), (1, 3)), ((1, 2), (1, 3)), ((1, 0),), ((1, 3),), ((1, 0), (1, 1)),
        ((1, 2), (-1, 0)), ((1, 1), (-1, 3)))
_RHS = (((1, 0), (1, 3)), ((1, 0),), ((1, 1), (-1, 3)), ((1, 2), (-1, 0)), ((1, 3),),
        ((1, 0), (1, 1)), ((1, 2), (1, 3)))


def _comb(terms, quad):
    v = quad(terms[0][1])
    for sign, q in terms[1:]:
        v = v + quad(q) if sign > 0 else v - quad(q)
    return v


def _ops7(table, quads):
    return [_comb(t, quads.__getitem__) for t in table]


def _ops49(table, i, block):
    return _ops7(table, [
        _comb(table[i], lambda q: block(2 * (q // 2) + r, 2 * (q % 2) + c))
        for r in range(2) for c in range(2)])


def _out4(m):
    return (m[0] + m[3] - m[4] + m[6], m[2] + m[4], m[1] + m[3], m[0] - m[1] + m[2] + m[5])


def _out16(m):
    inner = [_out4(m[7 * i:7 * i + 7]) for i in range(7)]
    return {(2 * (q // 2) + p // 2, 2 * (q % 2) + p % 2): v
            for p in range(4) for q, v in enumerate(_out4([c[p] for c in inner]))}


def _after(v, token, i):
    return jnp.where(i < 0, pltpu.bitcast(token, v.dtype), v)


def _silu(g):
    hg = 0.5 * g
    return hg * jnp.tanh(hg) + hg


def _norm(x):
    m = jnp.mean(x, axis=-1, keepdims=True)
    xc = x - m
    v = jnp.mean(xc * xc, axis=-1, keepdims=True)
    return xc * lax.rsqrt(v + 1e-5)


def _kernel(c_ref, mem0_ref, x_hbm, wq_hbm, wk_hbm, wv_hbm, wo_hbm, w1_hbm, w3_hbm, w2_hbm,
            wmod_hbm, out_hbm,
            xb, ab, wqkv, pre, wo, mod, hin, ru, rd, h2f, h2b, ob,
            sem_x, sem_mod, sem_stg, sem_wo, sem_raw, sem_out):
    n_seg, seg, D = xb.shape
    M = mem0_ref.shape[0]
    L = M + seg
    H = wq_hbm.shape[1]
    F = w1_hbm.shape[2]
    n_grp, n_ct, n_hc = H // HG, D // LANE, H // HC
    n_it = n_seg // UNR
    n_blk, spb = n_seg * seg // FM, FM // seg
    hd, qd, qf = D // 2, D // 4, F // 4
    n_dr = qf // DR
    scale = float(LANE) ** -0.5

    def mrow(j):
        return mod[j, 0:1, :]

    x_cp = pltpu.make_async_copy(x_hbm, xb, sem_x.at[1])
    wo_cp = [pltpu.make_async_copy(wo_hbm.at[:, pl.ds(j * LANE, LANE)], wo.at[j], sem_wo.at[j])
             for j in range(n_ct)]

    def raw_cp(k, slot):
        rows = pl.ds(pl.multiple_of(lax.div(k, 2) * 16, 16), 16)
        cps = [pltpu.make_async_copy(
            w.at[:, rows, pl.ds(pl.multiple_of((2 * c + lax.rem(k, 2)) * qf, LANE), qf)],
            ru.at[slot, 2 * j + c], sem_raw.at[slot, 2 * j + c])
            for j, w in enumerate((w1_hbm, w3_hbm)) for c in range(2)]
        rows = pl.ds(pl.multiple_of(jnp.minimum(k, n_dr - 1) * DR, DR), DR)
        return cps + [pltpu.make_async_copy(w2_hbm.at[:, rows, :], rd.at[slot],
                                            sem_raw.at[slot, 4])]

    def warmup(xp, wmod, stg, tmp, hp):
        hw, hr = HC // 2, n_seg * PRE // 2
        mod_cp = [pltpu.make_async_copy(wmod_hbm.at[:, pl.ds(a * D, n * D)],
                                        wmod.at[:, pl.ds(a * D, n * D)], sem_mod.at[i])
                  for i, (a, n) in enumerate(((0, 1), (1, 1), (2, 4)))]
        xp_cp = pltpu.make_async_copy(x_hbm.at[:, pl.ds(seg - PRE, PRE), :], xp, sem_x.at[0])

        def stg_cp(t, hc, slot):
            src = (wq_hbm, wk_hbm, wv_hbm)[t]
            return pltpu.make_async_copy(src.at[:, pl.ds(pl.multiple_of(hc * HC, HC), HC), :],
                                         stg.at[slot], sem_stg.at[slot])

        xp_cp.start()
        mod_cp[0].start()
        mod_cp[1].start()
        cv = c_ref[...].astype(F32)
        sc = jnp.broadcast_to(_rnd(cv * jax.nn.sigmoid(cv)), (8, D))
        xp_cp.wait()
        xn = _norm(xp[...].astype(F32).reshape(2 * hr, D))
        mod_cp[0].wait()
        stg_cp(0, 0, 0).start()
        mod[0] = _mm(sc, wmod[:, 0:D])
        mod_cp[1].wait()
        for i in range(1, NSTG):
            stg_cp(i // n_hc, i % n_hc, i).start()
        mod[1] = _mm(sc, wmod[:, D:2 * D])
        h = xn * (1.0 + mrow(1)) + mrow(0)
        for i, o in enumerate(_ops7(_LHS, (h[:hr, :hd], h[:hr, hd:], h[hr:, :hd], h[hr:, hd:]))):
            hp[i] = _pack(o)

        def warm(i, carry):
            slot = lax.rem(i, NSTG)
            stg_cp(0, 0, slot).wait()
            for r in range(D // RP):
                v = stg[slot, pl.ds(r * RP, RP)].reshape(RP * HC, LANE)
                tmp[pl.ds(r * RP * hw, RP * hw), :] = pltpu.bitcast(v, U32)
            ops = []
            for j in range(hw):
                quad = []
                for half in range(2):
                    a = tmp[pl.ds(half * hd * hw + j, hd, stride=hw), :]
                    pair = [pltpu.bitcast(w, F32) for w in (a << 16, a & jnp.uint32(0xFFFF0000))]
                    for k, w in enumerate(_pack_all(pair)):
                        wqkv[i * HC + 2 * j + k, pl.ds(half * hd // 2, hd // 2), :] = w
                    quad += pair
                ops.append(_ops7(_RHS, quad))
            prod = {n: _mm(_unpack(hp[n]),
                           jnp.concatenate([o[n] for o in ops], axis=1).astype(BF16))
                    for n in (1, 5, 0, 2, 3, 4, 6)}
            for n, cq in enumerate(_out4(prod)):
                cq = _pack(cq)
                for j in range(hw):
                    pre[i * HC + 2 * j + n % 2, pl.ds((n // 2) * hr // 2, hr // 2), :] = (
                        cq[:, j * LANE:(j + 1) * LANE])
            nx = i + NSTG
            for t in range(3):
                @pl.when(lax.div(nx, n_hc) == t)
                def _(t=t):
                    stg_cp(t, lax.rem(nx, n_hc), slot).start()

            for at, cps in ((0, [x_cp]), (2, wo_cp[:n_ct // 2]), (4, wo_cp[n_ct // 2:]),
                            (6, [mod_cp[2]] + raw_cp(0, 0))):
                @pl.when(i == at)
                def _(cps=cps):
                    for cp in cps:
                        cp.start()

            return carry

        lax.fori_loop(0, 3 * n_hc, warm, 0)
        mod_cp[2].wait()

        def mod_rest(j, carry):
            mod[j] = _mm(sc, wmod[:, pl.ds(pl.multiple_of(j * D, D), D)])
            return carry

        lax.fori_loop(2, 6, mod_rest, 0)

    pl.run_scoped(warmup,
                  pltpu.VMEM((n_seg, PRE, D), BF16),
                  pltpu.VMEM((D, 6 * D), BF16),
                  pltpu.VMEM((NSTG, D, HC, LANE), BF16),
                  pltpu.VMEM((D * HC // 2, LANE), U32),
                  pltpu.VMEM((7, n_seg * PRE // 4, hd), U32))
    x_cp.wait()
    for cp in wo_cp:
        cp.wait()

    def pre_attn(s):
        xs = xb[s].astype(F32)[0:seg - PRE]
        return _norm(xs) * (1.0 + mrow(1)) + mrow(0)

    def step(k, u, side):
        s = k * UNR + u
        h = _unpack(hin[...])
        ri = lax.broadcasted_iota(jnp.int32, (L, L), 0)
        ci = lax.broadcasted_iota(jnp.int32, (L, L), 1)
        mask = (ri < M) | (ri >= ci)
        prow = pl.ds(pl.multiple_of(k * PRE, PRE), PRE)
        qkv, prob, att = {}, {}, {}

        def proj(g, ts):
            heads = [(t, g * HG + j) for t in ts for j in range(HG)]
            r = _mm(h, jnp.concatenate([_unpack(wqkv[t * H + n]) for t, n in heads], axis=1))
            for i, (t, n) in enumerate(heads):
                early = pre[t * H + n, prow, :]
                if (t, n) in side:
                    early = side[t, n](early)
                early = _unpack(early).astype(F32)[u * PRE:(u + 1) * PRE]
                qkv[t, n] = jnp.concatenate([r[:, i * LANE:(i + 1) * LANE], early], axis=0)

        def scores(g):
            for n in range(g * HG, (g + 1) * HG):
                sv = _mm_nt(_rnd(qkv[0, n]), qkv[1, n].astype(BF16)) * scale
                sv = jnp.where(mask, sv, -1e9)
                e = jnp.exp(sv - jnp.max(sv, axis=-1, keepdims=True))
                prob[n] = _rnd(e / jnp.sum(e, axis=-1, keepdims=True))

        def values(g):
            for n in range(g * HG, (g + 1) * HG):
                att[n] = _rnd(_mm(prob[n], qkv[2, n].astype(BF16)))

        nxt = pre_attn(jnp.minimum(s + 1, n_seg - 1))
        for g in range(n_grp):
            proj(g, (0, 1))
            if g >= 1:
                scores(g - 1)
        for g in range(n_grp):
            proj(g, (2,))
            if g == 0:
                scores(n_grp - 1)
            if g >= VLAG:
                values(g - VLAG)
        for g in range(n_grp - VLAG, n_grp):
            values(g)
        acc = _mm(jnp.concatenate([att[n] for n in range(H)], axis=1),
                  jnp.concatenate([wo[j] for j in range(n_ct)], axis=1))
        hin[...] = _pack(jnp.concatenate([acc[0:M], nxt], axis=0))
        ab[s] = acc[M:L].astype(BF16)

    def main(wu, wd):
        def steps(k, carry):
            slot = lax.rem(k, 2)
            for cp in raw_cp(k, slot):
                cp.wait()

            @pl.when(k + 1 < n_it)
            def _():
                for cp in raw_cp(k + 1, 1 - slot):
                    cp.start()

            kd = jnp.minimum(k, n_dr - 1)

            def up_piece(t, i, v):
                cols = pl.ds(t * LANE, LANE)
                ops = _ops49(_RHS, i, lambda r, c: ru[slot, c, r, :, cols].astype(F32))
                for j, o in enumerate(_pack_all(ops)):
                    wu[lax.div(k, 2), slot, 7 * i + j, :, cols] = o
                return _after(v, wu[lax.div(k, 2), jnp.minimum(slot, 1), 7 * i, :, cols], k)

            def down_piece(a, t, i, v):
                rows, cols = pl.ds(a * 8, 8), pl.ds(t * LANE, LANE)
                ops = _ops49(_RHS, i, lambda r, c: rd[
                    slot, r, pl.ds(a * 16, 16), pl.ds(c * qd + t * LANE, LANE)].astype(F32))
                for j, o in enumerate(_pack_all(ops)):
                    wd[kd, 7 * i + j, rows, cols] = o
                return _after(v, wd[jnp.minimum(kd, n_it), 7 * i, rows, cols], k)

            pieces = [functools.partial(up_piece, t, i)
                      for t in range(qf // LANE) for i in range(7)]
            pieces += [functools.partial(down_piece, a, t, i) for a in range(DR // 16)
                       for t in range(qd // LANE) for i in range(7)]
            spots = [(u, t, n) for u in range(UNR) for t, m in SPOT for n in range(H) if n % 4 < m]
            assert len(pieces) <= len(spots)
            for u in range(UNR):
                step(k, u, {sp[1:]: f for sp, f in zip(spots, pieces) if sp[0] == u})
            return carry

        hin[...] = _pack(jnp.concatenate([mem0_ref[...].astype(F32), pre_attn(0)], axis=0))
        lax.fori_loop(0, n_it, steps, 0)

        def resid(sg, rows):
            return xb[sg, rows, :].astype(F32) + mrow(2) * ab[sg, rows, :].astype(F32)

        def norm_piece(b, r, a):
            rows = pl.ds(a * 16, 16)
            h2f[r, rows, :] = _norm(resid(b * 4 + r, rows)) * (1.0 + mrow(4)) + mrow(3)
            return h2f[jnp.minimum(b, 0) + r, pl.ds(a * 16, 8), 0:qd]

        def lhs_piece(b, a, i):
            ops = _ops49(_LHS, i, lambda r, c: h2f[r, pl.ds(a * 16, 16), pl.ds(c * qd, qd)])
            for j, o in enumerate(ops):
                h2b[7 * i + j, pl.ds(a * 8, 8), :] = _pack(o)
            return h2b[jnp.minimum(b, 0) + 7 * i, pl.ds(a * 8, 8), :]

        ffn_in = [functools.partial(norm_piece, r=r, a=a)
                  for r in range(4) for a in range(seg // 16)]
        ffn_in += [functools.partial(lhs_piece, a=a, i=i)
                   for a in range(seg // 16) for i in range(7)]

        def out_cp(b):
            return pltpu.make_async_copy(ob.at[b % 2], out_hbm.at[pl.ds(b * FM, FM), :],
                                         sem_out.at[b % 2])

        def ffn(b, carry):
            @pl.when(b >= 2)
            def _():
                out_cp(b - 2).wait()

            slot = lax.rem(b, 2)
            lhs = []
            for f in range(qf // LANE):
                cols = pl.ds(f * LANE, LANE)
                gu = _out16([_mm(_unpack(h2b[n]), jnp.concatenate(
                    [_unpack(wu[:, c, n, :, cols].reshape(qd // 2, LANE)) for c in range(2)],
                    axis=1)) for n in range(49)])
                act = {}
                for r in range(4):
                    for c in range(2):
                        v = _silu(gu[r, c]) * gu[r, 2 + c]
                        act[r, 2 * c], act[r, 2 * c + 1] = v[:, :LANE], v[:, LANE:]
                lhs.append([o for i in range(7)
                            for o in _ops49(_LHS, i, lambda r, c: act[r, c])])
            prod, late = [], []
            for n in range(49):
                w = wd[:, n].reshape(qf // 2, qd)
                if n % 2 == 1 and n // 2 < len(ffn_in):
                    token = ffn_in[n // 2](jnp.minimum(b + 1, n_blk - 1))
                    w = jnp.concatenate([_after(w[:8], token, b), w[8:]], axis=0)
                a = [l[n] for l in lhs]
                if n < NSPLIT:
                    ks = (qf - LANE) // 2
                    late.append((a.pop().astype(BF16), _unpack(w[ks:])))
                    w = w[:ks]
                prod.append(_mm(jnp.concatenate(a, axis=1).astype(BF16), _unpack(w)))
                if n == NSPLIT - 1:
                    prod = [_mm(*t) + v for t, v in zip(late, prod)]
            y = _out16(prod)
            for r in range(4):
                yr = jnp.concatenate([y[r, c] for c in range(4)], axis=1)
                ob[slot, pl.ds(r * seg, seg), :] = (
                    resid(b * 4 + r, slice(None)) + mrow(5) * yr).astype(ob.dtype)
            out_cp(b).start()
            return carry

        for piece in ffn_in:
            piece(0)
        lax.fori_loop(0, n_blk, ffn, 0)
        for b in range(n_blk - 2, n_blk):
            out_cp(b).wait()

    pl.run_scoped(main, pltpu.VMEM((n_it // 2, 2, 49, 8, qf), U32),
                  pltpu.VMEM((n_dr, 49, DR // 2, qd), U32))


@functools.partial(jax.jit, static_argnames=("A_seg_len",))
def pallas_adaLN_cond__memory_aug_recurrent_mem_tr__glu_gated_swiglu__prompt_kernel(
    A_x, A_mem0, A_Wq, A_Wk, A_Wv, A_Wo, A_seg_len, B_x, B_w1, B_w3, B_w2, c, w_mod,
):
    del B_x
    B, S, D = A_x.shape
    H, Dh = A_Wq.shape[1], A_Wq.shape[2]
    M = A_mem0.shape[1]
    F = B_w1.shape[1]
    seg = int(A_seg_len)
    n_seg = S // seg
    assert B == 1 and Dh == LANE and S % seg == 0 and S % FM == 0 and F % FC == 0
    hbm = pl.BlockSpec(memory_space=pl.ANY)
    vmem = pl.BlockSpec(memory_space=pltpu.VMEM)
    dma = pltpu.SemaphoreType.DMA
    out = pl.pallas_call(
        _kernel,
        out_shape=jax.ShapeDtypeStruct((S, D), A_x.dtype),
        in_specs=[vmem, vmem] + [hbm] * 9,
        out_specs=hbm,
        scratch_shapes=[
            pltpu.VMEM((n_seg, seg, D), BF16),
            pltpu.VMEM((n_seg, seg, D), BF16),
            pltpu.VMEM((3 * H, D // 2, LANE), U32),
            pltpu.VMEM((3 * H, n_seg * PRE // 2, LANE), U32),
            pltpu.VMEM((D // LANE, H * Dh, LANE), BF16),
            pltpu.VMEM((6, 8, D), F32),
            pltpu.VMEM(((M + seg - PRE) // 2, D), U32),
            pltpu.VMEM((2, 4, 4, 16, F // 4), BF16),
            pltpu.VMEM((2, 4, DR, D), BF16),
            pltpu.VMEM((4, seg, D), F32),
            pltpu.VMEM((49, seg // 2, D // 4), U32),
            pltpu.VMEM((2, FM, D), A_x.dtype),
            dma((2,)), dma((3,)), dma((NSTG,)), dma((D // LANE,)), dma((2, 5)), dma((2,)),
        ],
        compiler_params=pltpu.CompilerParams(vmem_limit_bytes=127 * 2**20),
    )(c, A_mem0.reshape(M, D), A_x.reshape(n_seg, seg, D), A_Wq, A_Wk, A_Wv,
      A_Wo.reshape(H * Dh, D), B_w1.reshape(4, D // 4, F), B_w3.reshape(4, D // 4, F),
      B_w2.reshape(4, F // 4, D), w_mod)
    return out.reshape(B, S, D)
```

```python
import functools

import jax
import jax.numpy as jnp
from jax import lax
import jax.experimental.pallas as pl
import jax.experimental.pallas.tpu as pltpu

F32 = jnp.float32
BF16 = jnp.bfloat16
U32 = jnp.uint32
LANE = 128
LOG2E = 1.4426950408889634
HG = 4
HC = 8
RP = 64
VLAG = 3
SPOT = ((1, 3), (2, 2))
DR = 32
UNR = 2
NSPLIT = 6
NSTG = 4
PRE = 8
FM = 128
FC = 256


def _mm(a, b):
    return lax.dot_general(a, b, (((1,), (0,)), ((), ())), preferred_element_type=F32)


def _mm_nt(a, b):
    return lax.dot_general(a, b, (((1,), (1,)), ((), ())), preferred_element_type=F32)


def _rnd(v):
    return v.astype(BF16).astype(F32)


def _pack(v):
    return pltpu.bitcast(v.astype(BF16), U32)


def _pack_all(vs):
    n = vs[0].shape[1]
    w = _pack(jnp.concatenate(vs, axis=1))
    return [w[:, i * n:(i + 1) * n] for i in range(len(vs))]


def _unpack(v):
    return pltpu.bitcast(v, BF16)


_LHS = (((1, 0), (1, 3)), ((1, 2), (1, 3)), ((1, 0),), ((1, 3),), ((1, 0), (1, 1)),
        ((1, 2), (-1, 0)), ((1, 1), (-1, 3)))
_RHS = (((1, 0), (1, 3)), ((1, 0),), ((1, 1), (-1, 3)), ((1, 2), (-1, 0)), ((1, 3),),
        ((1, 0), (1, 1)), ((1, 2), (1, 3)))


def _comb(terms, quad):
    v = quad(terms[0][1])
    for sign, q in terms[1:]:
        v = v + quad(q) if sign > 0 else v - quad(q)
    return v


def _ops7(table, quads):
    return [_comb(t, quads.__getitem__) for t in table]


def _ops49(table, i, block):
    return _ops7(table, [
        _comb(table[i], lambda q: block(2 * (q // 2) + r, 2 * (q % 2) + c))
        for r in range(2) for c in range(2)])


def _out4(m):
    return (m[0] + m[3] - m[4] + m[6], m[2] + m[4], m[1] + m[3], m[0] - m[1] + m[2] + m[5])


def _out16(m):
    inner = [_out4(m[7 * i:7 * i + 7]) for i in range(7)]
    return {(2 * (q // 2) + p // 2, 2 * (q % 2) + p % 2): v
            for p in range(4) for q, v in enumerate(_out4([c[p] for c in inner]))}


def _after(v, token, i):
    return jnp.where(i < 0, pltpu.bitcast(token, v.dtype), v)


def _silu(g):
    hg = 0.5 * g
    return hg * jnp.tanh(hg) + hg


def _norm(x):
    m = jnp.mean(x, axis=-1, keepdims=True)
    xc = x - m
    v = jnp.mean(xc * xc, axis=-1, keepdims=True)
    return xc * lax.rsqrt(v + 1e-5)


def _kernel(c_ref, mem0_ref, x_hbm, wq_hbm, wk_hbm, wv_hbm, wo_hbm, w1_hbm, w3_hbm, w2_hbm,
            wmod_hbm, out_hbm,
            xb, ab, wqkv, pre, wo, mod, hin, ru, rd, h2f, h2b, ob,
            sem_x, sem_mod, sem_stg, sem_wo, sem_raw, sem_out):
    n_seg, seg, D = xb.shape
    M = mem0_ref.shape[0]
    L = M + seg
    H = wq_hbm.shape[1]
    F = w1_hbm.shape[2]
    n_grp, n_ct, n_hc = H // HG, D // LANE, H // HC
    n_it = n_seg // UNR
    n_blk, spb = n_seg * seg // FM, FM // seg
    hd, qd, qf = D // 2, D // 4, F // 4
    n_dr = qf // DR
    scale = float(LANE) ** -0.5

    def mrow(j):
        return mod[j, 0:1, :]

    x_cp = pltpu.make_async_copy(x_hbm, xb, sem_x.at[1])
    wo_cp = [pltpu.make_async_copy(wo_hbm.at[:, pl.ds(j * LANE, LANE)], wo.bitcast(BF16).at[j],
                                   sem_wo.at[j])
             for j in range(n_ct)]

    def raw_cp(k, slot):
        rows = pl.ds(pl.multiple_of(lax.div(k, 2) * 16, 16), 16)
        cps = [pltpu.make_async_copy(
            w.at[:, rows, pl.ds(pl.multiple_of((2 * c + lax.rem(k, 2)) * qf, LANE), qf)],
            ru.at[slot, 2 * j + c], sem_raw.at[slot, 2 * j + c])
            for j, w in enumerate((w1_hbm, w3_hbm)) for c in range(2)]
        rows = pl.ds(pl.multiple_of(jnp.minimum(k, n_dr - 1) * DR, DR), DR)
        return cps + [pltpu.make_async_copy(w2_hbm.at[:, rows, :], rd.at[slot],
                                            sem_raw.at[slot, 4])]

    def warmup(xp, wmod, stg, tmp, hp):
        hw, hr = HC // 2, n_seg * PRE // 2
        mod_cp = [pltpu.make_async_copy(wmod_hbm.at[:, pl.ds(a * D, n * D)],
                                        wmod.at[:, pl.ds(a * D, n * D)], sem_mod.at[i])
                  for i, (a, n) in enumerate(((0, 1), (1, 1), (2, 4)))]
        xp_cp = pltpu.make_async_copy(x_hbm.at[:, pl.ds(seg - PRE, PRE), :], xp, sem_x.at[0])

        def stg_cp(t, hc, slot):
            src = (wq_hbm, wk_hbm, wv_hbm)[t]
            return pltpu.make_async_copy(src.at[:, pl.ds(pl.multiple_of(hc * HC, HC), HC), :],
                                         stg.at[slot], sem_stg.at[slot])

        xp_cp.start()
        mod_cp[0].start()
        mod_cp[1].start()
        cv = c_ref[...].astype(F32)
        sc = jnp.broadcast_to(_rnd(cv * jax.nn.sigmoid(cv)), (8, D))
        xp_cp.wait()
        xn = _norm(xp[...].astype(F32).reshape(2 * hr, D))
        mod_cp[0].wait()
        stg_cp(0, 0, 0).start()
        mod[0] = _mm(sc, wmod[:, 0:D])
        mod_cp[1].wait()
        for i in range(1, NSTG):
            stg_cp(i // n_hc, i % n_hc, i).start()
        mod[1] = _mm(sc, wmod[:, D:2 * D])
        h = xn * (1.0 + mrow(1)) + mrow(0)
        for i, o in enumerate(_ops7(_LHS, (h[:hr, :hd], h[:hr, hd:], h[hr:, :hd], h[hr:, hd:]))):
            hp[i] = _pack(o)

        def warm(i, carry):
            slot = lax.rem(i, NSTG)
            stg_cp(0, 0, slot).wait()
            for r in range(D // RP):
                v = stg[slot, pl.ds(r * RP, RP)].reshape(RP * HC, LANE)
                tmp[pl.ds(r * RP * hw, RP * hw), :] = pltpu.bitcast(v, U32)
            ops = []
            for j in range(hw):
                quad = []
                for half in range(2):
                    a = tmp[pl.ds(half * hd * hw + j, hd, stride=hw), :]
                    pair = [pltpu.bitcast(w, F32) for w in (a << 16, a & jnp.uint32(0xFFFF0000))]
                    for k, w in enumerate(_pack_all(pair)):
                        wqkv[i * HC + 2 * j + k, pl.ds(half * hd // 2, hd // 2), :] = w
                    quad += pair
                ops.append(_ops7(_RHS, quad))
            prod = {n: _mm(_unpack(hp[n]),
                           jnp.concatenate([o[n] for o in ops], axis=1).astype(BF16))
                    for n in (1, 5, 0, 2, 3, 4, 6)}
            for n, cq in enumerate(_out4(prod)):
                cq = _pack(cq)
                for j in range(hw):
                    pre[i * HC + 2 * j + n % 2, pl.ds((n // 2) * hr // 2, hr // 2), :] = (
                        cq[:, j * LANE:(j + 1) * LANE])
            nx = i + NSTG
            for t in range(3):
                @pl.when(lax.div(nx, n_hc) == t)
                def _(t=t):
                    stg_cp(t, lax.rem(nx, n_hc), slot).start()

            for at, cps in ((0, [x_cp]), (2, wo_cp[:n_ct // 2]), (4, wo_cp[n_ct // 2:]),
                            (6, [mod_cp[2]]), (9, raw_cp(0, 0) + raw_cp(1, 1))):
                @pl.when(i == at)
                def _(cps=cps):
                    for cp in cps:
                        cp.start()

            return carry

        lax.fori_loop(0, 3 * n_hc, warm, 0)
        mod_cp[2].wait()

        def mod_rest(j, carry):
            mod[j] = _mm(sc, wmod[:, pl.ds(pl.multiple_of(j * D, D), D)])
            return carry

        lax.fori_loop(2, 6, mod_rest, 0)

    pl.run_scoped(warmup,
                  pltpu.VMEM((n_seg, PRE, D), BF16),
                  pltpu.VMEM((D, 6 * D), BF16),
                  pltpu.VMEM((NSTG, D, HC, LANE), BF16),
                  pltpu.VMEM((D * HC // 2, LANE), U32),
                  pltpu.VMEM((7, n_seg * PRE // 4, hd), U32))
    x_cp.wait()
    for cp in wo_cp:
        cp.wait()

    def pre_attn(s):
        xs = xb[s].astype(F32)[0:seg - PRE]
        return _norm(xs) * (1.0 + mrow(1)) + mrow(0)

    def step(k, u, side):
        s = k * UNR + u
        h = _unpack(hin[...])
        ri = lax.broadcasted_iota(jnp.int32, (L, L), 0)
        ci = lax.broadcasted_iota(jnp.int32, (L, L), 1)
        mask = (ri < M) | (ri >= ci)
        prow = pl.ds(pl.multiple_of(k * PRE, PRE), PRE)
        qkv, prob, att = {}, {}, {}

        def proj(g, ts):
            heads = [(t, g * HG + j) for t in ts for j in range(HG)]
            r = _mm(h, jnp.concatenate([_unpack(wqkv[t * H + n]) for t, n in heads], axis=1))
            for i, (t, n) in enumerate(heads):
                early = pre[t * H + n, prow, :]
                if (t, n) in side:
                    early = side[t, n](early)
                early = _unpack(early).astype(F32)[u * PRE:(u + 1) * PRE]
                qkv[t, n] = jnp.concatenate([r[:, i * LANE:(i + 1) * LANE], early], axis=0)

        def scores(g):
            for n in range(g * HG, (g + 1) * HG):
                sv = _mm_nt(_rnd(qkv[0, n]), qkv[1, n].astype(BF16)) * (scale * LOG2E)
                sv = jnp.where(mask, sv, -1e9 * LOG2E)
                e = jnp.exp2(sv - jnp.max(sv, axis=-1, keepdims=True))
                den = jnp.sum(e, axis=-1, keepdims=True)
                inv = pl.reciprocal(den, approx=True)
                prob[n] = _rnd(e * (inv * (2.0 - den * inv)))

        def values(g):
            for n in range(g * HG, (g + 1) * HG):
                att[n] = _rnd(_mm(prob[n], qkv[2, n].astype(BF16)))

        nxt = pre_attn(jnp.minimum(s + 1, n_seg - 1))
        for g in range(n_grp):
            proj(g, (0, 1))
            if g >= 1:
                scores(g - 1)
        for g in range(n_grp):
            proj(g, (2,))
            if g == 0:
                scores(n_grp - 1)
            if g >= VLAG:
                values(g - VLAG)
        for g in range(n_grp - VLAG, n_grp):
            values(g)
        acc = _mm(jnp.concatenate([att[n] for n in range(H)], axis=1),
                  jnp.concatenate([_unpack(wo[j]) for j in range(n_ct)], axis=1))
        hin[...] = _pack(jnp.concatenate([acc[0:M], nxt], axis=0))
        ab[s] = acc[M:L].astype(BF16)

    def main(wu, wd):
        def steps(k, carry):
            slot = lax.rem(k, 2)
            for cp in raw_cp(k, slot):
                cp.wait()

            kd = jnp.minimum(k, n_dr - 1)

            def up_piece(t, i, v):
                cols = pl.ds(t * LANE, LANE)
                ops = _ops49(_RHS, i, lambda r, c: ru[slot, c, r, :, cols].astype(F32))
                for j, o in enumerate(_pack_all(ops)):
                    wu[lax.div(k, 2), slot, 7 * i + j, :, cols] = o
                return _after(v, wu[lax.div(k, 2), jnp.minimum(slot, 1), 7 * i, :, cols], k)

            def down_piece(a, t, i, v):
                rows, cols = pl.ds(a * 8, 8), pl.ds(t * LANE, LANE)
                ops = _ops49(_RHS, i, lambda r, c: rd[
                    slot, r, pl.ds(a * 16, 16), pl.ds(c * qd + t * LANE, LANE)].astype(F32))
                for j, o in enumerate(_pack_all(ops)):
                    wd[kd, 7 * i + j, rows, cols] = o
                return _after(v, wd[jnp.minimum(kd, n_it), 7 * i, rows, cols], k)

            pieces = [functools.partial(up_piece, t, i)
                      for t in range(qf // LANE) for i in range(7)]
            pieces += [functools.partial(down_piece, a, t, i) for a in range(DR // 16)
                       for t in range(qd // LANE) for i in range(7)]
            spots = [(u, t, n) for u in range(UNR) for t, m in SPOT for n in range(H) if n % 4 < m]
            assert len(pieces) <= len(spots)
            for u in range(UNR):
                step(k, u, {sp[1:]: f for sp, f in zip(spots, pieces) if sp[0] == u})

            @pl.when(k + 2 < n_it)
            def _():
                for cp in raw_cp(k + 2, slot):
                    cp.start()

            return carry

        hin[...] = _pack(jnp.concatenate([mem0_ref[...].astype(F32), pre_attn(0)], axis=0))
        lax.fori_loop(0, n_it, steps, 0)

        def resid(sg, rows):
            return xb[sg, rows, :].astype(F32) + mrow(2) * ab[sg, rows, :].astype(F32)

        def norm_piece(b, r, a):
            rows = pl.ds(a * 16, 16)
            h2f[r, rows, :] = _norm(resid(b * 4 + r, rows)) * (1.0 + mrow(4)) + mrow(3)
            return h2f[jnp.minimum(b, 0) + r, pl.ds(a * 16, 8), 0:qd]

        def lhs_piece(b, a, i):
            ops = _ops49(_LHS, i, lambda r, c: h2f[r, pl.ds(a * 16, 16), pl.ds(c * qd, qd)])
            for j, o in enumerate(ops):
                h2b[7 * i + j, pl.ds(a * 8, 8), :] = _pack(o)
            return h2b[jnp.minimum(b, 0) + 7 * i, pl.ds(a * 8, 8), :]

        ffn_in = [functools.partial(norm_piece, r=r, a=a)
                  for r in range(4) for a in range(seg // 16)]
        ffn_in += [functools.partial(lhs_piece, a=a, i=i)
                   for a in range(seg // 16) for i in range(7)]

        def out_cp(b):
            return pltpu.make_async_copy(ob.at[b % 2], out_hbm.at[pl.ds(b * FM, FM), :],
                                         sem_out.at[b % 2])

        def ffn(b, carry):
            @pl.when(b >= 2)
            def _():
                out_cp(b - 2).wait()

            slot = lax.rem(b, 2)
            lhs = []
            for f in range(qf // LANE):
                cols = pl.ds(f * LANE, LANE)
                gu = _out16([_mm(_unpack(h2b[n]), jnp.concatenate(
                    [_unpack(wu[:, c, n, :, cols].reshape(qd // 2, LANE)) for c in range(2)],
                    axis=1)) for n in range(49)])
                act = {}
                for r in range(4):
                    for c in range(2):
                        v = _silu(gu[r, c]) * gu[r, 2 + c]
                        act[r, 2 * c], act[r, 2 * c + 1] = v[:, :LANE], v[:, LANE:]
                lhs.append([o for i in range(7)
                            for o in _ops49(_LHS, i, lambda r, c: act[r, c])])
            prod, late = [], []
            for n in range(49):
                w = wd[:, n].reshape(qf // 2, qd)
                if n % 2 == 1 and n // 2 < len(ffn_in):
                    token = ffn_in[n // 2](jnp.minimum(b + 1, n_blk - 1))
                    w = jnp.concatenate([_after(w[:8], token, b), w[8:]], axis=0)
                a = [l[n] for l in lhs]
                if n < NSPLIT:
                    ks = (qf - LANE) // 2
                    late.append((a.pop().astype(BF16), _unpack(w[ks:])))
                    w = w[:ks]
                prod.append(_mm(jnp.concatenate(a, axis=1).astype(BF16), _unpack(w)))
                if n == NSPLIT - 1:
                    prod = [_mm(*t) + v for t, v in zip(late, prod)]
            y = _out16(prod)
            for r in range(4):
                yr = jnp.concatenate([y[r, c] for c in range(4)], axis=1)
                ob[slot, pl.ds(r * seg, seg), :] = (
                    resid(b * 4 + r, slice(None)) + mrow(5) * yr).astype(ob.dtype)
            out_cp(b).start()
            return carry

        for piece in ffn_in:
            piece(0)
        lax.fori_loop(0, n_blk, ffn, 0)
        for b in range(n_blk - 2, n_blk):
            out_cp(b).wait()

    pl.run_scoped(main, pltpu.VMEM((n_it // 2, 2, 49, 8, qf), U32),
                  pltpu.VMEM((n_dr, 49, DR // 2, qd), U32))


@functools.partial(jax.jit, static_argnames=("A_seg_len",))
def pallas_adaLN_cond__memory_aug_recurrent_mem_tr__glu_gated_swiglu__prompt_kernel(
    A_x, A_mem0, A_Wq, A_Wk, A_Wv, A_Wo, A_seg_len, B_x, B_w1, B_w3, B_w2, c, w_mod,
):
    del B_x
    B, S, D = A_x.shape
    H, Dh = A_Wq.shape[1], A_Wq.shape[2]
    M = A_mem0.shape[1]
    F = B_w1.shape[1]
    seg = int(A_seg_len)
    n_seg = S // seg
    assert B == 1 and Dh == LANE and S % seg == 0 and S % FM == 0 and F % FC == 0
    hbm = pl.BlockSpec(memory_space=pl.ANY)
    vmem = pl.BlockSpec(memory_space=pltpu.VMEM)
    dma = pltpu.SemaphoreType.DMA
    out = pl.pallas_call(
        _kernel,
        out_shape=jax.ShapeDtypeStruct((S, D), A_x.dtype),
        in_specs=[vmem, vmem] + [hbm] * 9,
        out_specs=hbm,
        scratch_shapes=[
            pltpu.VMEM((n_seg, seg, D), BF16),
            pltpu.VMEM((n_seg, seg, D), BF16),
            pltpu.VMEM((3 * H, D // 2, LANE), U32),
            pltpu.VMEM((3 * H, n_seg * PRE // 2, LANE), U32),
            pltpu.VMEM((D // LANE, H * Dh // 2, LANE), U32),
            pltpu.VMEM((6, 8, D), F32),
            pltpu.VMEM(((M + seg - PRE) // 2, D), U32),
            pltpu.VMEM((2, 4, 4, 16, F // 4), BF16),
            pltpu.VMEM((2, 4, DR, D), BF16),
            pltpu.VMEM((4, seg, D), F32),
            pltpu.VMEM((49, seg // 2, D // 4), U32),
            pltpu.VMEM((2, FM, D), A_x.dtype),
            dma((2,)), dma((3,)), dma((NSTG,)), dma((D // LANE,)), dma((2, 5)), dma((2,)),
        ],
        compiler_params=pltpu.CompilerParams(vmem_limit_bytes=127 * 2**20),
    )(c, A_mem0.reshape(M, D), A_x.reshape(n_seg, seg, D), A_Wq, A_Wk, A_Wv,
      A_Wo.reshape(H * Dh, D), B_w1.reshape(4, D // 4, F), B_w3.reshape(4, D // 4, F),
      B_w2.reshape(4, F // 4, D), w_mod)
    return out.reshape(B, S, D)
```

```python
import functools

import jax
import jax.numpy as jnp
from jax import lax
import jax.experimental.pallas as pl
import jax.experimental.pallas.tpu as pltpu

F32 = jnp.float32
BF16 = jnp.bfloat16
U32 = jnp.uint32
LANE = 128
LOG2E = 1.4426950408889634
HG = 4
HC = 8
RP = 64
VLAG = 4
SPOT = ((1, 1), (2, 1), (3, 3))
DR = 32
UNR = 2
NSPLIT = 6
NSTG = 4
PRE = 8
FM = 128
FC = 256


def _mm(a, b):
    return lax.dot_general(a, b, (((1,), (0,)), ((), ())), preferred_element_type=F32)


def _mm_nt(a, b):
    return lax.dot_general(a, b, (((1,), (1,)), ((), ())), preferred_element_type=F32)


def _rnd(v):
    return v.astype(BF16).astype(F32)


def _pack(v):
    return pltpu.bitcast(v.astype(BF16), U32)


def _pack_all(vs):
    n = vs[0].shape[1]
    w = _pack(jnp.concatenate(vs, axis=1))
    return [w[:, i * n:(i + 1) * n] for i in range(len(vs))]


def _unpack(v):
    return pltpu.bitcast(v, BF16)


_LHS = (((1, 0), (1, 3)), ((1, 2), (1, 3)), ((1, 0),), ((1, 3),), ((1, 0), (1, 1)),
        ((1, 2), (-1, 0)), ((1, 1), (-1, 3)))
_RHS = (((1, 0), (1, 3)), ((1, 0),), ((1, 1), (-1, 3)), ((1, 2), (-1, 0)), ((1, 3),),
        ((1, 0), (1, 1)), ((1, 2), (1, 3)))


def _comb(terms, quad):
    v = quad(terms[0][1])
    for sign, q in terms[1:]:
        v = v + quad(q) if sign > 0 else v - quad(q)
    return v


def _ops7(table, quads):
    return [_comb(t, quads.__getitem__) for t in table]


def _ops49(table, i, block):
    return _ops7(table, [
        _comb(table[i], lambda q: block(2 * (q // 2) + r, 2 * (q % 2) + c))
        for r in range(2) for c in range(2)])


def _out4(m):
    return (m[0] + m[3] - m[4] + m[6], m[2] + m[4], m[1] + m[3], m[0] - m[1] + m[2] + m[5])


def _out16(m):
    inner = [_out4(m[7 * i:7 * i + 7]) for i in range(7)]
    return {(2 * (q // 2) + p // 2, 2 * (q % 2) + p % 2): v
            for p in range(4) for q, v in enumerate(_out4([c[p] for c in inner]))}


def _after(v, token, i):
    return jnp.where(i < 0, pltpu.bitcast(token, v.dtype), v)


def _silu(g):
    hg = 0.5 * g
    return hg * jnp.tanh(hg) + hg


def _norm(x):
    m = jnp.mean(x, axis=-1, keepdims=True)
    xc = x - m
    v = jnp.mean(xc * xc, axis=-1, keepdims=True)
    return xc * lax.rsqrt(v + 1e-5)


def _kernel(c_ref, mem0_ref, x_hbm, wq_hbm, wk_hbm, wv_hbm, wo_hbm, w1_hbm, w3_hbm, w2_hbm,
            wmod_hbm, out_hbm,
            xb, ab, wqkv, pre, wo, mod, hin, ru, rd, h2f, h2b, ob,
            sem_x, sem_mod, sem_stg, sem_wo, sem_raw, sem_out):
    n_seg, seg, D = xb.shape
    M = mem0_ref.shape[0]
    L = M + seg
    H = wq_hbm.shape[1]
    F = w1_hbm.shape[2]
    n_grp, n_ct, n_hc = H // HG, D // LANE, H // HC
    n_it = n_seg // UNR
    n_blk, spb = n_seg * seg // FM, FM // seg
    hd, qd, qf = D // 2, D // 4, F // 4
    n_dr = qf // DR
    scale = float(LANE) ** -0.5

    def mrow(j):
        return mod[j, 0:1, :]

    x_cp = pltpu.make_async_copy(x_hbm, xb, sem_x.at[1])
    wo_cp = [pltpu.make_async_copy(wo_hbm.at[:, pl.ds(j * LANE, LANE)], wo.bitcast(BF16).at[j],
                                   sem_wo.at[j])
             for j in range(n_ct)]

    def raw_cp(k, slot):
        rows = pl.ds(pl.multiple_of(lax.div(k, 2) * 16, 16), 16)
        cps = [pltpu.make_async_copy(
            w.at[:, rows, pl.ds(pl.multiple_of((2 * c + lax.rem(k, 2)) * qf, LANE), qf)],
            ru.bitcast(BF16).at[slot, 2 * j + c], sem_raw.at[slot, 2 * j + c])
            for j, w in enumerate((w1_hbm, w3_hbm)) for c in range(2)]
        rows = pl.ds(pl.multiple_of(jnp.minimum(k, n_dr - 1) * DR, DR), DR)
        return cps + [pltpu.make_async_copy(w2_hbm.at[:, rows, :], rd.bitcast(BF16).at[slot],
                                            sem_raw.at[slot, 4])]

    def warmup(xp, wmod, stg, tmp, hp):
        hw, hr = HC // 2, n_seg * PRE // 2
        mod_cp = [pltpu.make_async_copy(wmod_hbm.at[:, pl.ds(a * D, n * D)],
                                        wmod.bitcast(BF16).at[:, pl.ds(a * D, n * D)],
                                        sem_mod.at[i])
                  for i, (a, n) in enumerate(((0, 1), (1, 1), (2, 4)))]
        xp_cp = pltpu.make_async_copy(x_hbm.at[:, pl.ds(seg - PRE, PRE), :], xp, sem_x.at[0])

        def stg_cp(t, hc, slot):
            src = (wq_hbm, wk_hbm, wv_hbm)[t]
            return pltpu.make_async_copy(src.at[:, pl.ds(pl.multiple_of(hc * HC, HC), HC), :],
                                         stg.at[slot], sem_stg.at[slot])

        xp_cp.start()
        mod_cp[0].start()
        mod_cp[1].start()
        cv = c_ref[...].astype(F32)
        sc = jnp.broadcast_to(_rnd(cv * jax.nn.sigmoid(cv)), (8, D))
        xp_cp.wait()
        xn = _norm(xp[...].astype(F32).reshape(2 * hr, D))
        mod_cp[0].wait()
        stg_cp(0, 0, 0).start()
        mod[0] = _mm(sc, _unpack(wmod[:, 0:D]))
        mod_cp[1].wait()
        for i in range(1, NSTG):
            stg_cp(i // n_hc, i % n_hc, i).start()
        mod[1] = _mm(sc, _unpack(wmod[:, D:2 * D]))
        h = xn * (1.0 + mrow(1)) + mrow(0)
        for i, o in enumerate(_ops7(_LHS, (h[:hr, :hd], h[:hr, hd:], h[hr:, :hd], h[hr:, hd:]))):
            hp[i] = _pack(o)

        def warm(i, carry):
            slot = lax.rem(i, NSTG)
            stg_cp(0, 0, slot).wait()
            for r in range(D // RP):
                v = stg[slot, pl.ds(r * RP, RP)].reshape(RP * HC, LANE)
                tmp[pl.ds(r * RP * hw, RP * hw), :] = pltpu.bitcast(v, U32)
            ops = []
            for j in range(hw):
                quad = []
                for half in range(2):
                    a = tmp[pl.ds(half * hd * hw + j, hd, stride=hw), :]
                    pair = [pltpu.bitcast(w, F32) for w in (a << 16, a & jnp.uint32(0xFFFF0000))]
                    for k, w in enumerate(_pack_all(pair)):
                        wqkv[i * HC + 2 * j + k, pl.ds(half * hd // 2, hd // 2), :] = w
                    quad += pair
                ops.append(_ops7(_RHS, quad))
            prod = {n: _mm(_unpack(hp[n]),
                           jnp.concatenate([o[n] for o in ops], axis=1).astype(BF16))
                    for n in (1, 5, 0, 2, 3, 4, 6)}
            for n, cq in enumerate(_out4(prod)):
                cq = _pack(cq)
                for j in range(hw):
                    pre[i * HC + 2 * j + n % 2, pl.ds((n // 2) * hr // 2, hr // 2), :] = (
                        cq[:, j * LANE:(j + 1) * LANE])
            nx = i + NSTG
            for t in range(3):
                @pl.when(lax.div(nx, n_hc) == t)
                def _(t=t):
                    stg_cp(t, lax.rem(nx, n_hc), slot).start()

            for at, cps in ((0, [x_cp]), (2, wo_cp[:n_ct // 2]), (4, wo_cp[n_ct // 2:]),
                            (6, [mod_cp[2]]), (9, raw_cp(0, 0) + raw_cp(1, 1))):
                @pl.when(i == at)
                def _(cps=cps):
                    for cp in cps:
                        cp.start()

            return carry

        lax.fori_loop(0, 3 * n_hc, warm, 0)
        mod_cp[2].wait()

        def mod_rest(j, carry):
            mod[j] = _mm(sc, _unpack(wmod[:, pl.ds(pl.multiple_of(j * D, D), D)]))
            return carry

        lax.fori_loop(2, 6, mod_rest, 0)

    pl.run_scoped(warmup,
                  pltpu.VMEM((n_seg, PRE, D), BF16),
                  pltpu.VMEM((hd, 6 * D), U32),
                  pltpu.VMEM((NSTG, D, HC, LANE), BF16),
                  pltpu.VMEM((D * HC // 2, LANE), U32),
                  pltpu.VMEM((7, n_seg * PRE // 4, hd), U32))
    x_cp.wait()
    for cp in wo_cp:
        cp.wait()

    def pre_attn(s):
        xs = xb[s].astype(F32)[0:seg - PRE]
        return _norm(xs) * (1.0 + mrow(1)) + mrow(0)

    def step(k, u, side):
        s = k * UNR + u
        h = _unpack(hin[...])
        ri = lax.broadcasted_iota(jnp.int32, (L, L), 0)
        ci = lax.broadcasted_iota(jnp.int32, (L, L), 1)
        mask = (ri < M) | (ri >= ci)
        prow = pl.ds(pl.multiple_of(k * PRE, PRE), PRE)
        qkv, prob, att = {}, {}, {}

        def proj(g, ts):
            heads = [(t, g * HG + j) for t in ts for j in range(HG)]
            r = _mm(h, jnp.concatenate([_unpack(wqkv[t * H + n]) for t, n in heads], axis=1))
            for i, (t, n) in enumerate(heads):
                early = pre[t * H + n, prow, :]
                if (t, n) in side:
                    early = side[t, n](early)
                early = _unpack(early).astype(F32)[u * PRE:(u + 1) * PRE]
                qkv[t, n] = jnp.concatenate([r[:, i * LANE:(i + 1) * LANE], early], axis=0)

        def scores(g):
            for n in range(g * HG, (g + 1) * HG):
                sv = _mm_nt(_rnd(qkv[0, n]), qkv[1, n].astype(BF16)) * (scale * LOG2E)
                sv = jnp.where(mask, sv, -1e9 * LOG2E)
                e = jnp.exp2(sv - jnp.max(sv, axis=-1, keepdims=True))
                den = jnp.sum(e, axis=-1, keepdims=True)
                inv = pl.reciprocal(den, approx=True)
                prob[n] = _rnd(e * (inv * (2.0 - den * inv)))

        def values(g):
            for n in range(g * HG, (g + 1) * HG):
                att[n] = _rnd(_mm(prob[n], qkv[2, n].astype(BF16)))

        nxt = pre_attn(jnp.minimum(s + 1, n_seg - 1))
        for g in range(n_grp):
            proj(g, (0, 1))
            if g >= 1:
                scores(g - 1)
        for g in range(n_grp):
            proj(g, (2,))
            if g == 0:
                scores(n_grp - 1)
            if g >= VLAG:
                values(g - VLAG)
        for g in range(n_grp - VLAG, n_grp):
            values(g)
        cols = []
        for j in range(n_ct):
            w, per = wo[j], H // n_ct
            rows = w.shape[0] // per
            parts = []
            for i in range(per):
                blk = w[i * rows:(i + 1) * rows]
                if (3, j * per + i) in side:
                    blk = jnp.concatenate([side[3, j * per + i](blk[:8]), blk[8:]], axis=0)
                parts.append(blk)
            cols.append(_unpack(jnp.concatenate(parts, axis=0)))
        acc = _mm(jnp.concatenate([att[n] for n in range(H)], axis=1),
                  jnp.concatenate(cols, axis=1))
        hin[...] = _pack(jnp.concatenate([acc[0:M], nxt], axis=0))
        ab[s] = acc[M:L].astype(BF16)

    def main(wu, wd):
        def steps(k, carry):
            slot = lax.rem(k, 2)
            for cp in raw_cp(k, slot):
                cp.wait()

            kd = jnp.minimum(k, n_dr - 1)

            def up_piece(t, i, v):
                cols = pl.ds(t * LANE, LANE)
                ops = _ops49(_RHS, i, lambda r, c: _unpack(ru[slot, c, r, :, cols]).astype(F32))
                for j, o in enumerate(_pack_all(ops)):
                    wu[lax.div(k, 2), slot, 7 * i + j, :, cols] = o
                return _after(v, wu[lax.div(k, 2), jnp.minimum(slot, 1), 7 * i, :, cols], k)

            def down_piece(a, t, i, v):
                rows, cols = pl.ds(a * 8, 8), pl.ds(t * LANE, LANE)
                ops = _ops49(_RHS, i, lambda r, c: _unpack(
                    rd[slot, r, rows, pl.ds(c * qd + t * LANE, LANE)]).astype(F32))
                for j, o in enumerate(_pack_all(ops)):
                    wd[kd, 7 * i + j, rows, cols] = o
                return _after(v, wd[jnp.minimum(kd, n_it), 7 * i, rows, cols], k)

            pieces = [functools.partial(up_piece, t, i)
                      for t in range(qf // LANE) for i in range(7)]
            pieces += [functools.partial(down_piece, a, t, i) for a in range(DR // 16)
                       for t in range(qd // LANE) for i in range(7)]
            spots = [(u, t, n) for u in range(UNR) for t, m in SPOT for n in range(H) if n % 4 < m]
            assert len(pieces) <= len(spots)
            for u in range(UNR):
                step(k, u, {sp[1:]: f for sp, f in zip(spots, pieces) if sp[0] == u})

            @pl.when(k + 2 < n_it)
            def _():
                for cp in raw_cp(k + 2, slot):
                    cp.start()

            return carry

        hin[...] = _pack(jnp.concatenate([mem0_ref[...].astype(F32), pre_attn(0)], axis=0))
        lax.fori_loop(0, n_it, steps, 0)

        def resid(sg, rows):
            return xb[sg, rows, :].astype(F32) + mrow(2) * ab[sg, rows, :].astype(F32)

        def norm_piece(b, r, a):
            rows = pl.ds(a * 16, 16)
            h2f[r, rows, :] = _norm(resid(b * 4 + r, rows)) * (1.0 + mrow(4)) + mrow(3)
            return h2f[jnp.minimum(b, 0) + r, pl.ds(a * 16, 8), 0:qd]

        def lhs_piece(b, a, i):
            ops = _ops49(_LHS, i, lambda r, c: h2f[r, pl.ds(a * 16, 16), pl.ds(c * qd, qd)])
            for j, o in enumerate(ops):
                h2b[7 * i + j, pl.ds(a * 8, 8), :] = _pack(o)
            return h2b[jnp.minimum(b, 0) + 7 * i, pl.ds(a * 8, 8), :]

        ffn_in = [functools.partial(norm_piece, r=r, a=a)
                  for r in range(4) for a in range(seg // 16)]
        ffn_in += [functools.partial(lhs_piece, a=a, i=i)
                   for a in range(seg // 16) for i in range(7)]

        def out_cp(b):
            return pltpu.make_async_copy(ob.at[b % 2], out_hbm.at[pl.ds(b * FM, FM), :],
                                         sem_out.at[b % 2])

        def ffn(b, carry):
            @pl.when(b >= 2)
            def _():
                out_cp(b - 2).wait()

            slot = lax.rem(b, 2)
            lhs = []
            for f in range(qf // LANE):
                cols = pl.ds(f * LANE, LANE)
                gu = _out16([_mm(_unpack(h2b[n]), jnp.concatenate(
                    [_unpack(wu[:, c, n, :, cols].reshape(qd // 2, LANE)) for c in range(2)],
                    axis=1)) for n in range(49)])
                act = {}
                for r in range(4):
                    for c in range(2):
                        v = _silu(gu[r, c]) * gu[r, 2 + c]
                        act[r, 2 * c], act[r, 2 * c + 1] = v[:, :LANE], v[:, LANE:]
                lhs.append([o for i in range(7)
                            for o in _ops49(_LHS, i, lambda r, c: act[r, c])])
            prod, late = [], []
            for n in range(49):
                w = wd[:, n].reshape(qf // 2, qd)
                if n % 2 == 1 and n // 2 < len(ffn_in):
                    token = ffn_in[n // 2](jnp.minimum(b + 1, n_blk - 1))
                    w = jnp.concatenate([_after(w[:8], token, b), w[8:]], axis=0)
                a = [l[n] for l in lhs]
                if n < NSPLIT:
                    ks = (qf - LANE) // 2
                    late.append((a.pop().astype(BF16), _unpack(w[ks:])))
                    w = w[:ks]
                prod.append(_mm(jnp.concatenate(a, axis=1).astype(BF16), _unpack(w)))
                if n == NSPLIT - 1:
                    prod = [_mm(*t) + v for t, v in zip(late, prod)]
            y = _out16(prod)
            for r in range(4):
                yr = jnp.concatenate([y[r, c] for c in range(4)], axis=1)
                ob[slot, pl.ds(r * seg, seg), :] = (
                    resid(b * 4 + r, slice(None)) + mrow(5) * yr).astype(ob.dtype)
            out_cp(b).start()
            return carry

        for piece in ffn_in:
            piece(0)
        lax.fori_loop(0, n_blk, ffn, 0)
        for b in range(n_blk - 2, n_blk):
            out_cp(b).wait()

    pl.run_scoped(main, pltpu.VMEM((n_it // 2, 2, 49, 8, qf), U32),
                  pltpu.VMEM((n_dr, 49, DR // 2, qd), U32))


@functools.partial(jax.jit, static_argnames=("A_seg_len",))
def pallas_adaLN_cond__memory_aug_recurrent_mem_tr__glu_gated_swiglu__prompt_kernel(
    A_x, A_mem0, A_Wq, A_Wk, A_Wv, A_Wo, A_seg_len, B_x, B_w1, B_w3, B_w2, c, w_mod,
):
    del B_x
    B, S, D = A_x.shape
    H, Dh = A_Wq.shape[1], A_Wq.shape[2]
    M = A_mem0.shape[1]
    F = B_w1.shape[1]
    seg = int(A_seg_len)
    n_seg = S // seg
    assert B == 1 and Dh == LANE and S % seg == 0 and S % FM == 0 and F % FC == 0
    hbm = pl.BlockSpec(memory_space=pl.ANY)
    vmem = pl.BlockSpec(memory_space=pltpu.VMEM)
    dma = pltpu.SemaphoreType.DMA
    out = pl.pallas_call(
        _kernel,
        out_shape=jax.ShapeDtypeStruct((S, D), A_x.dtype),
        in_specs=[vmem, vmem] + [hbm] * 9,
        out_specs=hbm,
        scratch_shapes=[
            pltpu.VMEM((n_seg, seg, D), BF16),
            pltpu.VMEM((n_seg, seg, D), BF16),
            pltpu.VMEM((3 * H, D // 2, LANE), U32),
            pltpu.VMEM((3 * H, n_seg * PRE // 2, LANE), U32),
            pltpu.VMEM((D // LANE, H * Dh // 2, LANE), U32),
            pltpu.VMEM((6, 8, D), F32),
            pltpu.VMEM(((M + seg - PRE) // 2, D), U32),
            pltpu.VMEM((2, 4, 4, 8, F // 4), U32),
            pltpu.VMEM((2, 4, DR // 2, D), U32),
            pltpu.VMEM((4, seg, D), F32),
            pltpu.VMEM((49, seg // 2, D // 4), U32),
            pltpu.VMEM((2, FM, D), A_x.dtype),
            dma((2,)), dma((3,)), dma((NSTG,)), dma((D // LANE,)), dma((2, 5)), dma((2,)),
        ],
        compiler_params=pltpu.CompilerParams(vmem_limit_bytes=127 * 2**20),
    )(c, A_mem0.reshape(M, D), A_x.reshape(n_seg, seg, D), A_Wq, A_Wk, A_Wv,
      A_Wo.reshape(H * Dh, D), B_w1.reshape(4, D // 4, F), B_w3.reshape(4, D // 4, F),
      B_w2.reshape(4, F // 4, D), w_mod)
    return out.reshape(B, S, D)
```

```python
import functools

import jax
import jax.numpy as jnp
from jax import lax
import jax.experimental.pallas as pl
import jax.experimental.pallas.tpu as pltpu

F32 = jnp.float32
BF16 = jnp.bfloat16
U32 = jnp.uint32
LANE = 128
LOG2E = 1.4426950408889634
HG = 4
HC = 8
RP = 64
VLAG = 4
SPOT = ((1, 1), (2, 1), (3, 3))
DR = 32
UNR = 2
NSPLIT = 6
NSTG = 4
PRE = 8
FM = 128
FC = 256


def _mm(a, b):
    return lax.dot_general(a, b, (((1,), (0,)), ((), ())), preferred_element_type=F32)


def _mm_nt(a, b):
    return lax.dot_general(a, b, (((1,), (1,)), ((), ())), preferred_element_type=F32)


def _rnd(v):
    return v.astype(BF16).astype(F32)


def _pack(v):
    return pltpu.bitcast(v.astype(BF16), U32)


def _pack_all(vs):
    n = vs[0].shape[1]
    w = _pack(jnp.concatenate(vs, axis=1))
    return [w[:, i * n:(i + 1) * n] for i in range(len(vs))]


def _unpack(v):
    return pltpu.bitcast(v, BF16)


_LHS = (((1, 0), (1, 3)), ((1, 2), (1, 3)), ((1, 0),), ((1, 3),), ((1, 0), (1, 1)),
        ((1, 2), (-1, 0)), ((1, 1), (-1, 3)))
_RHS = (((1, 0), (1, 3)), ((1, 0),), ((1, 1), (-1, 3)), ((1, 2), (-1, 0)), ((1, 3),),
        ((1, 0), (1, 1)), ((1, 2), (1, 3)))


def _comb(terms, quad):
    v = quad(terms[0][1])
    for sign, q in terms[1:]:
        v = v + quad(q) if sign > 0 else v - quad(q)
    return v


def _ops7(table, quads):
    return [_comb(t, quads.__getitem__) for t in table]


def _ops49(table, i, block):
    return _ops7(table, [
        _comb(table[i], lambda q: block(2 * (q // 2) + r, 2 * (q % 2) + c))
        for r in range(2) for c in range(2)])


def _out4(m):
    return (m[0] + m[3] - m[4] + m[6], m[2] + m[4], m[1] + m[3], m[0] - m[1] + m[2] + m[5])


def _out16(m):
    inner = [_out4(m[7 * i:7 * i + 7]) for i in range(7)]
    return {(2 * (q // 2) + p // 2, 2 * (q % 2) + p % 2): v
            for p in range(4) for q, v in enumerate(_out4([c[p] for c in inner]))}


def _after(v, token, i):
    return jnp.where(i < 0, pltpu.bitcast(token, v.dtype), v)


def _silu(g):
    hg = 0.5 * g
    return hg * jnp.tanh(hg) + hg


def _norm(x):
    m = jnp.mean(x, axis=-1, keepdims=True)
    xc = x - m
    v = jnp.mean(xc * xc, axis=-1, keepdims=True)
    return xc * lax.rsqrt(v + 1e-5)


def _kernel(c_ref, mem0_ref, x_hbm, wq_hbm, wk_hbm, wv_hbm, wo_hbm, w1_hbm, w3_hbm, w2_hbm,
            wmod_hbm, out_hbm,
            xb, ab, wqkv, pre, wo, mod, hin, ru, rd, h2f, h2b, ob,
            sem_x, sem_mod, sem_stg, sem_wo, sem_raw, sem_out):
    n_seg, seg, D = xb.shape
    M = mem0_ref.shape[0]
    L = M + seg
    H = wq_hbm.shape[1]
    F = w1_hbm.shape[2]
    n_grp, n_ct, n_hc = H // HG, D // LANE, H // HC
    n_it = n_seg // UNR
    n_blk, spb = n_seg * seg // FM, FM // seg
    hd, qd, qf = D // 2, D // 4, F // 4
    n_dr = qf // DR
    scale = float(LANE) ** -0.5

    def mrow(j):
        return mod[j, 0:1, :]

    x_cp = pltpu.make_async_copy(x_hbm, xb, sem_x.at[1])
    wo_cp = [pltpu.make_async_copy(wo_hbm.at[:, pl.ds(j * LANE, LANE)], wo.bitcast(BF16).at[j],
                                   sem_wo.at[j])
             for j in range(n_ct)]

    def raw_cp(kp, slot):
        rows = pl.ds(pl.multiple_of(kp * 16, 16), 16)
        cps = [pltpu.make_async_copy(w.at[:, rows, :], ru.bitcast(BF16).at[slot, j],
                                     sem_raw.at[slot, j])
               for j, w in enumerate((w1_hbm, w3_hbm))]
        rows = pl.ds(pl.multiple_of(jnp.minimum(kp, n_dr // 2 - 1) * 2 * DR, 2 * DR), 2 * DR)
        return cps + [pltpu.make_async_copy(w2_hbm.at[:, rows, :], rd.bitcast(BF16).at[slot],
                                            sem_raw.at[slot, 2])]

    def warmup(xp, wmod, stg, tmp, hp):
        hw, hr = HC // 2, n_seg * PRE // 2
        mod_cp = [pltpu.make_async_copy(wmod_hbm.at[:, pl.ds(a * D, n * D)],
                                        wmod.bitcast(BF16).at[:, pl.ds(a * D, n * D)],
                                        sem_mod.at[i])
                  for i, (a, n) in enumerate(((0, 1), (1, 1), (2, 4)))]
        xp_cp = pltpu.make_async_copy(x_hbm.at[:, pl.ds(seg - PRE, PRE), :], xp, sem_x.at[0])

        def stg_cp(t, hc, slot):
            src = (wq_hbm, wk_hbm, wv_hbm)[t]
            return pltpu.make_async_copy(src.at[:, pl.ds(pl.multiple_of(hc * HC, HC), HC), :],
                                         stg.at[slot], sem_stg.at[slot])

        xp_cp.start()
        mod_cp[1].start()
        mod_cp[0].start()
        cv = c_ref[...].astype(F32)
        sc = jnp.broadcast_to(_rnd(cv * jax.nn.sigmoid(cv)), (8, D))
        xp_cp.wait()
        xn = _norm(xp[...].astype(F32).reshape(2 * hr, D))
        mod_cp[1].wait()
        stg_cp(0, 0, 0).start()
        mod[1] = _mm(sc, _unpack(wmod[:, D:2 * D]))
        h = xn * (1.0 + mrow(1))
        scaled = _ops7(_LHS, (h[:hr, :hd], h[:hr, hd:], h[hr:, :hd], h[hr:, hd:]))
        mod_cp[0].wait()
        for i in range(1, NSTG):
            stg_cp(i // n_hc, i % n_hc, i).start()
        mod[0] = _mm(sc, _unpack(wmod[:, 0:D]))
        shift = _ops7(_LHS, (mrow(0)[:, :hd], mrow(0)[:, hd:]) * 2)
        for i in range(7):
            hp[i] = _pack(scaled[i] + shift[i])

        def warm(i, carry):
            slot = lax.rem(i, NSTG)
            stg_cp(0, 0, slot).wait()
            for r in range(D // RP):
                v = stg[slot, pl.ds(r * RP, RP)].reshape(RP * HC, LANE)
                tmp[pl.ds(r * RP * hw, RP * hw), :] = pltpu.bitcast(v, U32)
            ops = []
            for j in range(hw):
                quad = []
                for half in range(2):
                    a = tmp[pl.ds(half * hd * hw + j, hd, stride=hw), :]
                    pair = [pltpu.bitcast(w, F32) for w in (a << 16, a & jnp.uint32(0xFFFF0000))]
                    for k, w in enumerate(_pack_all(pair)):
                        wqkv[i * HC + 2 * j + k, pl.ds(half * hd // 2, hd // 2), :] = w
                    quad += pair
                ops.append(_ops7(_RHS, quad))
            prod = {n: _mm(_unpack(hp[n]),
                           jnp.concatenate([o[n] for o in ops], axis=1).astype(BF16))
                    for n in (1, 5, 0, 2, 3, 4, 6)}
            for n, cq in enumerate(_out4(prod)):
                cq = _pack(cq)
                for j in range(hw):
                    pre[i * HC + 2 * j + n % 2, pl.ds((n // 2) * hr // 2, hr // 2), :] = (
                        cq[:, j * LANE:(j + 1) * LANE])
            nx = i + NSTG
            for t in range(3):
                @pl.when(lax.div(nx, n_hc) == t)
                def _(t=t):
                    stg_cp(t, lax.rem(nx, n_hc), slot).start()

            for at, cps in ((0, [x_cp]), (2, wo_cp[:n_ct // 2]), (4, wo_cp[n_ct // 2:]),
                            (6, [mod_cp[2]]), (9, raw_cp(0, 0))):
                @pl.when(i == at)
                def _(cps=cps):
                    for cp in cps:
                        cp.start()

            return carry

        lax.fori_loop(0, 3 * n_hc, warm, 0)
        mod_cp[2].wait()

        def mod_rest(j, carry):
            mod[j] = _mm(sc, _unpack(wmod[:, pl.ds(pl.multiple_of(j * D, D), D)]))
            return carry

        lax.fori_loop(2, 6, mod_rest, 0)

    pl.run_scoped(warmup,
                  pltpu.VMEM((n_seg, PRE, D), BF16),
                  pltpu.VMEM((hd, 6 * D), U32),
                  pltpu.VMEM((NSTG, D, HC, LANE), BF16),
                  pltpu.VMEM((D * HC // 2, LANE), U32),
                  pltpu.VMEM((7, n_seg * PRE // 4, hd), U32))
    x_cp.wait()
    for cp in wo_cp:
        cp.wait()

    def pre_attn(s):
        xs = xb[s].astype(F32)[0:seg - PRE]
        return _norm(xs) * (1.0 + mrow(1)) + mrow(0)

    def step(k, u, side):
        s = k * UNR + u
        h = _unpack(hin[...])
        ri = lax.broadcasted_iota(jnp.int32, (L, L), 0)
        ci = lax.broadcasted_iota(jnp.int32, (L, L), 1)
        mask = (ri < M) | (ri >= ci)
        prow = pl.ds(pl.multiple_of(k * PRE, PRE), PRE)
        qkv, prob, att = {}, {}, {}

        def proj(g, ts):
            heads = [(t, g * HG + j) for t in ts for j in range(HG)]
            r = _mm(h, jnp.concatenate([_unpack(wqkv[t * H + n]) for t, n in heads], axis=1))
            for i, (t, n) in enumerate(heads):
                early = pre[t * H + n, prow, :]
                if (t, n) in side:
                    early = side[t, n](early)
                early = _unpack(early).astype(F32)[u * PRE:(u + 1) * PRE]
                qkv[t, n] = jnp.concatenate([r[:, i * LANE:(i + 1) * LANE], early], axis=0)

        def scores(g):
            for n in range(g * HG, (g + 1) * HG):
                sv = _mm_nt(_rnd(qkv[0, n]), qkv[1, n].astype(BF16)) * (scale * LOG2E)
                sv = jnp.where(mask, sv, -1e9 * LOG2E)
                e = jnp.exp2(sv - jnp.max(sv, axis=-1, keepdims=True))
                den = jnp.sum(e, axis=-1, keepdims=True)
                inv = pl.reciprocal(den, approx=True)
                prob[n] = _rnd(e * (inv * (2.0 - den * inv)))

        def values(g):
            for n in range(g * HG, (g + 1) * HG):
                att[n] = _rnd(_mm(prob[n], qkv[2, n].astype(BF16)))

        nxt = pre_attn(jnp.minimum(s + 1, n_seg - 1))
        for g in range(n_grp):
            proj(g, (0, 1))
            if g >= 1:
                scores(g - 1)
        for g in range(n_grp):
            proj(g, (2,))
            if g == 0:
                scores(n_grp - 1)
            if g >= VLAG:
                values(g - VLAG)
        for g in range(n_grp - VLAG, n_grp):
            values(g)
        cols = []
        for j in range(n_ct):
            w, per = wo[j], H // n_ct
            rows = w.shape[0] // per
            parts = []
            for i in range(per):
                blk = w[i * rows:(i + 1) * rows]
                if (3, j * per + i) in side:
                    blk = jnp.concatenate([side[3, j * per + i](blk[:8]), blk[8:]], axis=0)
                parts.append(blk)
            cols.append(_unpack(jnp.concatenate(parts, axis=0)))
        acc = _mm(jnp.concatenate([att[n] for n in range(H)], axis=1),
                  jnp.concatenate(cols, axis=1))
        hin[...] = _pack(jnp.concatenate([acc[0:M], nxt], axis=0))
        ab[s] = acc[M:L].astype(BF16)

    def main(wu, wd):
        def steps(k, carry):
            kp, odd = lax.div(k, 2), lax.rem(k, 2)
            slot = lax.rem(kp, 2)
            kd = jnp.minimum(kp, n_dr // 2 - 1) * 2 + odd

            @pl.when(odd == 0)
            def _():
                for cp in raw_cp(kp, slot):
                    cp.wait()

            def up_piece(t, i, v):
                cols = pl.ds(t * LANE, LANE)
                ops = _ops49(_RHS, i, lambda r, c: _unpack(ru[
                    slot, c // 2, r, :,
                    pl.ds(pl.multiple_of((2 * (c % 2) + odd) * qf + t * LANE, LANE), LANE)
                ]).astype(F32))
                for j, o in enumerate(_pack_all(ops)):
                    wu[kp, odd, 7 * i + j, :, cols] = o
                return _after(v, wu[kp, jnp.minimum(odd, 1), 7 * i, :, cols], k)

            def down_piece(a, t, i, v):
                rows, cols = pl.ds(a * 8, 8), pl.ds(t * LANE, LANE)
                src = pl.ds(pl.multiple_of(odd * (DR // 2) + a * 8, 8), 8)
                ops = _ops49(_RHS, i, lambda r, c: _unpack(
                    rd[slot, r, src, pl.ds(c * qd + t * LANE, LANE)]).astype(F32))
                for j, o in enumerate(_pack_all(ops)):
                    wd[kd, 7 * i + j, rows, cols] = o
                return _after(v, wd[jnp.minimum(kd, n_it), 7 * i, rows, cols], k)

            pieces = [functools.partial(up_piece, t, i)
                      for t in range(qf // LANE) for i in range(7)]
            pieces += [functools.partial(down_piece, a, t, i) for a in range(DR // 16)
                       for t in range(qd // LANE) for i in range(7)]
            spots = [(u, t, n) for u in range(UNR) for t, m in SPOT for n in range(H) if n % 4 < m]
            assert len(pieces) <= len(spots)
            for u in range(UNR):
                step(k, u, {sp[1:]: f for sp, f in zip(spots, pieces) if sp[0] == u})

            @pl.when((odd == 0) & (k + 2 < n_it))
            def _():
                for cp in raw_cp(kp + 1, 1 - slot):
                    cp.start()

            return carry

        hin[...] = _pack(jnp.concatenate([mem0_ref[...].astype(F32), pre_attn(0)], axis=0))
        lax.fori_loop(0, n_it, steps, 0)

        def resid(sg, rows):
            return xb[sg, rows, :].astype(F32) + mrow(2) * ab[sg, rows, :].astype(F32)

        def norm_piece(b, r, a):
            rows = pl.ds(a * 16, 16)
            h2f[r, rows, :] = _norm(resid(b * 4 + r, rows)) * (1.0 + mrow(4)) + mrow(3)
            return h2f[jnp.minimum(b, 0) + r, pl.ds(a * 16, 8), 0:qd]

        def lhs_piece(b, a, i):
            ops = _ops49(_LHS, i, lambda r, c: h2f[r, pl.ds(a * 16, 16), pl.ds(c * qd, qd)])
            for j, o in enumerate(ops):
                h2b[7 * i + j, pl.ds(a * 8, 8), :] = _pack(o)
            return h2b[jnp.minimum(b, 0) + 7 * i, pl.ds(a * 8, 8), :]

        ffn_in = [functools.partial(norm_piece, r=r, a=a)
                  for r in range(4) for a in range(seg // 16)]
        ffn_in += [functools.partial(lhs_piece, a=a, i=i)
                   for a in range(seg // 16) for i in range(7)]

        def out_cp(b):
            return pltpu.make_async_copy(ob.at[b % 2], out_hbm.at[pl.ds(b * FM, FM), :],
                                         sem_out.at[b % 2])

        def ffn(b, carry):
            @pl.when(b >= 2)
            def _():
                out_cp(b - 2).wait()

            slot = lax.rem(b, 2)
            lhs = []
            for f in range(qf // LANE):
                cols = pl.ds(f * LANE, LANE)
                gu = _out16([_mm(_unpack(h2b[n]), jnp.concatenate(
                    [_unpack(wu[:, c, n, :, cols].reshape(qd // 2, LANE)) for c in range(2)],
                    axis=1)) for n in range(49)])
                act = {}
                for r in range(4):
                    for c in range(2):
                        v = _silu(gu[r, c]) * gu[r, 2 + c]
                        act[r, 2 * c], act[r, 2 * c + 1] = v[:, :LANE], v[:, LANE:]
                lhs.append([o for i in range(7)
                            for o in _ops49(_LHS, i, lambda r, c: act[r, c])])
            prod, late = [], []
            for n in range(49):
                w = wd[:, n].reshape(qf // 2, qd)
                if n % 2 == 1 and n // 2 < len(ffn_in):
                    token = ffn_in[n // 2](jnp.minimum(b + 1, n_blk - 1))
                    w = jnp.concatenate([_after(w[:8], token, b), w[8:]], axis=0)
                a = [l[n] for l in lhs]
                if n < NSPLIT:
                    ks = (qf - LANE) // 2
                    late.append((a.pop().astype(BF16), _unpack(w[ks:])))
                    w = w[:ks]
                prod.append(_mm(jnp.concatenate(a, axis=1).astype(BF16), _unpack(w)))
                if n == NSPLIT - 1:
                    prod = [_mm(*t) + v for t, v in zip(late, prod)]
            y = _out16(prod)
            for r in range(4):
                yr = jnp.concatenate([y[r, c] for c in range(4)], axis=1)
                ob[slot, pl.ds(r * seg, seg), :] = (
                    resid(b * 4 + r, slice(None)) + mrow(5) * yr).astype(ob.dtype)
            out_cp(b).start()
            return carry

        for piece in ffn_in:
            piece(0)
        lax.fori_loop(0, n_blk, ffn, 0)
        for b in range(n_blk - 2, n_blk):
            out_cp(b).wait()

    pl.run_scoped(main, pltpu.VMEM((n_it // 2, 2, 49, 8, qf), U32),
                  pltpu.VMEM((n_dr, 49, DR // 2, qd), U32))


@functools.partial(jax.jit, static_argnames=("A_seg_len",))
def pallas_adaLN_cond__memory_aug_recurrent_mem_tr__glu_gated_swiglu__prompt_kernel(
    A_x, A_mem0, A_Wq, A_Wk, A_Wv, A_Wo, A_seg_len, B_x, B_w1, B_w3, B_w2, c, w_mod,
):
    del B_x
    B, S, D = A_x.shape
    H, Dh = A_Wq.shape[1], A_Wq.shape[2]
    M = A_mem0.shape[1]
    F = B_w1.shape[1]
    seg = int(A_seg_len)
    n_seg = S // seg
    assert B == 1 and Dh == LANE and S % seg == 0 and S % FM == 0 and F % FC == 0
    hbm = pl.BlockSpec(memory_space=pl.ANY)
    vmem = pl.BlockSpec(memory_space=pltpu.VMEM)
    dma = pltpu.SemaphoreType.DMA
    out = pl.pallas_call(
        _kernel,
        out_shape=jax.ShapeDtypeStruct((S, D), A_x.dtype),
        in_specs=[vmem, vmem] + [hbm] * 9,
        out_specs=hbm,
        scratch_shapes=[
            pltpu.VMEM((n_seg, seg, D), BF16),
            pltpu.VMEM((n_seg, seg, D), BF16),
            pltpu.VMEM((3 * H, D // 2, LANE), U32),
            pltpu.VMEM((3 * H, n_seg * PRE // 2, LANE), U32),
            pltpu.VMEM((D // LANE, H * Dh // 2, LANE), U32),
            pltpu.VMEM((6, 8, D), F32),
            pltpu.VMEM(((M + seg - PRE) // 2, D), U32),
            pltpu.VMEM((2, 2, 4, 8, F), U32),
            pltpu.VMEM((2, 4, DR, D), U32),
            pltpu.VMEM((4, seg, D), F32),
            pltpu.VMEM((49, seg // 2, D // 4), U32),
            pltpu.VMEM((2, FM, D), A_x.dtype),
            dma((2,)), dma((3,)), dma((NSTG,)), dma((D // LANE,)), dma((2, 3)), dma((2,)),
        ],
        compiler_params=pltpu.CompilerParams(vmem_limit_bytes=127 * 2**20),
    )(c, A_mem0.reshape(M, D), A_x.reshape(n_seg, seg, D), A_Wq, A_Wk, A_Wv,
      A_Wo.reshape(H * Dh, D), B_w1.reshape(4, D // 4, F), B_w3.reshape(4, D // 4, F),
      B_w2.reshape(4, F // 4, D), w_mod)
    return out.reshape(B, S, D)
```

```python
import functools

import jax
import jax.numpy as jnp
from jax import lax
import jax.experimental.pallas as pl
import jax.experimental.pallas.tpu as pltpu

F32 = jnp.float32
BF16 = jnp.bfloat16
U32 = jnp.uint32
LANE = 128
LOG2E = 1.4426950408889634
HG = 4
HC = 8
RP = 64
VLAG = 4
SPOT = ((1, 1), (2, 1), (3, 3))
DR = 32
UNR = 2
NSPLIT = 6
KCUT = {1: (0, 128, 512)}
NSTG = 4
PRE = 8
FM = 128
FC = 256


def _mm(a, b):
    return lax.dot_general(a, b, (((1,), (0,)), ((), ())), preferred_element_type=F32)


def _mm_nt(a, b):
    return lax.dot_general(a, b, (((1,), (1,)), ((), ())), preferred_element_type=F32)


def _rnd(v):
    return v.astype(BF16).astype(F32)


def _pack(v):
    return pltpu.bitcast(v.astype(BF16), U32)


def _pack_all(vs):
    n = vs[0].shape[1]
    w = _pack(jnp.concatenate(vs, axis=1))
    return [w[:, i * n:(i + 1) * n] for i in range(len(vs))]


def _unpack(v):
    return pltpu.bitcast(v, BF16)


_LHS = (((1, 0), (1, 3)), ((1, 2), (1, 3)), ((1, 0),), ((1, 3),), ((1, 0), (1, 1)),
        ((1, 2), (-1, 0)), ((1, 1), (-1, 3)))
_RHS = (((1, 0), (1, 3)), ((1, 0),), ((1, 1), (-1, 3)), ((1, 2), (-1, 0)), ((1, 3),),
        ((1, 0), (1, 1)), ((1, 2), (1, 3)))


def _comb(terms, quad):
    v = quad(terms[0][1])
    for sign, q in terms[1:]:
        v = v + quad(q) if sign > 0 else v - quad(q)
    return v


def _ops7(table, quads):
    return [_comb(t, quads.__getitem__) for t in table]


def _ops49(table, i, block):
    return _ops7(table, [
        _comb(table[i], lambda q: block(2 * (q // 2) + r, 2 * (q % 2) + c))
        for r in range(2) for c in range(2)])


def _out4(m):
    return (m[0] + m[3] - m[4] + m[6], m[2] + m[4], m[1] + m[3], m[0] - m[1] + m[2] + m[5])


def _out16(m):
    inner = [_out4(m[7 * i:7 * i + 7]) for i in range(7)]
    return {(2 * (q // 2) + p // 2, 2 * (q % 2) + p % 2): v
            for p in range(4) for q, v in enumerate(_out4([c[p] for c in inner]))}


def _after(v, token, i):
    return jnp.where(i < 0, pltpu.bitcast(token, v.dtype), v)


def _silu(g):
    hg = 0.5 * g
    return hg * jnp.tanh(hg) + hg


def _norm(x):
    m = jnp.mean(x, axis=-1, keepdims=True)
    xc = x - m
    v = jnp.mean(xc * xc, axis=-1, keepdims=True)
    return xc * lax.rsqrt(v + 1e-5)


def _kernel(c_ref, mem0_ref, x_hbm, wq_hbm, wk_hbm, wv_hbm, wo_hbm, w1_hbm, w3_hbm, w2_hbm,
            wmod_hbm, out_hbm,
            xb, ab, wqkv, pre, wo, mod, hin, ru, rd, h2f, h2b, ob,
            sem_x, sem_mod, sem_stg, sem_wo, sem_raw, sem_out):
    n_seg, seg, D = xb.shape
    M = mem0_ref.shape[0]
    L = M + seg
    H = wq_hbm.shape[1]
    F = w1_hbm.shape[2]
    n_grp, n_ct, n_hc = H // HG, D // LANE, H // HC
    n_it = n_seg // UNR
    n_blk, spb = n_seg * seg // FM, FM // seg
    hd, qd, qf = D // 2, D // 4, F // 4
    n_dr = qf // DR
    scale = float(LANE) ** -0.5

    def mrow(j):
        return mod[j, 0:1, :]

    x_cp = pltpu.make_async_copy(x_hbm, xb, sem_x.at[1])
    wo_cp = [pltpu.make_async_copy(wo_hbm.at[:, pl.ds(j * LANE, LANE)], wo.bitcast(BF16).at[j],
                                   sem_wo.at[j])
             for j in range(n_ct)]

    def raw_cp(kp, slot):
        rows = pl.ds(pl.multiple_of(kp * 16, 16), 16)
        cps = [pltpu.make_async_copy(w.at[:, rows, :], ru.bitcast(BF16).at[slot, j],
                                     sem_raw.at[slot, j])
               for j, w in enumerate((w1_hbm, w3_hbm))]
        rows = pl.ds(pl.multiple_of(jnp.minimum(kp, n_dr // 2 - 1) * 2 * DR, 2 * DR), 2 * DR)
        return cps + [pltpu.make_async_copy(w2_hbm.at[:, rows, :], rd.bitcast(BF16).at[slot],
                                            sem_raw.at[slot, 2])]

    def warmup(xp, wmod, stg, tmp, hp):
        hw, hr = HC // 2, n_seg * PRE // 2
        mod_cp = [pltpu.make_async_copy(wmod_hbm.at[:, pl.ds(a * D, n * D)],
                                        wmod.bitcast(BF16).at[:, pl.ds(a * D, n * D)],
                                        sem_mod.at[i])
                  for i, (a, n) in enumerate(((0, 1), (1, 1), (2, 4)))]
        xp_cp = pltpu.make_async_copy(x_hbm.at[:, pl.ds(seg - PRE, PRE), :], xp, sem_x.at[0])

        def stg_cp(t, hc, slot):
            src = (wq_hbm, wk_hbm, wv_hbm)[t]
            return pltpu.make_async_copy(src.at[:, pl.ds(pl.multiple_of(hc * HC, HC), HC), :],
                                         stg.at[slot], sem_stg.at[slot])

        xp_cp.start()
        mod_cp[1].start()
        mod_cp[0].start()
        cv = c_ref[...].astype(F32)
        sc = jnp.broadcast_to(_rnd(cv * jax.nn.sigmoid(cv)), (8, D))
        xp_cp.wait()
        xn = _norm(xp[...].astype(F32).reshape(2 * hr, D))
        mod_cp[1].wait()
        stg_cp(0, 0, 0).start()
        mod[1] = _mm(sc, _unpack(wmod[:, D:2 * D]))
        h = xn * (1.0 + mrow(1))
        scaled = _ops7(_LHS, (h[:hr, :hd], h[:hr, hd:], h[hr:, :hd], h[hr:, hd:]))
        mod_cp[0].wait()
        for i in range(1, NSTG):
            stg_cp(i // n_hc, i % n_hc, i).start()
        mod[0] = _mm(sc, _unpack(wmod[:, 0:D]))
        shift = _ops7(_LHS, (mrow(0)[:, :hd], mrow(0)[:, hd:]) * 2)
        for i in range(7):
            hp[i] = _pack(scaled[i] + shift[i])

        def warm(i, carry):
            slot = lax.rem(i, NSTG)
            stg_cp(0, 0, slot).wait()
            for r in range(D // RP):
                v = stg[slot, pl.ds(r * RP, RP)].reshape(RP * HC, LANE)
                tmp[pl.ds(r * RP * hw, RP * hw), :] = pltpu.bitcast(v, U32)
            ops = []
            for j in range(hw):
                quad = []
                for half in range(2):
                    a = tmp[pl.ds(half * hd * hw + j, hd, stride=hw), :]
                    pair = [pltpu.bitcast(w, F32) for w in (a << 16, a & jnp.uint32(0xFFFF0000))]
                    for k, w in enumerate(_pack_all(pair)):
                        wqkv[i * HC + 2 * j + k, pl.ds(half * hd // 2, hd // 2), :] = w
                    quad += pair
                ops.append(_ops7(_RHS, quad))
            prod = {}
            for n in (1, 5, 0, 2, 3, 4, 6):
                w = jnp.concatenate([o[n] for o in ops], axis=1)
                cuts = KCUT.get(n, (0, hd))
                for k0, k1 in zip(cuts, cuts[1:]):
                    v = _mm(_unpack(hp[n, :, k0:k1]), w[k0:k1].astype(BF16))
                    prod[n] = v + prod[n] if k0 else v
            for n, cq in enumerate(_out4(prod)):
                cq = _pack(cq)
                for j in range(hw):
                    pre[i * HC + 2 * j + n % 2, pl.ds((n // 2) * hr // 2, hr // 2), :] = (
                        cq[:, j * LANE:(j + 1) * LANE])
            nx = i + NSTG
            for t in range(3):
                @pl.when(lax.div(nx, n_hc) == t)
                def _(t=t):
                    stg_cp(t, lax.rem(nx, n_hc), slot).start()

            for at, cps in ((0, [x_cp]), (2, wo_cp[:n_ct // 2]), (4, wo_cp[n_ct // 2:]),
                            (3 * n_hc - NSTG - 1, [mod_cp[2]] + raw_cp(0, 0))):
                @pl.when(i == at)
                def _(cps=cps):
                    for cp in cps:
                        cp.start()

            return carry

        lax.fori_loop(0, 3 * n_hc, warm, 0)
        mod_cp[2].wait()

        def mod_rest(j, carry):
            mod[j] = _mm(sc, _unpack(wmod[:, pl.ds(pl.multiple_of(j * D, D), D)]))
            return carry

        lax.fori_loop(2, 6, mod_rest, 0)

    pl.run_scoped(warmup,
                  pltpu.VMEM((n_seg, PRE, D), BF16),
                  pltpu.VMEM((hd, 6 * D), U32),
                  pltpu.VMEM((NSTG, D, HC, LANE), BF16),
                  pltpu.VMEM((D * HC // 2, LANE), U32),
                  pltpu.VMEM((7, n_seg * PRE // 4, hd), U32))
    x_cp.wait()
    for cp in wo_cp:
        cp.wait()

    def pre_attn(s):
        xs = xb[s].astype(F32)[0:seg - PRE]
        return _norm(xs) * (1.0 + mrow(1)) + mrow(0)

    def step(k, u, side):
        s = k * UNR + u
        h = _unpack(hin[...])
        ri = lax.broadcasted_iota(jnp.int32, (L, L), 0)
        ci = lax.broadcasted_iota(jnp.int32, (L, L), 1)
        mask = (ri < M) | (ri >= ci)
        prow = pl.ds(pl.multiple_of(k * PRE, PRE), PRE)
        qkv, prob, att = {}, {}, {}

        def proj(g, ts):
            heads = [(t, g * HG + j) for t in ts for j in range(HG)]
            r = _mm(h, jnp.concatenate([_unpack(wqkv[t * H + n]) for t, n in heads], axis=1))
            for i, (t, n) in enumerate(heads):
                early = pre[t * H + n, prow, :]
                if (t, n) in side:
                    early = side[t, n](early)
                early = _unpack(early).astype(F32)[u * PRE:(u + 1) * PRE]
                qkv[t, n] = jnp.concatenate([r[:, i * LANE:(i + 1) * LANE], early], axis=0)

        def scores(g):
            for n in range(g * HG, (g + 1) * HG):
                sv = _mm_nt(_rnd(qkv[0, n]), qkv[1, n].astype(BF16)) * (scale * LOG2E)
                sv = jnp.where(mask, sv, -1e9 * LOG2E)
                e = jnp.exp2(sv - jnp.max(sv, axis=-1, keepdims=True))
                den = jnp.sum(e, axis=-1, keepdims=True)
                inv = pl.reciprocal(den, approx=True)
                prob[n] = _rnd(e * (inv * (2.0 - den * inv)))

        def values(g):
            for n in range(g * HG, (g + 1) * HG):
                att[n] = _rnd(_mm(prob[n], qkv[2, n].astype(BF16)))

        nxt = pre_attn(jnp.minimum(s + 1, n_seg - 1))
        for g in range(n_grp):
            proj(g, (0, 1))
            if g >= 1:
                scores(g - 1)
        for g in range(n_grp):
            proj(g, (2,))
            if g == 0:
                scores(n_grp - 1)
            if g >= VLAG:
                values(g - VLAG)
        for g in range(n_grp - VLAG, n_grp):
            values(g)
        cols = []
        for j in range(n_ct):
            w, per = wo[j], H // n_ct
            rows = w.shape[0] // per
            parts = []
            for i in range(per):
                blk = w[i * rows:(i + 1) * rows]
                if (3, j * per + i) in side:
                    blk = jnp.concatenate([side[3, j * per + i](blk[:8]), blk[8:]], axis=0)
                parts.append(blk)
            cols.append(_unpack(jnp.concatenate(parts, axis=0)))
        acc = _mm(jnp.concatenate([att[n] for n in range(H)], axis=1),
                  jnp.concatenate(cols, axis=1))
        hin[...] = _pack(jnp.concatenate([acc[0:M], nxt], axis=0))
        ab[s] = acc[M:L].astype(BF16)

    def main(wu, wd):
        def steps(k, carry):
            kp, odd = lax.div(k, 2), lax.rem(k, 2)
            slot = lax.rem(kp, 2)
            kd = jnp.minimum(kp, n_dr // 2 - 1) * 2 + odd

            @pl.when(odd == 0)
            def _():
                for cp in raw_cp(kp, slot):
                    cp.wait()

            def up_piece(t, i, v):
                cols = pl.ds(t * LANE, LANE)
                ops = _ops49(_RHS, i, lambda r, c: _unpack(ru[
                    slot, c // 2, r, :,
                    pl.ds(pl.multiple_of((2 * (c % 2) + odd) * qf + t * LANE, LANE), LANE)
                ]).astype(F32))
                for j, o in enumerate(_pack_all(ops)):
                    wu[kp, odd, 7 * i + j, :, cols] = o
                return _after(v, wu[kp, jnp.minimum(odd, 1), 7 * i, :, cols], k)

            def down_piece(a, t, i, v):
                rows, cols = pl.ds(a * 8, 8), pl.ds(t * LANE, LANE)
                src = pl.ds(pl.multiple_of(odd * (DR // 2) + a * 8, 8), 8)
                ops = _ops49(_RHS, i, lambda r, c: _unpack(
                    rd[slot, r, src, pl.ds(c * qd + t * LANE, LANE)]).astype(F32))
                for j, o in enumerate(_pack_all(ops)):
                    wd[kd, 7 * i + j, rows, cols] = o
                return _after(v, wd[jnp.minimum(kd, n_it), 7 * i, rows, cols], k)

            pieces = [functools.partial(up_piece, t, i)
                      for t in range(qf // LANE) for i in range(7)]
            pieces += [functools.partial(down_piece, a, t, i) for a in range(DR // 16)
                       for t in range(qd // LANE) for i in range(7)]
            spots = [(u, t, n) for u in range(UNR) for t, m in SPOT for n in range(H) if n % 4 < m]
            assert len(pieces) <= len(spots)
            for u in range(UNR):
                step(k, u, {sp[1:]: f for sp, f in zip(spots, pieces) if sp[0] == u})

            @pl.when((odd == 0) & (k + 2 < n_it))
            def _():
                for cp in raw_cp(kp + 1, 1 - slot):
                    cp.start()

            return carry

        hin[...] = _pack(jnp.concatenate([mem0_ref[...].astype(F32), pre_attn(0)], axis=0))
        lax.fori_loop(0, n_it, steps, 0)

        def resid(sg, rows):
            return xb[sg, rows, :].astype(F32) + mrow(2) * ab[sg, rows, :].astype(F32)

        def norm_piece(b, r, a):
            rows = pl.ds(a * 16, 16)
            h2f[r, rows, :] = _norm(resid(b * 4 + r, rows)) * (1.0 + mrow(4)) + mrow(3)
            return h2f[jnp.minimum(b, 0) + r, pl.ds(a * 16, 8), 0:qd]

        def lhs_piece(b, a, i):
            ops = _ops49(_LHS, i, lambda r, c: h2f[r, pl.ds(a * 16, 16), pl.ds(c * qd, qd)])
            for j, o in enumerate(ops):
                h2b[7 * i + j, pl.ds(a * 8, 8), :] = _pack(o)
            return h2b[jnp.minimum(b, 0) + 7 * i, pl.ds(a * 8, 8), :]

        ffn_in = [functools.partial(norm_piece, r=r, a=a)
                  for r in range(4) for a in range(seg // 16)]
        ffn_in += [functools.partial(lhs_piece, a=a, i=i)
                   for a in range(seg // 16) for i in range(7)]

        def out_cp(b):
            return pltpu.make_async_copy(ob.at[b % 2], out_hbm.at[pl.ds(b * FM, FM), :],
                                         sem_out.at[b % 2])

        def ffn(b, carry):
            @pl.when(b >= 2)
            def _():
                out_cp(b - 2).wait()

            slot = lax.rem(b, 2)
            lhs = []
            for f in range(qf // LANE):
                cols = pl.ds(f * LANE, LANE)
                gu = _out16([_mm(_unpack(h2b[n]), jnp.concatenate(
                    [_unpack(wu[:, c, n, :, cols].reshape(qd // 2, LANE)) for c in range(2)],
                    axis=1)) for n in range(49)])
                act = {}
                for r in range(4):
                    for c in range(2):
                        v = _silu(gu[r, c]) * gu[r, 2 + c]
                        act[r, 2 * c], act[r, 2 * c + 1] = v[:, :LANE], v[:, LANE:]
                lhs.append([o for i in range(7)
                            for o in _ops49(_LHS, i, lambda r, c: act[r, c])])
            prod, late = [], []
            for n in range(49):
                w = wd[:, n].reshape(qf // 2, qd)
                if n % 2 == 1 and n // 2 < len(ffn_in):
                    token = ffn_in[n // 2](jnp.minimum(b + 1, n_blk - 1))
                    w = jnp.concatenate([_after(w[:8], token, b), w[8:]], axis=0)
                a = [l[n] for l in lhs]
                if n < NSPLIT:
                    ks = (qf - LANE) // 2
                    late.append((a.pop().astype(BF16), _unpack(w[ks:])))
                    w = w[:ks]
                prod.append(_mm(jnp.concatenate(a, axis=1).astype(BF16), _unpack(w)))
                if n == NSPLIT - 1:
                    prod = [_mm(*t) + v for t, v in zip(late, prod)]
            y = _out16(prod)
            for r in range(4):
                yr = jnp.concatenate([y[r, c] for c in range(4)], axis=1)
                ob[slot, pl.ds(r * seg, seg), :] = (
                    resid(b * 4 + r, slice(None)) + mrow(5) * yr).astype(ob.dtype)
            out_cp(b).start()
            return carry

        for piece in ffn_in:
            piece(0)
        lax.fori_loop(0, n_blk, ffn, 0)
        for b in range(n_blk - 2, n_blk):
            out_cp(b).wait()

    pl.run_scoped(main, pltpu.VMEM((n_it // 2, 2, 49, 8, qf), U32),
                  pltpu.VMEM((n_dr, 49, DR // 2, qd), U32))


@functools.partial(jax.jit, static_argnames=("A_seg_len",))
def pallas_adaLN_cond__memory_aug_recurrent_mem_tr__glu_gated_swiglu__prompt_kernel(
    A_x, A_mem0, A_Wq, A_Wk, A_Wv, A_Wo, A_seg_len, B_x, B_w1, B_w3, B_w2, c, w_mod,
):
    del B_x
    B, S, D = A_x.shape
    H, Dh = A_Wq.shape[1], A_Wq.shape[2]
    M = A_mem0.shape[1]
    F = B_w1.shape[1]
    seg = int(A_seg_len)
    n_seg = S // seg
    assert B == 1 and Dh == LANE and S % seg == 0 and S % FM == 0 and F % FC == 0
    hbm = pl.BlockSpec(memory_space=pl.ANY)
    vmem = pl.BlockSpec(memory_space=pltpu.VMEM)
    dma = pltpu.SemaphoreType.DMA
    out = pl.pallas_call(
        _kernel,
        out_shape=jax.ShapeDtypeStruct((S, D), A_x.dtype),
        in_specs=[vmem, vmem] + [hbm] * 9,
        out_specs=hbm,
        scratch_shapes=[
            pltpu.VMEM((n_seg, seg, D), BF16),
            pltpu.VMEM((n_seg, seg, D), BF16),
            pltpu.VMEM((3 * H, D // 2, LANE), U32),
            pltpu.VMEM((3 * H, n_seg * PRE // 2, LANE), U32),
            pltpu.VMEM((D // LANE, H * Dh // 2, LANE), U32),
            pltpu.VMEM((6, 8, D), F32),
            pltpu.VMEM(((M + seg - PRE) // 2, D), U32),
            pltpu.VMEM((2, 2, 4, 8, F), U32),
            pltpu.VMEM((2, 4, DR, D), U32),
            pltpu.VMEM((4, seg, D), F32),
            pltpu.VMEM((49, seg // 2, D // 4), U32),
            pltpu.VMEM((2, FM, D), A_x.dtype),
            dma((2,)), dma((3,)), dma((NSTG,)), dma((D // LANE,)), dma((2, 3)), dma((2,)),
        ],
        compiler_params=pltpu.CompilerParams(vmem_limit_bytes=127 * 2**20),
    )(c, A_mem0.reshape(M, D), A_x.reshape(n_seg, seg, D), A_Wq, A_Wk, A_Wv,
      A_Wo.reshape(H * Dh, D), B_w1.reshape(4, D // 4, F), B_w3.reshape(4, D // 4, F),
      B_w2.reshape(4, F // 4, D), w_mod)
    return out.reshape(B, S, D)
```

```python
import functools

import jax
import jax.numpy as jnp
from jax import lax
import jax.experimental.pallas as pl
import jax.experimental.pallas.tpu as pltpu

F32 = jnp.float32
BF16 = jnp.bfloat16
U32 = jnp.uint32
LANE = 128
LOG2E = 1.4426950408889634
HG = 4
HC = 8
RP = 64
VLAG = 4
SPOT = ((1, 1), (2, 1), (3, 3))
DR = 32
UNR = 2
NSPLIT = 6
KCUT = {1: (0, 128, 512)}
TIES = tuple(range(14, 36))
NSTG = 4
PRE = 8
FM = 128
FC = 256


def _mm(a, b):
    return lax.dot_general(a, b, (((1,), (0,)), ((), ())), preferred_element_type=F32)


def _mm_nt(a, b):
    return lax.dot_general(a, b, (((1,), (1,)), ((), ())), preferred_element_type=F32)


def _rnd(v):
    return v.astype(BF16).astype(F32)


def _pack(v):
    return pltpu.bitcast(v.astype(BF16), U32)


def _pack_all(vs):
    n = vs[0].shape[1]
    w = _pack(jnp.concatenate(vs, axis=1))
    return [w[:, i * n:(i + 1) * n] for i in range(len(vs))]


def _unpack(v):
    return pltpu.bitcast(v, BF16)


_LHS = (((1, 0), (1, 3)), ((1, 2), (1, 3)), ((1, 0),), ((1, 3),), ((1, 0), (1, 1)),
        ((1, 2), (-1, 0)), ((1, 1), (-1, 3)))
_RHS = (((1, 0), (1, 3)), ((1, 0),), ((1, 1), (-1, 3)), ((1, 2), (-1, 0)), ((1, 3),),
        ((1, 0), (1, 1)), ((1, 2), (1, 3)))


def _comb(terms, quad):
    v = quad(terms[0][1])
    for sign, q in terms[1:]:
        v = v + quad(q) if sign > 0 else v - quad(q)
    return v


def _ops7(table, quads):
    return [_comb(t, quads.__getitem__) for t in table]


def _ops49(table, i, block):
    return _ops7(table, [
        _comb(table[i], lambda q: block(2 * (q // 2) + r, 2 * (q % 2) + c))
        for r in range(2) for c in range(2)])


def _out4(m):
    return (m[0] + m[3] - m[4] + m[6], m[2] + m[4], m[1] + m[3], m[0] - m[1] + m[2] + m[5])


def _out16(m):
    inner = [_out4(m[7 * i:7 * i + 7]) for i in range(7)]
    return {(2 * (q // 2) + p // 2, 2 * (q % 2) + p % 2): v
            for p in range(4) for q, v in enumerate(_out4([c[p] for c in inner]))}


def _after(v, token, i):
    return jnp.where(i < 0, pltpu.bitcast(token, v.dtype), v)


def _silu(g):
    hg = 0.5 * g
    return hg * jnp.tanh(hg) + hg


def _norm(x):
    m = jnp.mean(x, axis=-1, keepdims=True)
    xc = x - m
    v = jnp.mean(xc * xc, axis=-1, keepdims=True)
    return xc * lax.rsqrt(v + 1e-5)


def _kernel(c_ref, mem0_ref, x_hbm, wq_hbm, wk_hbm, wv_hbm, wo_hbm, w1_hbm, w3_hbm, w2_hbm,
            wmod_hbm, out_hbm,
            xb, ab, wqkv, pre, wo, mod, hin, ru, rd, h2f, h2b, ob,
            sem_x, sem_mod, sem_stg, sem_raw, sem_out):
    n_seg, seg, D = xb.shape
    M = mem0_ref.shape[0]
    L = M + seg
    H = wq_hbm.shape[1]
    F = w1_hbm.shape[2]
    n_grp, n_ct, n_hc = H // HG, D // LANE, H // HC
    n_it = n_seg // UNR
    n_blk, spb = n_seg * seg // FM, FM // seg
    hd, qd, qf = D // 2, D // 4, F // 4
    n_dr = qf // DR
    scale = float(LANE) ** -0.5

    def mrow(j):
        return mod[j, 0:1, :]

    def pre_attn(s):
        xs = xb[s].astype(F32)[0:seg - PRE]
        return _norm(xs) * (1.0 + mrow(1)) + mrow(0)

    x_cp = pltpu.make_async_copy(x_hbm, xb, sem_x.at[1])
    wo_cp = pltpu.make_async_copy(wo_hbm, wo.bitcast(BF16), sem_x.at[2])

    def raw_cp(kp, slot):
        rows = pl.ds(pl.multiple_of(kp * 16, 16), 16)
        cps = [pltpu.make_async_copy(w.at[:, rows, :], ru.bitcast(BF16).at[slot, j],
                                     sem_raw.at[slot, j])
               for j, w in enumerate((w1_hbm, w3_hbm))]
        rows = pl.ds(pl.multiple_of(jnp.minimum(kp, n_dr // 2 - 1) * 2 * DR, 2 * DR), 2 * DR)
        return cps + [pltpu.make_async_copy(w2_hbm.at[:, rows, :], rd.bitcast(BF16).at[slot],
                                            sem_raw.at[slot, 2])]

    def warmup(xp, wm0, wm1, wm2, stg, tmp, hp):
        hw, hr = HC // 2, n_seg * PRE // 2
        mod_cp = [pltpu.make_async_copy(wmod_hbm.at[:, pl.ds(i * D, w.shape[1])],
                                        w.bitcast(BF16), sem_mod.at[i])
                  for i, w in enumerate((wm0, wm1, wm2))]
        xp_cp = pltpu.make_async_copy(x_hbm.at[:, pl.ds(seg - PRE, PRE), :], xp, sem_x.at[0])

        def stg_cp(t, hc, slot):
            src = (wq_hbm, wk_hbm, wv_hbm)[t]
            return pltpu.make_async_copy(src.at[:, pl.ds(pl.multiple_of(hc * HC, HC), HC), :],
                                         stg.at[slot], sem_stg.at[slot])

        xp_cp.start()
        mod_cp[1].start()
        mod_cp[0].start()
        cv = c_ref[...].astype(F32)
        sc = jnp.broadcast_to(_rnd(cv * jax.nn.sigmoid(cv)), (8, D))
        xp_cp.wait()
        xn = _norm(xp[...].astype(F32).reshape(2 * hr, D))
        mod_cp[1].wait()
        stg_cp(0, 0, 0).start()
        mod[1] = _mm(sc, _unpack(wm1[...]))
        h = xn * (1.0 + mrow(1))
        scaled = _ops7(_LHS, (h[:hr, :hd], h[:hr, hd:], h[hr:, :hd], h[hr:, hd:]))
        mod_cp[0].wait()
        for i in range(1, NSTG):
            stg_cp(i // n_hc, i % n_hc, i).start()
        mod[0] = _mm(sc, _unpack(wm0[...]))
        shift = _ops7(_LHS, (mrow(0)[:, :hd], mrow(0)[:, hd:]) * 2)
        for i in range(7):
            hp[i] = _pack(scaled[i] + shift[i])

        def warm(i, carry):
            slot = lax.rem(i, NSTG)
            stg_cp(0, 0, slot).wait()
            for r in range(D // RP):
                v = stg[slot, pl.ds(r * RP, RP)].reshape(RP * HC, LANE)
                tmp[pl.ds(r * RP * hw, RP * hw), :] = pltpu.bitcast(v, U32)
            ops = []
            for j in range(hw):
                quad = []
                for half in range(2):
                    a = tmp[pl.ds(half * hd * hw + j, hd, stride=hw), :]
                    pair = [pltpu.bitcast(w, F32) for w in (a << 16, a & jnp.uint32(0xFFFF0000))]
                    for k, w in enumerate(_pack_all(pair)):
                        wqkv[i * HC + 2 * j + k, pl.ds(half * hd // 2, hd // 2), :] = w
                    quad += pair
                ops.append(_ops7(_RHS, quad))
            prod = {}
            for n in (1, 5, 0, 2, 3, 4, 6):
                w = jnp.concatenate([o[n] for o in ops], axis=1)
                cuts = KCUT.get(n, (0, hd))
                for k0, k1 in zip(cuts, cuts[1:]):
                    v = _mm(_unpack(hp[n, :, k0:k1]), w[k0:k1].astype(BF16))
                    prod[n] = v + prod[n] if k0 else v
            for n, cq in enumerate(_out4(prod)):
                cq = _pack(cq)
                for j in range(hw):
                    pre[i * HC + 2 * j + n % 2, pl.ds((n // 2) * hr // 2, hr // 2), :] = (
                        cq[:, j * LANE:(j + 1) * LANE])
            nx = i + NSTG
            for t in range(3):
                @pl.when(lax.div(nx, n_hc) == t)
                def _(t=t):
                    stg_cp(t, lax.rem(nx, n_hc), slot).start()

            for at, cps in ((0, [x_cp]), (2, [wo_cp]),
                            (3 * n_hc - NSTG - 1, [mod_cp[2]] + raw_cp(0, 0))):
                @pl.when(i == at)
                def _(cps=cps):
                    for cp in cps:
                        cp.start()

            return carry

        lax.fori_loop(0, 3 * n_hc, warm, 0)
        mod_cp[2].wait()
        x_cp.wait()
        hin[...] = _pack(jnp.concatenate([mem0_ref[...].astype(F32), pre_attn(0)], axis=0))
        rest = _mm(sc, _unpack(wm2[...]))
        for j in range(4):
            mod[2 + j] = rest[:, j * D:(j + 1) * D]

    pl.run_scoped(warmup,
                  pltpu.VMEM((n_seg, PRE, D), BF16),
                  pltpu.VMEM((hd, D), U32),
                  pltpu.VMEM((hd, D), U32),
                  pltpu.VMEM((hd, 4 * D), U32),
                  pltpu.VMEM((NSTG, D, HC, LANE), BF16),
                  pltpu.VMEM((D * HC // 2 + 8, LANE), U32),
                  pltpu.VMEM((7, n_seg * PRE // 4, hd), U32))
    wo_cp.wait()

    def step(k, u, side):
        s = k * UNR + u
        h = _unpack(hin[...])
        ri = lax.broadcasted_iota(jnp.int32, (L, L), 0)
        ci = lax.broadcasted_iota(jnp.int32, (L, L), 1)
        mask = (ri < M) | (ri >= ci)
        prow = pl.ds(pl.multiple_of(k * PRE, PRE), PRE)
        qkv, prob, att = {}, {}, {}

        def proj(g, ts):
            heads = [(t, g * HG + j) for t in ts for j in range(HG)]
            r = _mm(h, jnp.concatenate([_unpack(wqkv[t * H + n]) for t, n in heads], axis=1))
            for i, (t, n) in enumerate(heads):
                early = pre[t * H + n, prow, :]
                if (t, n) in side:
                    early = side[t, n](early)
                early = _unpack(early).astype(F32)[u * PRE:(u + 1) * PRE]
                qkv[t, n] = jnp.concatenate([r[:, i * LANE:(i + 1) * LANE], early], axis=0)

        def scores(g):
            for n in range(g * HG, (g + 1) * HG):
                sv = _mm_nt(_rnd(qkv[0, n]), qkv[1, n].astype(BF16)) * (scale * LOG2E)
                sv = jnp.where(mask, sv, -1e9 * LOG2E)
                e = jnp.exp2(sv - jnp.max(sv, axis=-1, keepdims=True))
                den = jnp.sum(e, axis=-1, keepdims=True)
                inv = pl.reciprocal(den, approx=True)
                prob[n] = _rnd(e * (inv * (2.0 - den * inv)))

        def values(g):
            for n in range(g * HG, (g + 1) * HG):
                att[n] = _rnd(_mm(prob[n], qkv[2, n].astype(BF16)))

        nxt = pre_attn(jnp.minimum(s + 1, n_seg - 1))
        for g in range(n_grp):
            proj(g, (0, 1))
            if g >= 1:
                scores(g - 1)
        for g in range(n_grp):
            proj(g, (2,))
            if g == 0:
                scores(n_grp - 1)
            if g >= VLAG:
                values(g - VLAG)
        for g in range(n_grp - VLAG, n_grp):
            values(g)
        cols = []
        for j in range(n_ct):
            w, per = wo[:, j * LANE:(j + 1) * LANE], H // n_ct
            rows = w.shape[0] // per
            parts = []
            for i in range(per):
                blk = w[i * rows:(i + 1) * rows]
                if (3, j * per + i) in side:
                    blk = jnp.concatenate([side[3, j * per + i](blk[:8]), blk[8:]], axis=0)
                parts.append(blk)
            cols.append(_unpack(jnp.concatenate(parts, axis=0)))
        acc = _mm(jnp.concatenate([att[n] for n in range(H)], axis=1),
                  jnp.concatenate(cols, axis=1))
        hin[...] = _pack(jnp.concatenate([acc[0:M], nxt], axis=0))
        ab[s] = acc[M:L].astype(BF16)

    def main(wu, wd):
        def steps(k, carry):
            kp, odd = lax.div(k, 2), lax.rem(k, 2)
            slot = lax.rem(kp, 2)
            kd = jnp.minimum(kp, n_dr // 2 - 1) * 2 + odd

            @pl.when(odd == 0)
            def _():
                for cp in raw_cp(kp, slot):
                    cp.wait()

            def up_piece(t, i, v):
                cols = pl.ds(t * LANE, LANE)
                ops = _ops49(_RHS, i, lambda r, c: _unpack(ru[
                    slot, c // 2, r, :,
                    pl.ds(pl.multiple_of((2 * (c % 2) + odd) * qf + t * LANE, LANE), LANE)
                ]).astype(F32))
                for j, o in enumerate(_pack_all(ops)):
                    wu[kp, odd, 7 * i + j, :, cols] = o
                return _after(v, wu[kp, jnp.minimum(odd, 1), 7 * i, :, cols], k)

            def down_piece(a, t, i, v):
                rows, cols = pl.ds(a * 8, 8), pl.ds(t * LANE, LANE)
                src = pl.ds(pl.multiple_of(odd * (DR // 2) + a * 8, 8), 8)
                ops = _ops49(_RHS, i, lambda r, c: _unpack(
                    rd[slot, r, src, pl.ds(c * qd + t * LANE, LANE)]).astype(F32))
                for j, o in enumerate(_pack_all(ops)):
                    wd[kd, 7 * i + j, rows, cols] = o
                return _after(v, wd[jnp.minimum(kd, n_it), 7 * i, rows, cols], k)

            pieces = [functools.partial(up_piece, t, i)
                      for t in range(qf // LANE) for i in range(7)]
            pieces += [functools.partial(down_piece, a, t, i) for a in range(DR // 16)
                       for t in range(qd // LANE) for i in range(7)]
            spots = [(u, t, n) for u in range(UNR) for t, m in SPOT for n in range(H) if n % 4 < m]
            assert len(pieces) <= len(spots)
            for u in range(UNR):
                step(k, u, {sp[1:]: f for sp, f in zip(spots, pieces) if sp[0] == u})

            @pl.when((odd == 0) & (k + 2 < n_it))
            def _():
                for cp in raw_cp(kp + 1, 1 - slot):
                    cp.start()

            return carry

        lax.fori_loop(0, n_it, steps, 0)

        def resid(sg, rows):
            return xb[sg, rows, :].astype(F32) + mrow(2) * ab[sg, rows, :].astype(F32)

        def norm_piece(b, r, a):
            rows = pl.ds(a * 16, 16)
            h2f[r, rows, :] = _norm(resid(b * 4 + r, rows)) * (1.0 + mrow(4)) + mrow(3)
            return h2f[jnp.minimum(b, 0) + r, pl.ds(a * 16, 8), 0:qd]

        def lhs_piece(b, a, i):
            ops = _ops49(_LHS, i, lambda r, c: h2f[r, pl.ds(a * 16, 16), pl.ds(c * qd, qd)])
            for j, o in enumerate(ops):
                h2b[7 * i + j, pl.ds(a * 8, 8), :] = _pack(o)
            return h2b[jnp.minimum(b, 0) + 7 * i, pl.ds(a * 8, 8), :]

        ffn_in = [functools.partial(norm_piece, r=r, a=a)
                  for r in range(4) for a in range(seg // 16)]
        ffn_in += [functools.partial(lhs_piece, a=a, i=i)
                   for a in range(seg // 16) for i in range(7)]

        def out_cp(b):
            return pltpu.make_async_copy(ob.at[b % 2], out_hbm.at[pl.ds(b * FM, FM), :],
                                         sem_out.at[b % 2])

        def ffn(b, carry):
            @pl.when(b >= 2)
            def _():
                out_cp(b - 2).wait()

            slot = lax.rem(b, 2)
            lhs = []
            for f in range(qf // LANE):
                cols = pl.ds(f * LANE, LANE)
                gu = _out16([_mm(_unpack(h2b[n]), jnp.concatenate(
                    [_unpack(wu[:, c, n, :, cols].reshape(qd // 2, LANE)) for c in range(2)],
                    axis=1)) for n in range(49)])
                act = {}
                for r in range(4):
                    for c in range(2):
                        v = _silu(gu[r, c]) * gu[r, 2 + c]
                        act[r, 2 * c], act[r, 2 * c + 1] = v[:, :LANE], v[:, LANE:]
                lhs.append([o for i in range(7)
                            for o in _ops49(_LHS, i, lambda r, c: act[r, c])])
            prod, late = [], []
            for n in range(49):
                w = wd[:, n].reshape(qf // 2, qd)
                if n in TIES:
                    token = ffn_in[TIES.index(n)](jnp.minimum(b + 1, n_blk - 1))
                    w = jnp.concatenate([_after(w[:8], token, b), w[8:]], axis=0)
                a = [l[n] for l in lhs]
                if n < NSPLIT:
                    ks = (qf - LANE) // 2
                    late.append((a.pop().astype(BF16), _unpack(w[ks:])))
                    w = w[:ks]
                prod.append(_mm(jnp.concatenate(a, axis=1).astype(BF16), _unpack(w)))
                if n == NSPLIT - 1:
                    prod = [_mm(*t) + v for t, v in zip(late, prod)]
            y = _out16(prod)
            for r in range(4):
                yr = jnp.concatenate([y[r, c] for c in range(4)], axis=1)
                ob[slot, pl.ds(r * seg, seg), :] = (
                    resid(b * 4 + r, slice(None)) + mrow(5) * yr).astype(ob.dtype)
            out_cp(b).start()
            return carry

        for piece in ffn_in:
            piece(0)
        lax.fori_loop(0, n_blk, ffn, 0)
        for b in range(n_blk - 2, n_blk):
            out_cp(b).wait()

    pl.run_scoped(main, pltpu.VMEM((n_it // 2, 2, 49, 8, qf), U32),
                  pltpu.VMEM((n_dr, 49, DR // 2, qd), U32))


@functools.partial(jax.jit, static_argnames=("A_seg_len",))
def pallas_adaLN_cond__memory_aug_recurrent_mem_tr__glu_gated_swiglu__prompt_kernel(
    A_x, A_mem0, A_Wq, A_Wk, A_Wv, A_Wo, A_seg_len, B_x, B_w1, B_w3, B_w2, c, w_mod,
):
    del B_x
    B, S, D = A_x.shape
    H, Dh = A_Wq.shape[1], A_Wq.shape[2]
    M = A_mem0.shape[1]
    F = B_w1.shape[1]
    seg = int(A_seg_len)
    n_seg = S // seg
    assert B == 1 and Dh == LANE and S % seg == 0 and S % FM == 0 and F % FC == 0
    hbm = pl.BlockSpec(memory_space=pl.ANY)
    vmem = pl.BlockSpec(memory_space=pltpu.VMEM)
    dma = pltpu.SemaphoreType.DMA
    out = pl.pallas_call(
        _kernel,
        out_shape=jax.ShapeDtypeStruct((S, D), A_x.dtype),
        in_specs=[vmem, vmem] + [hbm] * 9,
        out_specs=hbm,
        scratch_shapes=[
            pltpu.VMEM((n_seg, seg, D), BF16),
            pltpu.VMEM((n_seg, seg, D), BF16),
            pltpu.VMEM((3 * H, D // 2, LANE), U32),
            pltpu.VMEM((3 * H, n_seg * PRE // 2, LANE), U32),
            pltpu.VMEM((H * Dh // 2, D), U32),
            pltpu.VMEM((6, 8, D), F32),
            pltpu.VMEM(((M + seg - PRE) // 2, D), U32),
            pltpu.VMEM((2, 2, 4, 8, F), U32),
            pltpu.VMEM((2, 4, DR, D), U32),
            pltpu.VMEM((4, seg, D), F32),
            pltpu.VMEM((49, seg // 2, D // 4), U32),
            pltpu.VMEM((2, FM, D), A_x.dtype),
            dma((3,)), dma((3,)), dma((NSTG,)), dma((2, 3)), dma((2,)),
        ],
        compiler_params=pltpu.CompilerParams(vmem_limit_bytes=127 * 2**20),
    )(c, A_mem0.reshape(M, D), A_x.reshape(n_seg, seg, D), A_Wq, A_Wk, A_Wv,
      A_Wo.reshape(H * Dh, D), B_w1.reshape(4, D // 4, F), B_w3.reshape(4, D // 4, F),
      B_w2.reshape(4, F // 4, D), w_mod)
    return out.reshape(B, S, D)
```

```python
import functools

import jax
import jax.numpy as jnp
from jax import lax
import jax.experimental.pallas as pl
import jax.experimental.pallas.tpu as pltpu

F32 = jnp.float32
BF16 = jnp.bfloat16
U32 = jnp.uint32
LANE = 128
LOG2E = 1.4426950408889634
HG = 4
HC = 8
RP = 64
VLAG = 4
SPOT = ((1, 1), (2, 1), (3, 3))
DR = 32
UNR = 2
NSPLIT = 6
KCUT = {1: (0, 128, 512)}
TIES = tuple(range(14, 36))
NSTG = 4
PRE = 8
FM = 128
FC = 256


def _mm(a, b):
    return lax.dot_general(a, b, (((1,), (0,)), ((), ())), preferred_element_type=F32)


def _mm_nt(a, b):
    return lax.dot_general(a, b, (((1,), (1,)), ((), ())), preferred_element_type=F32)


def _rnd(v):
    return v.astype(BF16).astype(F32)


def _pack(v):
    return pltpu.bitcast(v.astype(BF16), U32)


def _pack_all(vs):
    n = vs[0].shape[1]
    w = _pack(jnp.concatenate(vs, axis=1))
    return [w[:, i * n:(i + 1) * n] for i in range(len(vs))]


def _unpack(v):
    return pltpu.bitcast(v, BF16)


_LHS = (((1, 0), (1, 3)), ((1, 2), (1, 3)), ((1, 0),), ((1, 3),), ((1, 0), (1, 1)),
        ((1, 2), (-1, 0)), ((1, 1), (-1, 3)))
_RHS = (((1, 0), (1, 3)), ((1, 0),), ((1, 1), (-1, 3)), ((1, 2), (-1, 0)), ((1, 3),),
        ((1, 0), (1, 1)), ((1, 2), (1, 3)))


def _comb(terms, quad):
    v = quad(terms[0][1])
    for sign, q in terms[1:]:
        v = v + quad(q) if sign > 0 else v - quad(q)
    return v


def _ops7(table, quads):
    return [_comb(t, quads.__getitem__) for t in table]


def _ops49(table, i, block):
    return _ops7(table, [
        _comb(table[i], lambda q: block(2 * (q // 2) + r, 2 * (q % 2) + c))
        for r in range(2) for c in range(2)])


def _out4(m):
    return (m[0] + m[3] - m[4] + m[6], m[2] + m[4], m[1] + m[3], m[0] - m[1] + m[2] + m[5])


def _out16(m):
    inner = [_out4(m[7 * i:7 * i + 7]) for i in range(7)]
    return {(2 * (q // 2) + p // 2, 2 * (q % 2) + p % 2): v
            for p in range(4) for q, v in enumerate(_out4([c[p] for c in inner]))}


def _after(v, token, i):
    return jnp.where(i < 0, pltpu.bitcast(token, v.dtype), v)


def _silu(g):
    hg = 0.5 * g
    return hg * jnp.tanh(hg) + hg


def _norm(x):
    m = jnp.mean(x, axis=-1, keepdims=True)
    xc = x - m
    v = jnp.mean(xc * xc, axis=-1, keepdims=True)
    return xc * lax.rsqrt(v + 1e-5)


def _kernel(c_ref, mem0_ref, x_hbm, wq_hbm, wk_hbm, wv_hbm, wo_hbm, w1_hbm, w3_hbm, w2_hbm,
            wmod_hbm, out_hbm,
            xb, ab, wqkv, pre, wo, mod, hin, ru, rd, h2f, h2b, ob,
            sem_x, sem_mod, sem_stg, sem_wo, sem_raw, sem_out):
    n_seg, seg, D = xb.shape
    M = mem0_ref.shape[0]
    L = M + seg
    H = wq_hbm.shape[1]
    F = w1_hbm.shape[2]
    n_grp, n_ct, n_hc = H // HG, D // LANE, H // HC
    n_it = n_seg // UNR
    n_blk, spb = n_seg * seg // FM, FM // seg
    hd, qd, qf = D // 2, D // 4, F // 4
    n_dr = qf // DR
    scale = float(LANE) ** -0.5

    def mrow(j):
        return mod[j, 0:1, :]

    def pre_attn(s):
        xs = xb[s].astype(F32)[0:seg - PRE]
        return _norm(xs) * (1.0 + mrow(1)) + mrow(0)

    x_cp = pltpu.make_async_copy(x_hbm, xb, sem_x.at[1])
    wo_cp = [pltpu.make_async_copy(wo_hbm.at[:, pl.ds(j * LANE, LANE)], wo.at[j].bitcast(BF16),
                                   sem_wo.at[j]) for j in range(n_ct)]

    def raw_cp(kp, slot):
        rows = pl.ds(pl.multiple_of(kp * 16, 16), 16)
        cps = [pltpu.make_async_copy(w.at[:, rows, :], ru.at[slot, j].bitcast(BF16),
                                     sem_raw.at[slot, j])
               for j, w in enumerate((w1_hbm, w3_hbm))]
        rows = pl.ds(pl.multiple_of(jnp.minimum(kp, n_dr // 2 - 1) * 2 * DR, 2 * DR), 2 * DR)
        return cps + [pltpu.make_async_copy(w2_hbm.at[:, rows, :], rd.at[slot].bitcast(BF16),
                                            sem_raw.at[slot, 2])]

    def warmup(xp, wm0, wm1, wm2, stg, tmp, hp):
        hw, hr = HC // 2, n_seg * PRE // 2
        mod_cp = [pltpu.make_async_copy(wmod_hbm.at[:, pl.ds(i * D, w.shape[1])],
                                        w.bitcast(BF16), sem_mod.at[i])
                  for i, w in enumerate((wm0, wm1, wm2))]
        xp_cp = pltpu.make_async_copy(x_hbm.at[:, pl.ds(seg - PRE, PRE), :], xp, sem_x.at[0])

        def stg_cp(t, hc, slot):
            src = (wq_hbm, wk_hbm, wv_hbm)[t]
            return pltpu.make_async_copy(src.at[:, pl.ds(pl.multiple_of(hc * HC, HC), HC), :],
                                         stg.at[slot], sem_stg.at[slot])

        xp_cp.start()
        mod_cp[1].start()
        mod_cp[0].start()
        cv = c_ref[...].astype(F32)
        sc = jnp.broadcast_to(_rnd(cv * jax.nn.sigmoid(cv)), (8, D))
        xp_cp.wait()
        xn = _norm(xp[...].astype(F32).reshape(2 * hr, D))
        mod_cp[1].wait()
        stg_cp(0, 0, 0).start()
        mod[1] = _mm(sc, _unpack(wm1[...]))
        h = xn * (1.0 + mrow(1))
        scaled = _ops7(_LHS, (h[:hr, :hd], h[:hr, hd:], h[hr:, :hd], h[hr:, hd:]))
        mod_cp[0].wait()
        for i in range(1, NSTG):
            stg_cp(i // n_hc, i % n_hc, i).start()
        mod[0] = _mm(sc, _unpack(wm0[...]))
        shift = _ops7(_LHS, (mrow(0)[:, :hd], mrow(0)[:, hd:]) * 2)
        for i in range(7):
            hp[i] = _pack(scaled[i] + shift[i])

        def warm(i, carry):
            slot = lax.rem(i, NSTG)
            stg_cp(0, 0, slot).wait()
            for r in range(D // RP):
                v = stg[slot, pl.ds(r * RP, RP)].reshape(RP * HC, LANE)
                tmp[pl.ds(r * RP * hw, RP * hw), :] = pltpu.bitcast(v, U32)
            ops = []
            for j in range(hw):
                quad = []
                for half in range(2):
                    a = tmp[pl.ds(half * hd * hw + j, hd, stride=hw), :]
                    pair = [pltpu.bitcast(w, F32) for w in (a << 16, a & jnp.uint32(0xFFFF0000))]
                    for k, w in enumerate(_pack_all(pair)):
                        wqkv[i * HC + 2 * j + k, pl.ds(half * hd // 2, hd // 2), :] = w
                    quad += pair
                ops.append(_ops7(_RHS, quad))
            prod = {}
            for n in (1, 5, 0, 2, 3, 4, 6):
                w = jnp.concatenate([o[n] for o in ops], axis=1)
                cuts = KCUT.get(n, (0, hd))
                for k0, k1 in zip(cuts, cuts[1:]):
                    v = _mm(_unpack(hp[n, :, k0:k1]), w[k0:k1].astype(BF16))
                    prod[n] = v + prod[n] if k0 else v
            for n, cq in enumerate(_out4(prod)):
                cq = _pack(cq)
                for j in range(hw):
                    pre[i * HC + 2 * j + n % 2, pl.ds((n // 2) * hr // 2, hr // 2), :] = (
                        cq[:, j * LANE:(j + 1) * LANE])
            nx = i + NSTG
            for t in range(3):
                @pl.when(lax.div(nx, n_hc) == t)
                def _(t=t):
                    stg_cp(t, lax.rem(nx, n_hc), slot).start()

            for at, cps in ((0, [x_cp]), (2, wo_cp[:n_ct // 2]), (4, wo_cp[n_ct // 2:]),
                            (3 * n_hc - NSTG - 1, [mod_cp[2]] + raw_cp(0, 0))):
                @pl.when(i == at)
                def _(cps=cps):
                    for cp in cps:
                        cp.start()

            return carry

        lax.fori_loop(0, 3 * n_hc, warm, 0)
        mod_cp[2].wait()
        x_cp.wait()
        hin[...] = _pack(jnp.concatenate([mem0_ref[...].astype(F32), pre_attn(0)], axis=0))
        rest = _mm(sc, _unpack(wm2[...]))
        for j in range(4):
            mod[2 + j] = rest[:, j * D:(j + 1) * D]

    pl.run_scoped(warmup,
                  pltpu.VMEM((n_seg, PRE, D), BF16),
                  pltpu.VMEM((hd, D), U32),
                  pltpu.VMEM((hd, D), U32),
                  pltpu.VMEM((hd, 4 * D), U32),
                  pltpu.VMEM((NSTG, D, HC, LANE), BF16),
                  pltpu.VMEM((D * HC // 2 + 8, LANE), U32),
                  pltpu.VMEM((7, n_seg * PRE // 4, hd), U32))
    for cp in wo_cp:
        cp.wait()

    def step(k, u, side):
        s = k * UNR + u
        h = _unpack(hin[...])
        ri = lax.broadcasted_iota(jnp.int32, (L, L), 0)
        ci = lax.broadcasted_iota(jnp.int32, (L, L), 1)
        mask = (ri < M) | (ri >= ci)
        prow = pl.ds(pl.multiple_of(k * PRE, PRE), PRE)
        qkv, prob, att = {}, {}, {}

        def proj(g, ts):
            heads = [(t, g * HG + j) for t in ts for j in range(HG)]
            r = _mm(h, jnp.concatenate([_unpack(wqkv[t * H + n]) for t, n in heads], axis=1))
            for i, (t, n) in enumerate(heads):
                early = pre[t * H + n, prow, :]
                if (t, n) in side:
                    early = side[t, n](early)
                early = _unpack(early).astype(F32)[u * PRE:(u + 1) * PRE]
                qkv[t, n] = jnp.concatenate([r[:, i * LANE:(i + 1) * LANE], early], axis=0)

        def scores(g):
            for n in range(g * HG, (g + 1) * HG):
                sv = _mm_nt(_rnd(qkv[0, n]), qkv[1, n].astype(BF16)) * (scale * LOG2E)
                sv = jnp.where(mask, sv, -1e9 * LOG2E)
                e = jnp.exp2(sv - jnp.max(sv, axis=-1, keepdims=True))
                den = jnp.sum(e, axis=-1, keepdims=True)
                inv = pl.reciprocal(den, approx=True)
                prob[n] = _rnd(e * (inv * (2.0 - den * inv)))

        def values(g):
            for n in range(g * HG, (g + 1) * HG):
                att[n] = _rnd(_mm(prob[n], qkv[2, n].astype(BF16)))

        nxt = pre_attn(jnp.minimum(s + 1, n_seg - 1))
        for g in range(n_grp):
            proj(g, (0, 1))
            if g >= 1:
                scores(g - 1)
        for g in range(n_grp):
            proj(g, (2,))
            if g == 0:
                scores(n_grp - 1)
            if g >= VLAG:
                values(g - VLAG)
        for g in range(n_grp - VLAG, n_grp):
            values(g)
        cols = []
        for j in range(n_ct):
            w, per = wo[j], H // n_ct
            rows = w.shape[0] // per
            parts = []
            for i in range(per):
                blk = w[i * rows:(i + 1) * rows]
                if (3, j * per + i) in side:
                    blk = jnp.concatenate([side[3, j * per + i](blk[:8]), blk[8:]], axis=0)
                parts.append(blk)
            cols.append(_unpack(jnp.concatenate(parts, axis=0)))
        acc = _mm(jnp.concatenate([att[n] for n in range(H)], axis=1),
                  jnp.concatenate(cols, axis=1))
        hin[...] = _pack(jnp.concatenate([acc[0:M], nxt], axis=0))
        ab[s] = acc[M:L].astype(BF16)

    def main(wu, wd):
        def steps(k, carry):
            kp, odd = lax.div(k, 2), lax.rem(k, 2)
            slot = lax.rem(kp, 2)
            kd = jnp.minimum(kp, n_dr // 2 - 1) * 2 + odd

            @pl.when(odd == 0)
            def _():
                for cp in raw_cp(kp, slot):
                    cp.wait()

            def up_piece(t, i, v):
                cols = pl.ds(t * LANE, LANE)
                ops = _ops49(_RHS, i, lambda r, c: _unpack(ru[
                    slot, c // 2, r, :,
                    pl.ds(pl.multiple_of((2 * (c % 2) + odd) * qf + t * LANE, LANE), LANE)
                ]).astype(F32))
                for j, o in enumerate(_pack_all(ops)):
                    wu[kp, odd, 7 * i + j, :, cols] = o
                return _after(v, wu[kp, jnp.minimum(odd, 1), 7 * i, :, cols], k)

            def down_piece(a, t, i, v):
                rows, cols = pl.ds(a * 8, 8), pl.ds(t * LANE, LANE)
                src = pl.ds(pl.multiple_of(odd * (DR // 2) + a * 8, 8), 8)
                ops = _ops49(_RHS, i, lambda r, c: _unpack(
                    rd[slot, r, src, pl.ds(c * qd + t * LANE, LANE)]).astype(F32))
                for j, o in enumerate(_pack_all(ops)):
                    wd[kd, 7 * i + j, rows, cols] = o
                return _after(v, wd[jnp.minimum(kd, n_it), 7 * i, rows, cols], k)

            pieces = [functools.partial(up_piece, t, i)
                      for t in range(qf // LANE) for i in range(7)]
            pieces += [functools.partial(down_piece, a, t, i) for a in range(DR // 16)
                       for t in range(qd // LANE) for i in range(7)]
            spots = [(u, t, n) for u in range(UNR) for t, m in SPOT for n in range(H) if n % 4 < m]
            assert len(pieces) <= len(spots)
            for u in range(UNR):
                step(k, u, {sp[1:]: f for sp, f in zip(spots, pieces) if sp[0] == u})

            @pl.when((odd == 0) & (k + 2 < n_it))
            def _():
                for cp in raw_cp(kp + 1, 1 - slot):
                    cp.start()

            return carry

        lax.fori_loop(0, n_it, steps, 0)

        def resid(sg, rows):
            return xb[sg, rows, :].astype(F32) + mrow(2) * ab[sg, rows, :].astype(F32)

        def norm_piece(b, r, a):
            rows = pl.ds(a * 16, 16)
            h2f[r, rows, :] = _norm(resid(b * 4 + r, rows)) * (1.0 + mrow(4)) + mrow(3)
            return h2f[jnp.minimum(b, 0) + r, pl.ds(a * 16, 8), 0:qd]

        def lhs_piece(b, a, i):
            ops = _ops49(_LHS, i, lambda r, c: h2f[r, pl.ds(a * 16, 16), pl.ds(c * qd, qd)])
            for j, o in enumerate(ops):
                h2b[7 * i + j, pl.ds(a * 8, 8), :] = _pack(o)
            return h2b[jnp.minimum(b, 0) + 7 * i, pl.ds(a * 8, 8), :]

        ffn_in = [functools.partial(norm_piece, r=r, a=a)
                  for r in range(4) for a in range(seg // 16)]
        ffn_in += [functools.partial(lhs_piece, a=a, i=i)
                   for a in range(seg // 16) for i in range(7)]

        def out_cp(b):
            return pltpu.make_async_copy(ob.at[b % 2], out_hbm.at[pl.ds(b * FM, FM), :],
                                         sem_out.at[b % 2])

        def ffn(b, carry):
            @pl.when(b >= 2)
            def _():
                out_cp(b - 2).wait()

            slot = lax.rem(b, 2)
            lhs = []
            for f in range(qf // LANE):
                cols = pl.ds(f * LANE, LANE)
                gu = _out16([_mm(_unpack(h2b[n]), jnp.concatenate(
                    [_unpack(wu[:, c, n, :, cols].reshape(qd // 2, LANE)) for c in range(2)],
                    axis=1)) for n in range(49)])
                act = {}
                for r in range(4):
                    for c in range(2):
                        v = _silu(gu[r, c]) * gu[r, 2 + c]
                        act[r, 2 * c], act[r, 2 * c + 1] = v[:, :LANE], v[:, LANE:]
                lhs.append([o for i in range(7)
                            for o in _ops49(_LHS, i, lambda r, c: act[r, c])])
            prod, late = [], []
            for n in range(49):
                w = wd[:, n].reshape(qf // 2, qd)
                if n in TIES:
                    token = ffn_in[TIES.index(n)](jnp.minimum(b + 1, n_blk - 1))
                    w = jnp.concatenate([_after(w[:8], token, b), w[8:]], axis=0)
                a = [l[n] for l in lhs]
                if n < NSPLIT:
                    ks = (qf - LANE) // 2
                    late.append((a.pop().astype(BF16), _unpack(w[ks:])))
                    w = w[:ks]
                prod.append(_mm(jnp.concatenate(a, axis=1).astype(BF16), _unpack(w)))
                if n == NSPLIT - 1:
                    prod = [_mm(*t) + v for t, v in zip(late, prod)]
            y = _out16(prod)
            for r in range(4):
                yr = jnp.concatenate([y[r, c] for c in range(4)], axis=1)
                ob[slot, pl.ds(r * seg, seg), :] = (
                    resid(b * 4 + r, slice(None)) + mrow(5) * yr).astype(ob.dtype)
            out_cp(b).start()
            return carry

        for piece in ffn_in:
            piece(0)
        lax.fori_loop(0, n_blk, ffn, 0)
        for b in range(n_blk - 2, n_blk):
            out_cp(b).wait()

    pl.run_scoped(main, pltpu.VMEM((n_it // 2, 2, 49, 8, qf), U32),
                  pltpu.VMEM((n_dr, 49, DR // 2, qd), U32))


@functools.partial(jax.jit, static_argnames=("A_seg_len",))
def pallas_adaLN_cond__memory_aug_recurrent_mem_tr__glu_gated_swiglu__prompt_kernel(
    A_x, A_mem0, A_Wq, A_Wk, A_Wv, A_Wo, A_seg_len, B_x, B_w1, B_w3, B_w2, c, w_mod,
):
    del B_x
    B, S, D = A_x.shape
    H, Dh = A_Wq.shape[1], A_Wq.shape[2]
    M = A_mem0.shape[1]
    F = B_w1.shape[1]
    seg = int(A_seg_len)
    n_seg = S // seg
    assert B == 1 and Dh == LANE and S % seg == 0 and S % FM == 0 and F % FC == 0
    hbm = pl.BlockSpec(memory_space=pl.ANY)
    vmem = pl.BlockSpec(memory_space=pltpu.VMEM)
    dma = pltpu.SemaphoreType.DMA
    out = pl.pallas_call(
        _kernel,
        out_shape=jax.ShapeDtypeStruct((S, D), A_x.dtype),
        in_specs=[vmem, vmem] + [hbm] * 9,
        out_specs=hbm,
        scratch_shapes=[
            pltpu.VMEM((n_seg, seg, D), BF16),
            pltpu.VMEM((n_seg, seg, D), BF16),
            pltpu.VMEM((3 * H, D // 2, LANE), U32),
            pltpu.VMEM((3 * H, n_seg * PRE // 2, LANE), U32),
            pltpu.VMEM((D // LANE, H * Dh // 2, LANE), U32),
            pltpu.VMEM((6, 8, D), F32),
            pltpu.VMEM(((M + seg - PRE) // 2, D), U32),
            pltpu.VMEM((2, 2, 4, 8, F), U32),
            pltpu.VMEM((2, 4, DR, D), U32),
            pltpu.VMEM((4, seg, D), F32),
            pltpu.VMEM((49, seg // 2, D // 4), U32),
            pltpu.VMEM((2, FM, D), A_x.dtype),
            dma((2,)), dma((3,)), dma((NSTG,)), dma((D // LANE,)), dma((2, 3)), dma((2,)),
        ],
        compiler_params=pltpu.CompilerParams(vmem_limit_bytes=127 * 2**20),
    )(c, A_mem0.reshape(M, D), A_x.reshape(n_seg, seg, D), A_Wq, A_Wk, A_Wv,
      A_Wo.reshape(H * Dh, D), B_w1.reshape(4, D // 4, F), B_w3.reshape(4, D // 4, F),
      B_w2.reshape(4, F // 4, D), w_mod)
    return out.reshape(B, S, D)
```

```python
import functools

import jax
import jax.numpy as jnp
from jax import lax
import jax.experimental.pallas as pl
import jax.experimental.pallas.tpu as pltpu

F32 = jnp.float32
BF16 = jnp.bfloat16
U32 = jnp.uint32
LANE = 128
LOG2E = 1.4426950408889634
HG = 4
HC = 8
RP = 64
VLAG = 4
SPOT = ((1, 1), (2, 1), (3, 3))
DR = 32
UNR = 2
NSPLIT = 6
KCUT = {1: (0, 128, 512)}
TIES = tuple(range(14, 36))
NSTG = 4
PRE = 8
FM = 128
FC = 256


def _mm(a, b):
    return lax.dot_general(a, b, (((1,), (0,)), ((), ())), preferred_element_type=F32)


def _mm_nt(a, b):
    return lax.dot_general(a, b, (((1,), (1,)), ((), ())), preferred_element_type=F32)


def _rnd(v):
    return v.astype(BF16).astype(F32)


def _pack(v):
    return pltpu.bitcast(v.astype(BF16), U32)


def _pack_all(vs):
    n = vs[0].shape[1]
    w = _pack(jnp.concatenate(vs, axis=1))
    return [w[:, i * n:(i + 1) * n] for i in range(len(vs))]


def _unpack(v):
    return pltpu.bitcast(v, BF16)


_LHS = (((1, 0), (1, 3)), ((1, 2), (1, 3)), ((1, 0),), ((1, 3),), ((1, 0), (1, 1)),
        ((1, 2), (-1, 0)), ((1, 1), (-1, 3)))
_RHS = (((1, 0), (1, 3)), ((1, 0),), ((1, 1), (-1, 3)), ((1, 2), (-1, 0)), ((1, 3),),
        ((1, 0), (1, 1)), ((1, 2), (1, 3)))


def _comb(terms, quad):
    v = quad(terms[0][1])
    for sign, q in terms[1:]:
        v = v + quad(q) if sign > 0 else v - quad(q)
    return v


def _ops7(table, quads):
    return [_comb(t, quads.__getitem__) for t in table]


def _ops49(table, i, block):
    return _ops7(table, [
        _comb(table[i], lambda q: block(2 * (q // 2) + r, 2 * (q % 2) + c))
        for r in range(2) for c in range(2)])


def _out4(m):
    return (m[0] + m[3] - m[4] + m[6], m[2] + m[4], m[1] + m[3], m[0] - m[1] + m[2] + m[5])


def _out16(m):
    inner = [_out4(m[7 * i:7 * i + 7]) for i in range(7)]
    return {(2 * (q // 2) + p // 2, 2 * (q % 2) + p % 2): v
            for p in range(4) for q, v in enumerate(_out4([c[p] for c in inner]))}


def _after(v, token, i):
    return jnp.where(i < 0, pltpu.bitcast(token, v.dtype), v)


def _silu(g):
    hg = 0.5 * g
    return hg * jnp.tanh(hg) + hg


def _norm(x):
    m = jnp.mean(x, axis=-1, keepdims=True)
    xc = x - m
    v = jnp.mean(xc * xc, axis=-1, keepdims=True)
    return xc * lax.rsqrt(v + 1e-5)


def _kernel(c_ref, mem0_ref, x_hbm, wq_hbm, wk_hbm, wv_hbm, wo_hbm, w1_hbm, w3_hbm, w2_hbm,
            wmod_hbm, out_hbm,
            xb, ab, wqkv, pre, wo, mod, hin, ru, rd, h2f, h2b, ob,
            sem_x, sem_mod, sem_stg, sem_wo, sem_raw, sem_out):
    n_seg, seg, D = xb.shape
    M = mem0_ref.shape[0]
    L = M + seg
    H = wq_hbm.shape[1]
    F = w1_hbm.shape[2]
    n_grp, n_ct, n_hc = H // HG, D // LANE, H // HC
    n_it = n_seg // UNR
    n_blk, spb = n_seg * seg // FM, FM // seg
    hd, qd, qf = D // 2, D // 4, F // 4
    n_dr = qf // DR
    scale = float(LANE) ** -0.5

    def mrow(j):
        return mod[j, 0:1, :]

    def pre_attn(s):
        xs = xb[s].astype(F32)[0:seg - PRE]
        return _norm(xs) * (1.0 + mrow(1)) + mrow(0)

    x_cp = pltpu.make_async_copy(x_hbm, xb, sem_x.at[1])
    wo_cp = [pltpu.make_async_copy(wo_hbm.at[:, pl.ds(j * LANE, LANE)], wo.at[j],
                                   sem_wo.at[j]) for j in range(n_ct)]

    def raw_cp(kp, slot):
        rows = pl.ds(pl.multiple_of(kp * 16, 16), 16)
        cps = [pltpu.make_async_copy(w.at[:, rows, :], ru.at[slot, j],
                                     sem_raw.at[slot, j])
               for j, w in enumerate((w1_hbm, w3_hbm))]
        rows = pl.ds(pl.multiple_of(jnp.minimum(kp, n_dr // 2 - 1) * 2 * DR, 2 * DR), 2 * DR)
        return cps + [pltpu.make_async_copy(w2_hbm.at[:, rows, :], rd.at[slot],
                                            sem_raw.at[slot, 2])]

    def warmup(xp, wm0, wm1, wm2, stg, tmp, hp):
        hw, hr = HC // 2, n_seg * PRE // 2
        mod_cp = [pltpu.make_async_copy(wmod_hbm.at[:, pl.ds(i * D, w.shape[1])],
                                        w, sem_mod.at[i])
                  for i, w in enumerate((wm0, wm1, wm2))]
        xp_cp = pltpu.make_async_copy(x_hbm.at[:, pl.ds(seg - PRE, PRE), :], xp, sem_x.at[0])

        def stg_cp(t, hc, slot):
            src = (wq_hbm, wk_hbm, wv_hbm)[t]
            return pltpu.make_async_copy(src.at[:, pl.ds(pl.multiple_of(hc * HC, HC), HC), :],
                                         stg.at[slot], sem_stg.at[slot])

        xp_cp.start()
        mod_cp[1].start()
        mod_cp[0].start()
        cv = c_ref[...].astype(F32)
        sc = jnp.broadcast_to(_rnd(cv * jax.nn.sigmoid(cv)), (8, D))
        xp_cp.wait()
        xn = _norm(xp[...].astype(F32).reshape(2 * hr, D))
        mod_cp[1].wait()
        stg_cp(0, 0, 0).start()
        mod[1] = _mm(sc, wm1[...])
        h = xn * (1.0 + mrow(1))
        scaled = _ops7(_LHS, (h[:hr, :hd], h[:hr, hd:], h[hr:, :hd], h[hr:, hd:]))
        mod_cp[0].wait()
        for i in range(1, NSTG):
            stg_cp(i // n_hc, i % n_hc, i).start()
        mod[0] = _mm(sc, wm0[...])
        shift = _ops7(_LHS, (mrow(0)[:, :hd], mrow(0)[:, hd:]) * 2)
        for i in range(7):
            hp[i] = _pack(scaled[i] + shift[i])

        def warm(i, carry):
            slot = lax.rem(i, NSTG)
            stg_cp(0, 0, slot).wait()
            for r in range(D // RP):
                v = stg[slot, pl.ds(r * RP, RP)].reshape(RP * HC, LANE)
                tmp[pl.ds(r * RP * hw, RP * hw), :] = pltpu.bitcast(v, U32)
            ops = []
            for j in range(hw):
                quad = []
                for half in range(2):
                    a = tmp[pl.ds(half * hd * hw + j, hd, stride=hw), :]
                    pair = [pltpu.bitcast(w, F32) for w in (a << 16, a & jnp.uint32(0xFFFF0000))]
                    for k, w in enumerate(_pack_all(pair)):
                        wqkv[i * HC + 2 * j + k, pl.ds(half * hd // 2, hd // 2), :] = w
                    quad += pair
                ops.append(_ops7(_RHS, quad))
            prod = {}
            for n in (1, 5, 0, 2, 3, 4, 6):
                w = jnp.concatenate([o[n] for o in ops], axis=1)
                cuts = KCUT.get(n, (0, hd))
                for k0, k1 in zip(cuts, cuts[1:]):
                    v = _mm(_unpack(hp[n, :, k0:k1]), w[k0:k1].astype(BF16))
                    prod[n] = v + prod[n] if k0 else v
            for n, cq in enumerate(_out4(prod)):
                cq = _pack(cq)
                for j in range(hw):
                    pre[i * HC + 2 * j + n % 2, pl.ds((n // 2) * hr // 2, hr // 2), :] = (
                        cq[:, j * LANE:(j + 1) * LANE])
            nx = i + NSTG
            for t in range(3):
                @pl.when(lax.div(nx, n_hc) == t)
                def _(t=t):
                    stg_cp(t, lax.rem(nx, n_hc), slot).start()

            for at, cps in ((0, [x_cp]), (2, wo_cp[:n_ct // 2]), (4, wo_cp[n_ct // 2:]),
                            (3 * n_hc - NSTG - 1, [mod_cp[2]] + raw_cp(0, 0))):
                @pl.when(i == at)
                def _(cps=cps):
                    for cp in cps:
                        cp.start()

            return carry

        lax.fori_loop(0, 3 * n_hc, warm, 0)
        mod_cp[2].wait()
        x_cp.wait()
        hin[...] = _pack(jnp.concatenate([mem0_ref[...].astype(F32), pre_attn(0)], axis=0))
        rest = _mm(sc, wm2[...])
        for j in range(4):
            mod[2 + j] = rest[:, j * D:(j + 1) * D]

    pl.run_scoped(warmup,
                  pltpu.VMEM((n_seg, PRE, D), BF16),
                  pltpu.VMEM((D, D), BF16),
                  pltpu.VMEM((D, D), BF16),
                  pltpu.VMEM((D, 4 * D), BF16),
                  pltpu.VMEM((NSTG, D, HC, LANE), BF16),
                  pltpu.VMEM((D * HC // 2 + 8, LANE), U32),
                  pltpu.VMEM((7, n_seg * PRE // 4, hd), U32))
    for cp in wo_cp:
        cp.wait()

    def step(k, u, side):
        s = k * UNR + u
        h = _unpack(hin[...])
        ri = lax.broadcasted_iota(jnp.int32, (L, L), 0)
        ci = lax.broadcasted_iota(jnp.int32, (L, L), 1)
        mask = (ri < M) | (ri >= ci)
        prow = pl.ds(pl.multiple_of(k * PRE, PRE), PRE)
        qkv, prob, att = {}, {}, {}

        def proj(g, ts):
            heads = [(t, g * HG + j) for t in ts for j in range(HG)]
            r = _mm(h, jnp.concatenate([_unpack(wqkv[t * H + n]) for t, n in heads], axis=1))
            for i, (t, n) in enumerate(heads):
                early = pre[t * H + n, prow, :]
                if (t, n) in side:
                    early = side[t, n](early)
                early = _unpack(early).astype(F32)[u * PRE:(u + 1) * PRE]
                qkv[t, n] = jnp.concatenate([r[:, i * LANE:(i + 1) * LANE], early], axis=0)

        def scores(g):
            for n in range(g * HG, (g + 1) * HG):
                sv = _mm_nt(_rnd(qkv[0, n]), qkv[1, n].astype(BF16)) * (scale * LOG2E)
                sv = jnp.where(mask, sv, -1e9 * LOG2E)
                e = jnp.exp2(sv - jnp.max(sv, axis=-1, keepdims=True))
                den = jnp.sum(e, axis=-1, keepdims=True)
                inv = pl.reciprocal(den, approx=True)
                prob[n] = _rnd(e * (inv * (2.0 - den * inv)))

        def values(g):
            for n in range(g * HG, (g + 1) * HG):
                att[n] = _rnd(_mm(prob[n], qkv[2, n].astype(BF16)))

        nxt = pre_attn(jnp.minimum(s + 1, n_seg - 1))
        for g in range(n_grp):
            proj(g, (0, 1))
            if g >= 1:
                scores(g - 1)
        for g in range(n_grp):
            proj(g, (2,))
            if g == 0:
                scores(n_grp - 1)
            if g >= VLAG:
                values(g - VLAG)
        for g in range(n_grp - VLAG, n_grp):
            values(g)
        cols = []
        for j in range(n_ct):
            w, per = pltpu.bitcast(wo[j], U32), H // n_ct
            rows = w.shape[0] // per
            parts = []
            for i in range(per):
                blk = w[i * rows:(i + 1) * rows]
                if (3, j * per + i) in side:
                    blk = jnp.concatenate([side[3, j * per + i](blk[:8]), blk[8:]], axis=0)
                parts.append(blk)
            cols.append(_unpack(jnp.concatenate(parts, axis=0)))
        acc = _mm(jnp.concatenate([att[n] for n in range(H)], axis=1),
                  jnp.concatenate(cols, axis=1))
        hin[...] = _pack(jnp.concatenate([acc[0:M], nxt], axis=0))
        ab[s] = acc[M:L].astype(BF16)

    def main(wu, wd):
        def steps(k, carry):
            kp, odd = lax.div(k, 2), lax.rem(k, 2)
            slot = lax.rem(kp, 2)
            kd = jnp.minimum(kp, n_dr // 2 - 1) * 2 + odd

            @pl.when(odd == 0)
            def _():
                for cp in raw_cp(kp, slot):
                    cp.wait()

            def up_piece(t, i, v):
                cols = pl.ds(t * LANE, LANE)
                ops = _ops49(_RHS, i, lambda r, c: ru[
                    slot, c // 2, r, :,
                    pl.ds(pl.multiple_of((2 * (c % 2) + odd) * qf + t * LANE, LANE), LANE)
                ].astype(F32))
                for j, o in enumerate(_pack_all(ops)):
                    wu[kp, odd, 7 * i + j, :, cols] = o
                return _after(v, wu[kp, jnp.minimum(odd, 1), 7 * i, :, cols], k)

            def down_piece(a, t, i, v):
                rows, cols = pl.ds(a * 8, 8), pl.ds(t * LANE, LANE)
                src = pl.ds(pl.multiple_of(odd * DR + a * 16, 16), 16)
                ops = _ops49(_RHS, i, lambda r, c: rd[
                    slot, r, src, pl.ds(c * qd + t * LANE, LANE)].astype(F32))
                for j, o in enumerate(_pack_all(ops)):
                    wd[kd, 7 * i + j, rows, cols] = o
                return _after(v, wd[jnp.minimum(kd, n_it), 7 * i, rows, cols], k)

            pieces = [functools.partial(up_piece, t, i)
                      for t in range(qf // LANE) for i in range(7)]
            pieces += [functools.partial(down_piece, a, t, i) for a in range(DR // 16)
                       for t in range(qd // LANE) for i in range(7)]
            spots = [(u, t, n) for u in range(UNR) for t, m in SPOT for n in range(H) if n % 4 < m]
            assert len(pieces) <= len(spots)
            for u in range(UNR):
                step(k, u, {sp[1:]: f for sp, f in zip(spots, pieces) if sp[0] == u})

            @pl.when((odd == 0) & (k + 2 < n_it))
            def _():
                for cp in raw_cp(kp + 1, 1 - slot):
                    cp.start()

            return carry

        lax.fori_loop(0, n_it, steps, 0)

        def resid(sg, rows):
            return xb[sg, rows, :].astype(F32) + mrow(2) * ab[sg, rows, :].astype(F32)

        def norm_piece(b, r, a):
            rows = pl.ds(a * 16, 16)
            h2f[r, rows, :] = _norm(resid(b * 4 + r, rows)) * (1.0 + mrow(4)) + mrow(3)
            return h2f[jnp.minimum(b, 0) + r, pl.ds(a * 16, 8), 0:qd]

        def lhs_piece(b, a, i):
            ops = _ops49(_LHS, i, lambda r, c: h2f[r, pl.ds(a * 16, 16), pl.ds(c * qd, qd)])
            for j, o in enumerate(ops):
                h2b[7 * i + j, pl.ds(a * 8, 8), :] = _pack(o)
            return h2b[jnp.minimum(b, 0) + 7 * i, pl.ds(a * 8, 8), :]

        ffn_in = [functools.partial(norm_piece, r=r, a=a)
                  for r in range(4) for a in range(seg // 16)]
        ffn_in += [functools.partial(lhs_piece, a=a, i=i)
                   for a in range(seg // 16) for i in range(7)]

        def out_cp(b):
            return pltpu.make_async_copy(ob.at[b % 2], out_hbm.at[pl.ds(b * FM, FM), :],
                                         sem_out.at[b % 2])

        def ffn(b, carry):
            @pl.when(b >= 2)
            def _():
                out_cp(b - 2).wait()

            slot = lax.rem(b, 2)
            lhs = []
            for f in range(qf // LANE):
                cols = pl.ds(f * LANE, LANE)
                gu = _out16([_mm(_unpack(h2b[n]), jnp.concatenate(
                    [_unpack(wu[:, c, n, :, cols].reshape(qd // 2, LANE)) for c in range(2)],
                    axis=1)) for n in range(49)])
                act = {}
                for r in range(4):
                    for c in range(2):
                        v = _silu(gu[r, c]) * gu[r, 2 + c]
                        act[r, 2 * c], act[r, 2 * c + 1] = v[:, :LANE], v[:, LANE:]
                lhs.append([o for i in range(7)
                            for o in _ops49(_LHS, i, lambda r, c: act[r, c])])
            prod, late = [], []
            for n in range(49):
                w = wd[:, n].reshape(qf // 2, qd)
                if n in TIES:
                    token = ffn_in[TIES.index(n)](jnp.minimum(b + 1, n_blk - 1))
                    w = jnp.concatenate([_after(w[:8], token, b), w[8:]], axis=0)
                a = [l[n] for l in lhs]
                if n < NSPLIT:
                    ks = (qf - LANE) // 2
                    late.append((a.pop().astype(BF16), _unpack(w[ks:])))
                    w = w[:ks]
                prod.append(_mm(jnp.concatenate(a, axis=1).astype(BF16), _unpack(w)))
                if n == NSPLIT - 1:
                    prod = [_mm(*t) + v for t, v in zip(late, prod)]
            y = _out16(prod)
            for r in range(4):
                yr = jnp.concatenate([y[r, c] for c in range(4)], axis=1)
                ob[slot, pl.ds(r * seg, seg), :] = (
                    resid(b * 4 + r, slice(None)) + mrow(5) * yr).astype(ob.dtype)
            out_cp(b).start()
            return carry

        for piece in ffn_in:
            piece(0)
        lax.fori_loop(0, n_blk, ffn, 0)
        for b in range(n_blk - 2, n_blk):
            out_cp(b).wait()

    pl.run_scoped(main, pltpu.VMEM((n_it // 2, 2, 49, 8, qf), U32),
                  pltpu.VMEM((n_dr, 49, DR // 2, qd), U32))


@functools.partial(jax.jit, static_argnames=("A_seg_len",))
def pallas_adaLN_cond__memory_aug_recurrent_mem_tr__glu_gated_swiglu__prompt_kernel(
    A_x, A_mem0, A_Wq, A_Wk, A_Wv, A_Wo, A_seg_len, B_x, B_w1, B_w3, B_w2, c, w_mod,
):
    del B_x
    B, S, D = A_x.shape
    H, Dh = A_Wq.shape[1], A_Wq.shape[2]
    M = A_mem0.shape[1]
    F = B_w1.shape[1]
    seg = int(A_seg_len)
    n_seg = S // seg
    assert B == 1 and Dh == LANE and S % seg == 0 and S % FM == 0 and F % FC == 0
    hbm = pl.BlockSpec(memory_space=pl.ANY)
    vmem = pl.BlockSpec(memory_space=pltpu.VMEM)
    dma = pltpu.SemaphoreType.DMA
    out = pl.pallas_call(
        _kernel,
        out_shape=jax.ShapeDtypeStruct((S, D), A_x.dtype),
        in_specs=[vmem, vmem] + [hbm] * 9,
        out_specs=hbm,
        scratch_shapes=[
            pltpu.VMEM((n_seg, seg, D), BF16),
            pltpu.VMEM((n_seg, seg, D), BF16),
            pltpu.VMEM((3 * H, D // 2, LANE), U32),
            pltpu.VMEM((3 * H, n_seg * PRE // 2, LANE), U32),
            pltpu.VMEM((D // LANE, H * Dh, LANE), BF16),
            pltpu.VMEM((6, 8, D), F32),
            pltpu.VMEM(((M + seg - PRE) // 2, D), U32),
            pltpu.VMEM((2, 2, 4, 16, F), BF16),
            pltpu.VMEM((2, 4, 2 * DR, D), BF16),
            pltpu.VMEM((4, seg, D), F32),
            pltpu.VMEM((49, seg // 2, D // 4), U32),
            pltpu.VMEM((2, FM, D), A_x.dtype),
            dma((2,)), dma((3,)), dma((NSTG,)), dma((D // LANE,)), dma((2, 3)), dma((2,)),
        ],
        compiler_params=pltpu.CompilerParams(vmem_limit_bytes=127 * 2**20),
    )(c, A_mem0.reshape(M, D), A_x.reshape(n_seg, seg, D), A_Wq, A_Wk, A_Wv,
      A_Wo.reshape(H * Dh, D), B_w1.reshape(4, D // 4, F), B_w3.reshape(4, D // 4, F),
      B_w2.reshape(4, F // 4, D), w_mod)
    return out.reshape(B, S, D)
```

```python
import functools

import jax
import jax.numpy as jnp
from jax import lax
import jax.experimental.pallas as pl
import jax.experimental.pallas.tpu as pltpu

F32 = jnp.float32
BF16 = jnp.bfloat16
U32 = jnp.uint32
LANE = 128
LOG2E = 1.4426950408889634
HG = 4
HC = 8
RP = 64
VLAG = 4
SPOT = ((1, 1), (2, 1), (3, 3))
DR = 32
UNR = 2
NSPLIT = 6
KCUT = {1: (0, 128, 512)}
TIES = tuple(range(14, 36))
MSP = (3, 3)
NSTG = 4
PRE = 8
FM = 128
FC = 256


def _mm(a, b):
    return lax.dot_general(a, b, (((1,), (0,)), ((), ())), preferred_element_type=F32)


def _mm_nt(a, b):
    return lax.dot_general(a, b, (((1,), (1,)), ((), ())), preferred_element_type=F32)


def _rnd(v):
    return v.astype(BF16).astype(F32)


def _pack(v):
    return pltpu.bitcast(v.astype(BF16), U32)


def _pack_all(vs):
    n = vs[0].shape[1]
    w = _pack(jnp.concatenate(vs, axis=1))
    return [w[:, i * n:(i + 1) * n] for i in range(len(vs))]


def _unpack(v):
    return pltpu.bitcast(v, BF16)


_LHS = (((1, 0), (1, 3)), ((1, 2), (1, 3)), ((1, 0),), ((1, 3),), ((1, 0), (1, 1)),
        ((1, 2), (-1, 0)), ((1, 1), (-1, 3)))
_RHS = (((1, 0), (1, 3)), ((1, 0),), ((1, 1), (-1, 3)), ((1, 2), (-1, 0)), ((1, 3),),
        ((1, 0), (1, 1)), ((1, 2), (1, 3)))


def _comb(terms, quad):
    v = quad(terms[0][1])
    for sign, q in terms[1:]:
        v = v + quad(q) if sign > 0 else v - quad(q)
    return v


def _ops7(table, quads):
    return [_comb(t, quads.__getitem__) for t in table]


def _ops49(table, i, block):
    return _ops7(table, [
        _comb(table[i], lambda q: block(2 * (q // 2) + r, 2 * (q % 2) + c))
        for r in range(2) for c in range(2)])


def _out4(m):
    return (m[0] + m[3] - m[4] + m[6], m[2] + m[4], m[1] + m[3], m[0] - m[1] + m[2] + m[5])


def _out16(m):
    inner = [_out4(m[7 * i:7 * i + 7]) for i in range(7)]
    return {(2 * (q // 2) + p // 2, 2 * (q % 2) + p % 2): v
            for p in range(4) for q, v in enumerate(_out4([c[p] for c in inner]))}


def _after(v, token, i):
    return jnp.where(i < 0, pltpu.bitcast(token, v.dtype), v)


def _silu(g):
    hg = 0.5 * g
    return hg * jnp.tanh(hg) + hg


def _norm(x):
    m = jnp.mean(x, axis=-1, keepdims=True)
    xc = x - m
    v = jnp.mean(xc * xc, axis=-1, keepdims=True)
    return xc * lax.rsqrt(v + 1e-5)


def _kernel(c_ref, mem0_ref, x_hbm, wq_hbm, wk_hbm, wv_hbm, wo_hbm, w1_hbm, w3_hbm, w2_hbm,
            wmod_hbm, out_hbm,
            xb, ab, wqkv, pre, wo, mod, hin, ru, rd, rm, scb, h2f, h2b, ob,
            sem_x, sem_mod, sem_stg, sem_wo, sem_raw, sem_out):
    n_seg, seg, D = xb.shape
    M = mem0_ref.shape[0]
    L = M + seg
    H = wq_hbm.shape[1]
    F = w1_hbm.shape[2]
    n_grp, n_ct, n_hc = H // HG, D // LANE, H // HC
    n_it = n_seg // UNR
    n_blk, spb = n_seg * seg // FM, FM // seg
    hd, qd, qf = D // 2, D // 4, F // 4
    n_dr, mr = qf // DR, D // n_it
    scale = float(LANE) ** -0.5

    def mrow(j):
        return mod[j, 0:1, :]

    def pre_attn(s):
        xs = xb[s].astype(F32)[0:seg - PRE]
        return _norm(xs) * (1.0 + mrow(1)) + mrow(0)

    x_cp = pltpu.make_async_copy(x_hbm, xb, sem_x.at[1])
    wo_cp = [pltpu.make_async_copy(wo_hbm.at[:, pl.ds(j * LANE, LANE)], wo.at[j],
                                   sem_wo.at[j]) for j in range(n_ct)]

    def raw_cp(kp, slot):
        rows = pl.ds(pl.multiple_of(kp * 16, 16), 16)
        cps = [pltpu.make_async_copy(w.at[:, rows, :], ru.at[slot, j],
                                     sem_raw.at[slot, j])
               for j, w in enumerate((w1_hbm, w3_hbm))]
        rows = pl.ds(pl.multiple_of(jnp.minimum(kp, n_dr // 2 - 1) * 2 * DR, 2 * DR), 2 * DR)
        cps.append(pltpu.make_async_copy(w2_hbm.at[:, rows, :], rd.at[slot], sem_raw.at[slot, 2]))
        rows = pl.ds(pl.multiple_of(kp * 2 * mr, 2 * mr), 2 * mr)
        return cps + [pltpu.make_async_copy(wmod_hbm.at[rows, pl.ds(2 * D, 4 * D)], rm.at[slot],
                                            sem_raw.at[slot, 3])]

    def warmup(xp, wm0, wm1, stg, tmp, hp):
        hw, hr = HC // 2, n_seg * PRE // 2
        mod_cp = [pltpu.make_async_copy(wmod_hbm.at[:, pl.ds(i * D, w.shape[1])],
                                        w, sem_mod.at[i])
                  for i, w in enumerate((wm0, wm1))]
        xp_cp = pltpu.make_async_copy(x_hbm.at[:, pl.ds(seg - PRE, PRE), :], xp, sem_x.at[0])

        def stg_cp(t, hc, slot):
            src = (wq_hbm, wk_hbm, wv_hbm)[t]
            return pltpu.make_async_copy(src.at[:, pl.ds(pl.multiple_of(hc * HC, HC), HC), :],
                                         stg.at[slot], sem_stg.at[slot])

        xp_cp.start()
        mod_cp[1].start()
        mod_cp[0].start()
        cv = c_ref[...].astype(F32)
        sc = jnp.broadcast_to(_rnd(cv * jax.nn.sigmoid(cv)), (8, D))
        for j in range(n_ct):
            scb[j * LANE:(j + 1) * LANE, :] = jnp.broadcast_to(
                sc[0:1, j * LANE:(j + 1) * LANE], (LANE, LANE)).T
        for j in range(2, 6):
            mod[j] = jnp.zeros((8, D), F32)
        xp_cp.wait()
        xn = _norm(xp[...].astype(F32).reshape(2 * hr, D))
        mod_cp[1].wait()
        stg_cp(0, 0, 0).start()
        mod[1] = _mm(sc, wm1[...])
        h = xn * (1.0 + mrow(1))
        scaled = _ops7(_LHS, (h[:hr, :hd], h[:hr, hd:], h[hr:, :hd], h[hr:, hd:]))
        mod_cp[0].wait()
        for i in range(1, NSTG):
            stg_cp(i // n_hc, i % n_hc, i).start()
        mod[0] = _mm(sc, wm0[...])
        shift = _ops7(_LHS, (mrow(0)[:, :hd], mrow(0)[:, hd:]) * 2)
        for i in range(7):
            hp[i] = _pack(scaled[i] + shift[i])

        def warm(i, carry):
            slot = lax.rem(i, NSTG)
            stg_cp(0, 0, slot).wait()
            for r in range(D // RP):
                v = stg[slot, pl.ds(r * RP, RP)].reshape(RP * HC, LANE)
                tmp[pl.ds(r * RP * hw, RP * hw), :] = pltpu.bitcast(v, U32)
            ops = []
            for j in range(hw):
                quad = []
                for half in range(2):
                    a = tmp[pl.ds(half * hd * hw + j, hd, stride=hw), :]
                    pair = [pltpu.bitcast(w, F32) for w in (a << 16, a & jnp.uint32(0xFFFF0000))]
                    for k, w in enumerate(_pack_all(pair)):
                        wqkv[i * HC + 2 * j + k, pl.ds(half * hd // 2, hd // 2), :] = w
                    quad += pair
                ops.append(_ops7(_RHS, quad))
            prod = {}
            for n in (1, 5, 0, 2, 3, 4, 6):
                w = jnp.concatenate([o[n] for o in ops], axis=1)
                cuts = KCUT.get(n, (0, hd))
                for k0, k1 in zip(cuts, cuts[1:]):
                    v = _mm(_unpack(hp[n, :, k0:k1]), w[k0:k1].astype(BF16))
                    prod[n] = v + prod[n] if k0 else v
            for n, cq in enumerate(_out4(prod)):
                cq = _pack(cq)
                for j in range(hw):
                    pre[i * HC + 2 * j + n % 2, pl.ds((n // 2) * hr // 2, hr // 2), :] = (
                        cq[:, j * LANE:(j + 1) * LANE])
            nx = i + NSTG
            for t in range(3):
                @pl.when(lax.div(nx, n_hc) == t)
                def _(t=t):
                    stg_cp(t, lax.rem(nx, n_hc), slot).start()

            for at, cps in ((0, [x_cp]), (2, wo_cp[:n_ct // 2]), (4, wo_cp[n_ct // 2:]),
                            (3 * n_hc - NSTG - 1, raw_cp(0, 0))):
                @pl.when(i == at)
                def _(cps=cps):
                    for cp in cps:
                        cp.start()

            return carry

        lax.fori_loop(0, 3 * n_hc, warm, 0)

    pl.run_scoped(warmup,
                  pltpu.VMEM((n_seg, PRE, D), BF16),
                  pltpu.VMEM((D, D), BF16),
                  pltpu.VMEM((D, D), BF16),
                  pltpu.VMEM((NSTG, D, HC, LANE), BF16),
                  pltpu.VMEM((D * HC // 2 + 8, LANE), U32),
                  pltpu.VMEM((7, n_seg * PRE // 4, hd), U32))
    for cp in [x_cp] + wo_cp:
        cp.wait()
    hin[...] = _pack(jnp.concatenate([mem0_ref[...].astype(F32), pre_attn(0)], axis=0))

    def step(k, u, side):
        s = k * UNR + u
        h = _unpack(hin[...])
        ri = lax.broadcasted_iota(jnp.int32, (L, L), 0)
        ci = lax.broadcasted_iota(jnp.int32, (L, L), 1)
        mask = (ri < M) | (ri >= ci)
        prow = pl.ds(pl.multiple_of(k * PRE, PRE), PRE)
        qkv, prob, att = {}, {}, {}

        def proj(g, ts):
            heads = [(t, g * HG + j) for t in ts for j in range(HG)]
            r = _mm(h, jnp.concatenate([_unpack(wqkv[t * H + n]) for t, n in heads], axis=1))
            for i, (t, n) in enumerate(heads):
                early = pre[t * H + n, prow, :]
                if (t, n) in side:
                    early = side[t, n](early)
                early = _unpack(early).astype(F32)[u * PRE:(u + 1) * PRE]
                qkv[t, n] = jnp.concatenate([r[:, i * LANE:(i + 1) * LANE], early], axis=0)

        def scores(g):
            for n in range(g * HG, (g + 1) * HG):
                sv = _mm_nt(_rnd(qkv[0, n]), qkv[1, n].astype(BF16)) * (scale * LOG2E)
                sv = jnp.where(mask, sv, -1e9 * LOG2E)
                e = jnp.exp2(sv - jnp.max(sv, axis=-1, keepdims=True))
                den = jnp.sum(e, axis=-1, keepdims=True)
                inv = pl.reciprocal(den, approx=True)
                prob[n] = _rnd(e * (inv * (2.0 - den * inv)))

        def values(g):
            for n in range(g * HG, (g + 1) * HG):
                att[n] = _rnd(_mm(prob[n], qkv[2, n].astype(BF16)))

        nxt = pre_attn(jnp.minimum(s + 1, n_seg - 1))
        for g in range(n_grp):
            proj(g, (0, 1))
            if g >= 1:
                scores(g - 1)
        for g in range(n_grp):
            proj(g, (2,))
            if g == 0:
                scores(n_grp - 1)
            if g >= VLAG:
                values(g - VLAG)
        for g in range(n_grp - VLAG, n_grp):
            values(g)
        cols = []
        for j in range(n_ct):
            w, per = pltpu.bitcast(wo[j], U32), H // n_ct
            rows = w.shape[0] // per
            parts = []
            for i in range(per):
                blk = w[i * rows:(i + 1) * rows]
                if (3, j * per + i) in side:
                    blk = jnp.concatenate([side[3, j * per + i](blk[:8]), blk[8:]], axis=0)
                parts.append(blk)
            cols.append(_unpack(jnp.concatenate(parts, axis=0)))
        acc = _mm(jnp.concatenate([att[n] for n in range(H)], axis=1),
                  jnp.concatenate(cols, axis=1))
        hin[...] = _pack(jnp.concatenate([acc[0:M], nxt], axis=0))
        ab[s] = acc[M:L].astype(BF16)

    def main(wu, wd):
        def steps(k, carry):
            kp, odd = lax.div(k, 2), lax.rem(k, 2)
            slot = lax.rem(kp, 2)
            kd = jnp.minimum(kp, n_dr // 2 - 1) * 2 + odd

            @pl.when(odd == 0)
            def _():
                for cp in raw_cp(kp, slot):
                    cp.wait()

            def up_piece(t, i, v):
                cols = pl.ds(t * LANE, LANE)
                ops = _ops49(_RHS, i, lambda r, c: ru[
                    slot, c // 2, r, :,
                    pl.ds(pl.multiple_of((2 * (c % 2) + odd) * qf + t * LANE, LANE), LANE)
                ].astype(F32))
                for j, o in enumerate(_pack_all(ops)):
                    wu[kp, odd, 7 * i + j, :, cols] = o
                return _after(v, wu[kp, jnp.minimum(odd, 1), 7 * i, :, cols], k)

            def down_piece(a, t, i, v):
                rows, cols = pl.ds(a * 8, 8), pl.ds(t * LANE, LANE)
                src = pl.ds(pl.multiple_of(odd * DR + a * 16, 16), 16)
                ops = _ops49(_RHS, i, lambda r, c: rd[
                    slot, r, src, pl.ds(c * qd + t * LANE, LANE)].astype(F32))
                for j, o in enumerate(_pack_all(ops)):
                    wd[kd, 7 * i + j, rows, cols] = o
                return _after(v, wd[jnp.minimum(kd, n_it), 7 * i, rows, cols], k)

            def mod_piece(j, c, v):
                w = rm[slot, pl.ds(pl.multiple_of(odd * mr, mr), mr), pl.ds(j * D + c * hd, hd)]
                sv = scb[pl.ds(pl.multiple_of(k * mr, mr), mr), :]
                t = w.astype(F32) * jnp.concatenate([sv] * (hd // LANE), axis=1)
                cols = pl.ds(c * hd, hd)
                mod[2 + j, :, cols] += sum(t[r:r + 8] for r in range(8, mr, 8)) + t[0:8]
                return _after(v, mod[jnp.minimum(k, 0) + 2 + j, :, pl.ds(c * hd, LANE)], k)

            pieces = [functools.partial(up_piece, t, i)
                      for t in range(qf // LANE) for i in range(7)]
            pieces += [functools.partial(down_piece, a, t, i) for a in range(DR // 16)
                       for t in range(qd // LANE) for i in range(7)]
            spots = [(u, t, n) for u in range(UNR) for t, m in SPOT for n in range(H) if n % 4 < m]
            assert len(pieces) <= len(spots)
            side = dict(zip(spots, pieces))
            for j in range(4):
                for c in range(2):
                    side[c, MSP[0], MSP[1] + 8 * j] = functools.partial(mod_piece, j, c)
            for u in range(UNR):
                step(k, u, {sp[1:]: f for sp, f in side.items() if sp[0] == u})

            @pl.when((odd == 0) & (k + 2 < n_it))
            def _():
                for cp in raw_cp(kp + 1, 1 - slot):
                    cp.start()

            return carry

        lax.fori_loop(0, n_it, steps, 0)
        for j in range(2, 6):
            mod[j] = jnp.broadcast_to(jnp.sum(mod[j], axis=0, keepdims=True), (8, D))

        def resid(sg, rows):
            return xb[sg, rows, :].astype(F32) + mrow(2) * ab[sg, rows, :].astype(F32)

        def norm_piece(b, r, a):
            rows = pl.ds(a * 16, 16)
            h2f[r, rows, :] = _norm(resid(b * 4 + r, rows)) * (1.0 + mrow(4)) + mrow(3)
            return h2f[jnp.minimum(b, 0) + r, pl.ds(a * 16, 8), 0:qd]

        def lhs_piece(b, a, i):
            ops = _ops49(_LHS, i, lambda r, c: h2f[r, pl.ds(a * 16, 16), pl.ds(c * qd, qd)])
            for j, o in enumerate(ops):
                h2b[7 * i + j, pl.ds(a * 8, 8), :] = _pack(o)
            return h2b[jnp.minimum(b, 0) + 7 * i, pl.ds(a * 8, 8), :]

        ffn_in = [functools.partial(norm_piece, r=r, a=a)
                  for r in range(4) for a in range(seg // 16)]
        ffn_in += [functools.partial(lhs_piece, a=a, i=i)
                   for a in range(seg // 16) for i in range(7)]

        def out_cp(b):
            return pltpu.make_async_copy(ob.at[b % 2], out_hbm.at[pl.ds(b * FM, FM), :],
                                         sem_out.at[b % 2])

        def ffn(b, carry):
            @pl.when(b >= 2)
            def _():
                out_cp(b - 2).wait()

            slot = lax.rem(b, 2)
            lhs = []
            for f in range(qf // LANE):
                cols = pl.ds(f * LANE, LANE)
                gu = _out16([_mm(_unpack(h2b[n]), jnp.concatenate(
                    [_unpack(wu[:, c, n, :, cols].reshape(qd // 2, LANE)) for c in range(2)],
                    axis=1)) for n in range(49)])
                act = {}
                for r in range(4):
                    for c in range(2):
                        v = _silu(gu[r, c]) * gu[r, 2 + c]
                        act[r, 2 * c], act[r, 2 * c + 1] = v[:, :LANE], v[:, LANE:]
                lhs.append([o for i in range(7)
                            for o in _ops49(_LHS, i, lambda r, c: act[r, c])])
            prod, late = [], []
            for n in range(49):
                w = wd[:, n].reshape(qf // 2, qd)
                if n in TIES:
                    token = ffn_in[TIES.index(n)](jnp.minimum(b + 1, n_blk - 1))
                    w = jnp.concatenate([_after(w[:8], token, b), w[8:]], axis=0)
                a = [l[n] for l in lhs]
                if n < NSPLIT:
                    ks = (qf - LANE) // 2
                    late.append((a.pop().astype(BF16), _unpack(w[ks:])))
                    w = w[:ks]
                prod.append(_mm(jnp.concatenate(a, axis=1).astype(BF16), _unpack(w)))
                if n == NSPLIT - 1:
                    prod = [_mm(*t) + v for t, v in zip(late, prod)]
            y = _out16(prod)
            for r in range(4):
                yr = jnp.concatenate([y[r, c] for c in range(4)], axis=1)
                ob[slot, pl.ds(r * seg, seg), :] = (
                    resid(b * 4 + r, slice(None)) + mrow(5) * yr).astype(ob.dtype)
            out_cp(b).start()
            return carry

        for piece in ffn_in:
            piece(0)
        lax.fori_loop(0, n_blk, ffn, 0)
        for b in range(n_blk - 2, n_blk):
            out_cp(b).wait()

    pl.run_scoped(main, pltpu.VMEM((n_it // 2, 2, 49, 8, qf), U32),
                  pltpu.VMEM((n_dr, 49, DR // 2, qd), U32))


@functools.partial(jax.jit, static_argnames=("A_seg_len",))
def pallas_adaLN_cond__memory_aug_recurrent_mem_tr__glu_gated_swiglu__prompt_kernel(
    A_x, A_mem0, A_Wq, A_Wk, A_Wv, A_Wo, A_seg_len, B_x, B_w1, B_w3, B_w2, c, w_mod,
):
    del B_x
    B, S, D = A_x.shape
    H, Dh = A_Wq.shape[1], A_Wq.shape[2]
    M = A_mem0.shape[1]
    F = B_w1.shape[1]
    seg = int(A_seg_len)
    n_seg = S // seg
    assert B == 1 and Dh == LANE and S % seg == 0 and S % FM == 0 and F % FC == 0
    hbm = pl.BlockSpec(memory_space=pl.ANY)
    vmem = pl.BlockSpec(memory_space=pltpu.VMEM)
    dma = pltpu.SemaphoreType.DMA
    out = pl.pallas_call(
        _kernel,
        out_shape=jax.ShapeDtypeStruct((S, D), A_x.dtype),
        in_specs=[vmem, vmem] + [hbm] * 9,
        out_specs=hbm,
        scratch_shapes=[
            pltpu.VMEM((n_seg, seg, D), BF16),
            pltpu.VMEM((n_seg, seg, D), BF16),
            pltpu.VMEM((3 * H, D // 2, LANE), U32),
            pltpu.VMEM((3 * H, n_seg * PRE // 2, LANE), U32),
            pltpu.VMEM((D // LANE, H * Dh, LANE), BF16),
            pltpu.VMEM((6, 8, D), F32),
            pltpu.VMEM(((M + seg - PRE) // 2, D), U32),
            pltpu.VMEM((2, 2, 4, 16, F), BF16),
            pltpu.VMEM((2, 4, 2 * DR, D), BF16),
            pltpu.VMEM((2, 2 * D * UNR // n_seg, 4 * D), BF16),
            pltpu.VMEM((D, LANE), F32),
            pltpu.VMEM((4, seg, D), F32),
            pltpu.VMEM((49, seg // 2, D // 4), U32),
            pltpu.VMEM((2, FM, D), A_x.dtype),
            dma((2,)), dma((2,)), dma((NSTG,)), dma((D // LANE,)), dma((2, 4)), dma((2,)),
        ],
        compiler_params=pltpu.CompilerParams(vmem_limit_bytes=127 * 2**20),
    )(c, A_mem0.reshape(M, D), A_x.reshape(n_seg, seg, D), A_Wq, A_Wk, A_Wv,
      A_Wo.reshape(H * Dh, D), B_w1.reshape(4, D // 4, F), B_w3.reshape(4, D // 4, F),
      B_w2.reshape(4, F // 4, D), w_mod)
    return out.reshape(B, S, D)
```

```python
import functools

import jax
import jax.numpy as jnp
from jax import lax
import jax.experimental.pallas as pl
import jax.experimental.pallas.tpu as pltpu

F32 = jnp.float32
BF16 = jnp.bfloat16
U32 = jnp.uint32
LANE = 128
LOG2E = 1.4426950408889634
PRE = 8
HC = 8
NSTG = 4
RP = 64
UNR = 2
HG = 4
VLAG = 4
DR = 32
SPOT = ((1, 1), (2, 1), (3, 3))
NSPLIT = 4
TIE0 = 17


def _mm(a, b):
    return lax.dot_general(a, b, (((1,), (0,)), ((), ())), preferred_element_type=F32)


def _mm_nt(a, b):
    return lax.dot_general(a, b, (((1,), (1,)), ((), ())), preferred_element_type=F32)


def _rnd(v):
    return v.astype(BF16).astype(F32)


def _pack(v):
    return pltpu.bitcast(v.astype(BF16), U32)


def _pack_all(vs):
    n = vs[0].shape[1]
    w = _pack(jnp.concatenate(vs, axis=1))
    return [w[:, i * n:(i + 1) * n] for i in range(len(vs))]


def _unpack(v):
    return pltpu.bitcast(v, BF16)


_LHS = (((1, 0), (1, 3)), ((1, 2), (1, 3)), ((1, 0),), ((1, 3),), ((1, 0), (1, 1)),
        ((1, 2), (-1, 0)), ((1, 1), (-1, 3)))
_RHS = (((1, 0), (1, 3)), ((1, 0),), ((1, 1), (-1, 3)), ((1, 2), (-1, 0)), ((1, 3),),
        ((1, 0), (1, 1)), ((1, 2), (1, 3)))


def _comb(terms, quad):
    v = quad(terms[0][1])
    for sign, q in terms[1:]:
        v = v + quad(q) if sign > 0 else v - quad(q)
    return v


def _ops7(table, quads):
    return [_comb(t, quads.__getitem__) for t in table]


def _ops49(table, i, block):
    return _ops7(table, [
        _comb(table[i], lambda q: block(2 * (q // 2) + r, 2 * (q % 2) + c))
        for r in range(2) for c in range(2)])


def _out4(m):
    return (m[0] + m[3] - m[4] + m[6], m[2] + m[4], m[1] + m[3], m[0] - m[1] + m[2] + m[5])


def _out16(m):
    inner = [_out4(m[7 * i:7 * i + 7]) for i in range(7)]
    return {(2 * (q // 2) + p // 2, 2 * (q % 2) + p % 2): v
            for p in range(4) for q, v in enumerate(_out4([c[p] for c in inner]))}


def _after(v, token, i):
    return jnp.where(i < 0, pltpu.bitcast(token, v.dtype), v)


def _silu(g):
    hg = 0.5 * g
    return hg * jnp.tanh(hg) + hg


def _norm(x):
    m = jnp.mean(x, axis=-1, keepdims=True)
    xc = x - m
    v = jnp.mean(xc * xc, axis=-1, keepdims=True)
    return xc * lax.rsqrt(v + 1e-5)


def _kernel(c_ref, mem0_ref, x_hbm, wq_hbm, wk_hbm, wv_hbm, wo_hbm, w1_hbm, w3_hbm, w2_hbm,
            wmod_hbm, out_hbm,
            xb, ab, wqkv, pre, wo, mod, hin, ru, rd, rm, scb, h2f, h2b, ob,
            sem_x, sem_mod, sem_stg, sem_wo, sem_raw, sem_out):
    n_seg, seg, D = xb.shape
    M = mem0_ref.shape[0]
    L = M + seg
    H = wq_hbm.shape[1]
    F = w1_hbm.shape[2]
    n_grp, n_ct, n_hc = H // HG, D // LANE, H // HC
    n_it = n_seg // UNR
    n_blk, fm = n_seg // 4, 4 * seg
    hd, qd, qf = D // 2, D // 4, F // 4
    n_dr, mr = qf // DR, D // n_it
    scale = float(LANE) ** -0.5

    def mrow(j):
        return mod[j, 0:1, :]

    def pre_attn(s):
        xs = xb[s].astype(F32)[0:seg - PRE]
        return _norm(xs) * (1.0 + mrow(1)) + mrow(0)

    x_cp = pltpu.make_async_copy(x_hbm, xb, sem_x.at[1])
    wo_cp = [pltpu.make_async_copy(wo_hbm.at[:, pl.ds(j * LANE, LANE)], wo.at[j],
                                   sem_wo.at[j]) for j in range(n_ct)]

    def raw_cp(kp, slot):
        rows = pl.ds(pl.multiple_of(kp * 16, 16), 16)
        cps = [pltpu.make_async_copy(w.at[:, rows, :], ru.at[slot, j],
                                     sem_raw.at[slot, j])
               for j, w in enumerate((w1_hbm, w3_hbm))]
        rows = pl.ds(pl.multiple_of(jnp.minimum(kp, n_dr // 2 - 1) * 2 * DR, 2 * DR), 2 * DR)
        cps.append(pltpu.make_async_copy(w2_hbm.at[:, rows, :], rd.at[slot], sem_raw.at[slot, 2]))
        rows = pl.ds(pl.multiple_of(kp * 2 * mr, 2 * mr), 2 * mr)
        return cps + [pltpu.make_async_copy(wmod_hbm.at[rows, pl.ds(2 * D, 4 * D)], rm.at[slot],
                                            sem_raw.at[slot, 3])]

    def warmup(xp, wm0, wm1, stg, tmp, hp):
        hw, hr = HC // 2, n_seg * PRE // 2
        mod_cp = [pltpu.make_async_copy(wmod_hbm.at[:, pl.ds(i * D, w.shape[1])],
                                        w, sem_mod.at[i])
                  for i, w in enumerate((wm0, wm1))]
        xp_cp = pltpu.make_async_copy(x_hbm.at[:, pl.ds(seg - PRE, PRE), :], xp, sem_x.at[0])

        def stg_cp(t, hc, slot):
            src = (wq_hbm, wk_hbm, wv_hbm)[t]
            return pltpu.make_async_copy(src.at[:, pl.ds(pl.multiple_of(hc * HC, HC), HC), :],
                                         stg.at[slot], sem_stg.at[slot])

        xp_cp.start()
        mod_cp[1].start()
        mod_cp[0].start()
        cv = c_ref[...].astype(F32)
        sc = jnp.broadcast_to(_rnd(cv * jax.nn.sigmoid(cv)), (8, D))
        for j in range(n_ct):
            scb[j * LANE:(j + 1) * LANE, :] = jnp.broadcast_to(
                sc[0:1, j * LANE:(j + 1) * LANE], (LANE, LANE)).T
        for j in range(2, 6):
            mod[j] = jnp.zeros((8, D), F32)
        xp_cp.wait()
        xn = _norm(xp[...].astype(F32).reshape(2 * hr, D))
        mod_cp[1].wait()
        stg_cp(0, 0, 0).start()
        mod[1] = _mm(sc, wm1[...])
        h = xn * (1.0 + mrow(1))
        scaled = _ops7(_LHS, (h[:hr, :hd], h[:hr, hd:], h[hr:, :hd], h[hr:, hd:]))
        mod_cp[0].wait()
        for i in range(1, NSTG):
            stg_cp(i // n_hc, i % n_hc, i).start()
        mod[0] = _mm(sc, wm0[...])
        shift = _ops7(_LHS, (mrow(0)[:, :hd], mrow(0)[:, hd:]) * 2)
        for i in range(7):
            hp[i] = _pack(scaled[i] + shift[i])

        def warm(i, carry):
            slot = lax.rem(i, NSTG)
            stg_cp(0, 0, slot).wait()
            for r in range(D // RP):
                v = stg[slot, pl.ds(r * RP, RP)].reshape(RP * HC, LANE)
                tmp[pl.ds(r * RP * hw, RP * hw), :] = pltpu.bitcast(v, U32)
            ops = []
            for j in range(hw):
                quad = []
                for half in range(2):
                    a = tmp[pl.ds(half * hd * hw + j, hd, stride=hw), :]
                    pair = [pltpu.bitcast(w, F32) for w in (a << 16, a & jnp.uint32(0xFFFF0000))]
                    for k, w in enumerate(_pack_all(pair)):
                        wqkv[i * HC + 2 * j + k, pl.ds(half * hd // 2, hd // 2), :] = w
                    quad += pair
                ops.append(_ops7(_RHS, quad))
            prod = {}
            for n in (1, 5, 0, 2, 3, 4, 6):
                w = jnp.concatenate([o[n] for o in ops], axis=1)
                cuts = (0, hd) if prod else (0, LANE, hd)
                for k0, k1 in zip(cuts, cuts[1:]):
                    v = _mm(_unpack(hp[n, :, k0:k1]), w[k0:k1].astype(BF16))
                    prod[n] = v + prod[n] if k0 else v
            for n, cq in enumerate(_out4(prod)):
                cq = _pack(cq)
                for j in range(hw):
                    pre[i * HC + 2 * j + n % 2, pl.ds((n // 2) * hr // 2, hr // 2), :] = (
                        cq[:, j * LANE:(j + 1) * LANE])
            nx = i + NSTG
            for t in range(3):
                @pl.when(lax.div(nx, n_hc) == t)
                def _(t=t):
                    stg_cp(t, lax.rem(nx, n_hc), slot).start()

            for at, cps in ((0, [x_cp]), (2, wo_cp[:n_ct // 2]), (4, wo_cp[n_ct // 2:]),
                            (3 * n_hc - NSTG - 1, raw_cp(0, 0))):
                @pl.when(i == at)
                def _(cps=cps):
                    for cp in cps:
                        cp.start()

            return carry

        lax.fori_loop(0, 3 * n_hc, warm, 0)

    pl.run_scoped(warmup,
                  pltpu.VMEM((n_seg, PRE, D), BF16),
                  pltpu.VMEM((D, D), BF16),
                  pltpu.VMEM((D, D), BF16),
                  pltpu.VMEM((NSTG, D, HC, LANE), BF16),
                  pltpu.VMEM((D * HC // 2 + 8, LANE), U32),
                  pltpu.VMEM((7, n_seg * PRE // 4, hd), U32))
    for cp in [x_cp] + wo_cp:
        cp.wait()
    hin[...] = _pack(jnp.concatenate([mem0_ref[...].astype(F32), pre_attn(0)], axis=0))

    def step(k, u, side):
        s = k * UNR + u
        h = _unpack(hin[...])
        ri = lax.broadcasted_iota(jnp.int32, (L, L), 0)
        ci = lax.broadcasted_iota(jnp.int32, (L, L), 1)
        mask = (ri < M) | (ri >= ci)
        prow = pl.ds(pl.multiple_of(k * PRE, PRE), PRE)
        qkv, prob, att = {}, {}, {}

        def proj(g, ts):
            heads = [(t, g * HG + j) for t in ts for j in range(HG)]
            r = _mm(h, jnp.concatenate([_unpack(wqkv[t * H + n]) for t, n in heads], axis=1))
            for i, (t, n) in enumerate(heads):
                early = pre[t * H + n, prow, :]
                if (t, n) in side:
                    early = side[t, n](early)
                early = _unpack(early).astype(F32)[u * PRE:(u + 1) * PRE]
                qkv[t, n] = jnp.concatenate([r[:, i * LANE:(i + 1) * LANE], early], axis=0)

        def scores(g):
            for n in range(g * HG, (g + 1) * HG):
                sv = _mm_nt(_rnd(qkv[0, n]), qkv[1, n].astype(BF16)) * (scale * LOG2E)
                sv = jnp.where(mask, sv, -1e9 * LOG2E)
                e = jnp.exp2(sv - jnp.max(sv, axis=-1, keepdims=True))
                den = jnp.sum(e, axis=-1, keepdims=True)
                inv = pl.reciprocal(den, approx=True)
                prob[n] = _rnd(e * (inv * (2.0 - den * inv)))

        def values(g):
            for n in range(g * HG, (g + 1) * HG):
                att[n] = _rnd(_mm(prob[n], qkv[2, n].astype(BF16)))

        nxt = pre_attn(jnp.minimum(s + 1, n_seg - 1))
        for g in range(n_grp):
            proj(g, (0, 1))
            if g >= 1:
                scores(g - 1)
        for g in range(n_grp):
            proj(g, (2,))
            if g == 0:
                scores(n_grp - 1)
            if g >= VLAG:
                values(g - VLAG)
        for g in range(n_grp - VLAG, n_grp):
            values(g)
        cols = []
        for j in range(n_ct):
            w, per = pltpu.bitcast(wo[j], U32), H // n_ct
            rows = w.shape[0] // per
            parts = []
            for i in range(per):
                blk = w[i * rows:(i + 1) * rows]
                if (3, j * per + i) in side:
                    blk = jnp.concatenate([side[3, j * per + i](blk[:8]), blk[8:]], axis=0)
                parts.append(blk)
            cols.append(_unpack(jnp.concatenate(parts, axis=0)))
        acc = _mm(jnp.concatenate([att[n] for n in range(H)], axis=1),
                  jnp.concatenate(cols, axis=1))
        hin[...] = _pack(jnp.concatenate([acc[0:M], nxt], axis=0))
        ab[s] = acc[M:L].astype(BF16)

    def main(wu, wd):
        def steps(k, carry):
            kp, odd = lax.div(k, 2), lax.rem(k, 2)
            slot = lax.rem(kp, 2)
            kd = jnp.minimum(kp, n_dr // 2 - 1) * 2 + odd

            @pl.when(odd == 0)
            def _():
                for cp in raw_cp(kp, slot):
                    cp.wait()

            def up_piece(t, i, v):
                cols = pl.ds(t * LANE, LANE)
                ops = _ops49(_RHS, i, lambda r, c: ru[
                    slot, c // 2, r, :,
                    pl.ds(pl.multiple_of((2 * (c % 2) + odd) * qf + t * LANE, LANE), LANE)
                ].astype(F32))
                for j, o in enumerate(_pack_all(ops)):
                    wu[kp, odd, 7 * i + j, :, cols] = o
                return _after(v, wu[kp, jnp.minimum(odd, 1), 7 * i, :, cols], k)

            def down_piece(a, t, i, v):
                rows, cols = pl.ds(a * 8, 8), pl.ds(t * LANE, LANE)
                src = pl.ds(pl.multiple_of(odd * DR + a * 16, 16), 16)
                ops = _ops49(_RHS, i, lambda r, c: rd[
                    slot, r, src, pl.ds(c * qd + t * LANE, LANE)].astype(F32))
                for j, o in enumerate(_pack_all(ops)):
                    wd[kd, 7 * i + j, rows, cols] = o
                return _after(v, wd[jnp.minimum(kd, n_it), 7 * i, rows, cols], k)

            def mod_piece(j, c, v):
                w = rm[slot, pl.ds(pl.multiple_of(odd * mr, mr), mr), pl.ds(j * D + c * hd, hd)]
                sv = scb[pl.ds(pl.multiple_of(k * mr, mr), mr), :]
                t = w.astype(F32) * jnp.concatenate([sv] * (hd // LANE), axis=1)
                cols = pl.ds(c * hd, hd)
                mod[2 + j, :, cols] += sum(t[r:r + 8] for r in range(8, mr, 8)) + t[0:8]
                return _after(v, mod[jnp.minimum(k, 0) + 2 + j, :, pl.ds(c * hd, LANE)], k)

            pieces = [functools.partial(up_piece, t, i)
                      for t in range(qf // LANE) for i in range(7)]
            pieces += [functools.partial(down_piece, a, t, i) for a in range(DR // 16)
                       for t in range(qd // LANE) for i in range(7)]
            spots = [(u, t, n) for u in range(UNR) for t, m in SPOT for n in range(H) if n % 4 < m]
            assert len(pieces) <= len(spots)
            side = dict(zip(spots, pieces))
            for j in range(4):
                for c in range(2):
                    side[c, 3, 3 + 8 * j] = functools.partial(mod_piece, j, c)
            for u in range(UNR):
                step(k, u, {sp[1:]: f for sp, f in side.items() if sp[0] == u})

            @pl.when((odd == 0) & (k + 2 < n_it))
            def _():
                for cp in raw_cp(kp + 1, 1 - slot):
                    cp.start()

            return carry

        lax.fori_loop(0, n_it, steps, 0)
        for j in range(2, 6):
            mod[j] = jnp.broadcast_to(jnp.sum(mod[j], axis=0, keepdims=True), (8, D))

        def resid(sg, rows):
            return xb[sg, rows, :].astype(F32) + mrow(2) * ab[sg, rows, :].astype(F32)

        def norm_piece(b, r, a):
            rows = pl.ds(a * 16, 16)
            h2f[r, rows, :] = _norm(resid(b * 4 + r, rows)) * (1.0 + mrow(4)) + mrow(3)
            return h2f[jnp.minimum(b, 0) + r, pl.ds(a * 16, 8), 0:qd]

        def lhs_piece(b, a, i):
            ops = _ops49(_LHS, i, lambda r, c: h2f[r, pl.ds(a * 16, 16), pl.ds(c * qd, qd)])
            for j, o in enumerate(ops):
                h2b[7 * i + j, pl.ds(a * 8, 8), :] = _pack(o)
            return h2b[jnp.minimum(b, 0) + 7 * i, pl.ds(a * 8, 8), :]

        ffn_in = [functools.partial(norm_piece, r=r, a=a)
                  for r in range(4) for a in range(seg // 16)]
        ffn_in += [functools.partial(lhs_piece, a=a, i=i)
                   for a in range(seg // 16) for i in range(7)]

        def out_cp(b):
            return pltpu.make_async_copy(ob.at[b % 2], out_hbm.at[pl.ds(b * fm, fm), :],
                                         sem_out.at[b % 2])

        def ffn(b, carry):
            @pl.when(b >= 2)
            def _():
                out_cp(b - 2).wait()

            slot = lax.rem(b, 2)
            lhs = []
            for f in range(qf // LANE):
                cols = pl.ds(f * LANE, LANE)
                gu = _out16([_mm(_unpack(h2b[n]), jnp.concatenate(
                    [_unpack(wu[:, c, n, :, cols].reshape(qd // 2, LANE)) for c in range(2)],
                    axis=1)) for n in range(49)])
                act = {}
                for r in range(4):
                    for c in range(2):
                        v = _silu(gu[r, c]) * gu[r, 2 + c]
                        act[r, 2 * c], act[r, 2 * c + 1] = v[:, :LANE], v[:, LANE:]
                lhs.append([o for i in range(7)
                            for o in _ops49(_LHS, i, lambda r, c: act[r, c])])
            prod, late = [], []
            for n in range(49):
                w = wd[:, n].reshape(qf // 2, qd)
                if 0 <= n - TIE0 < len(ffn_in):
                    token = ffn_in[n - TIE0](jnp.minimum(b + 1, n_blk - 1))
                    w = jnp.concatenate([_after(w[:8], token, b), w[8:]], axis=0)
                a = [l[n] for l in lhs]
                if n < NSPLIT:
                    ks = (qf - LANE) // 2
                    late.append((a.pop().astype(BF16), _unpack(w[ks:])))
                    w = w[:ks]
                prod.append(_mm(jnp.concatenate(a, axis=1).astype(BF16), _unpack(w)))
                if n == NSPLIT - 1:
                    prod = [_mm(*t) + v for t, v in zip(late, prod)]
            y = _out16(prod)
            for r in range(4):
                yr = jnp.concatenate([y[r, c] for c in range(4)], axis=1)
                ob[slot, pl.ds(r * seg, seg), :] = (
                    resid(b * 4 + r, slice(None)) + mrow(5) * yr).astype(ob.dtype)
            out_cp(b).start()
            return carry

        for piece in ffn_in:
            piece(0)
        lax.fori_loop(0, n_blk, ffn, 0)
        for b in range(n_blk - 2, n_blk):
            out_cp(b).wait()

    pl.run_scoped(main, pltpu.VMEM((n_it // 2, 2, 49, 8, qf), U32),
                  pltpu.VMEM((n_dr, 49, DR // 2, qd), U32))


@functools.partial(jax.jit, static_argnames=("A_seg_len",))
def pallas_adaLN_cond__memory_aug_recurrent_mem_tr__glu_gated_swiglu__prompt_kernel(
    A_x, A_mem0, A_Wq, A_Wk, A_Wv, A_Wo, A_seg_len, B_x, B_w1, B_w3, B_w2, c, w_mod,
):
    del B_x
    B, S, D = A_x.shape
    H, Dh = A_Wq.shape[1], A_Wq.shape[2]
    M = A_mem0.shape[1]
    F = B_w1.shape[1]
    seg = int(A_seg_len)
    n_seg = S // seg
    assert B == 1 and Dh == LANE and H == 32 and (M, seg) == (8, 32) and S == n_seg * seg
    assert D == 16 * n_seg and F % (4 * LANE) == 0 and F // 4 <= DR * n_seg // UNR
    hbm = pl.BlockSpec(memory_space=pl.ANY)
    vmem = pl.BlockSpec(memory_space=pltpu.VMEM)
    dma = pltpu.SemaphoreType.DMA
    out = pl.pallas_call(
        _kernel,
        out_shape=jax.ShapeDtypeStruct((S, D), A_x.dtype),
        in_specs=[vmem, vmem] + [hbm] * 9,
        out_specs=hbm,
        scratch_shapes=[
            pltpu.VMEM((n_seg, seg, D), BF16),
            pltpu.VMEM((n_seg, seg, D), BF16),
            pltpu.VMEM((3 * H, D // 2, LANE), U32),
            pltpu.VMEM((3 * H, n_seg * PRE // 2, LANE), U32),
            pltpu.VMEM((D // LANE, H * Dh, LANE), BF16),
            pltpu.VMEM((6, 8, D), F32),
            pltpu.VMEM(((M + seg - PRE) // 2, D), U32),
            pltpu.VMEM((2, 2, 4, 16, F), BF16),
            pltpu.VMEM((2, 4, 2 * DR, D), BF16),
            pltpu.VMEM((2, 2 * D * UNR // n_seg, 4 * D), BF16),
            pltpu.VMEM((D, LANE), F32),
            pltpu.VMEM((4, seg, D), F32),
            pltpu.VMEM((49, seg // 2, D // 4), U32),
            pltpu.VMEM((2, 4 * seg, D), A_x.dtype),
            dma((2,)), dma((2,)), dma((NSTG,)), dma((D // LANE,)), dma((2, 4)), dma((2,)),
        ],
        compiler_params=pltpu.CompilerParams(vmem_limit_bytes=127 * 2**20),
    )(c, A_mem0.reshape(M, D), A_x.reshape(n_seg, seg, D), A_Wq, A_Wk, A_Wv,
      A_Wo.reshape(H * Dh, D), B_w1.reshape(4, D // 4, F), B_w3.reshape(4, D // 4, F),
      B_w2.reshape(4, F // 4, D), w_mod)
    return out.reshape(B, S, D)
```

```python
import functools

import jax
import jax.numpy as jnp
from jax import lax
import jax.experimental.pallas as pl
import jax.experimental.pallas.tpu as pltpu

F32 = jnp.float32
BF16 = jnp.bfloat16
U32 = jnp.uint32
LANE = 128
LOG2E = 1.4426950408889634
PRE = 8
HC = 8
NSTG = 4
RP = 64
UNR = 2
HG = 4
VLAG = 4
DR = 32
SPOT = ((1, 1), (2, 1), (3, 3))
NSPLIT = 4
TIE0 = 17


def _mm(a, b):
    return lax.dot_general(a, b, (((1,), (0,)), ((), ())), preferred_element_type=F32)


def _mm_nt(a, b):
    return lax.dot_general(a, b, (((1,), (1,)), ((), ())), preferred_element_type=F32)


def _rnd(v):
    return v.astype(BF16).astype(F32)


def _pack(v):
    return pltpu.bitcast(v.astype(BF16), U32)


def _pack_all(vs):
    n = vs[0].shape[1]
    w = _pack(jnp.concatenate(vs, axis=1))
    return [w[:, i * n:(i + 1) * n] for i in range(len(vs))]


def _unpack(v):
    return pltpu.bitcast(v, BF16)


_LHS = (((1, 0), (1, 3)), ((1, 2), (1, 3)), ((1, 0),), ((1, 3),), ((1, 0), (1, 1)),
        ((1, 2), (-1, 0)), ((1, 1), (-1, 3)))
_RHS = (((1, 0), (1, 3)), ((1, 0),), ((1, 1), (-1, 3)), ((1, 2), (-1, 0)), ((1, 3),),
        ((1, 0), (1, 1)), ((1, 2), (1, 3)))


def _comb(terms, quad):
    v = quad(terms[0][1])
    for sign, q in terms[1:]:
        v = v + quad(q) if sign > 0 else v - quad(q)
    return v


def _ops7(table, quads):
    return [_comb(t, quads.__getitem__) for t in table]


def _ops49(table, i, block):
    return _ops7(table, [
        _comb(table[i], lambda q: block(2 * (q // 2) + r, 2 * (q % 2) + c))
        for r in range(2) for c in range(2)])


def _out4(m):
    return (m[0] + m[3] - m[4] + m[6], m[2] + m[4], m[1] + m[3], m[0] - m[1] + m[2] + m[5])


def _out16(m):
    inner = [_out4(m[7 * i:7 * i + 7]) for i in range(7)]
    return {(2 * (q // 2) + p // 2, 2 * (q % 2) + p % 2): v
            for p in range(4) for q, v in enumerate(_out4([c[p] for c in inner]))}


def _after(v, token, i):
    return jnp.where(i < 0, pltpu.bitcast(token, v.dtype), v)


def _silu(g):
    hg = 0.5 * g
    return hg * jnp.tanh(hg) + hg


def _norm(x):
    m = jnp.mean(x, axis=-1, keepdims=True)
    xc = x - m
    v = jnp.mean(xc * xc, axis=-1, keepdims=True)
    return xc * lax.rsqrt(v + 1e-5)


def _kernel(c_hbm, mem0_hbm, x_hbm, wq_hbm, wk_hbm, wv_hbm, wo_hbm, w1_hbm, w3_hbm, w2_hbm,
            wmod_hbm, out_hbm,
            xb, ab, wqkv, pre, wo, mod, hin, ru, rd, rm, scb, h2f, h2b, ob, mem0_ref,
            sem_x, sem_mod, sem_stg, sem_wo, sem_raw, sem_out):
    n_seg, seg, D = xb.shape
    M = mem0_ref.shape[0]
    L = M + seg
    H = wq_hbm.shape[1]
    F = w1_hbm.shape[2]
    n_grp, n_ct, n_hc = H // HG, D // LANE, H // HC
    n_it = n_seg // UNR
    n_blk, fm = n_seg // 4, 4 * seg
    hd, qd, qf = D // 2, D // 4, F // 4
    n_dr, mr = qf // DR, D // n_it
    scale = float(LANE) ** -0.5

    def mrow(j):
        return mod[j, 0:1, :]

    def pre_attn(s):
        xs = xb[s].astype(F32)[0:seg - PRE]
        return _norm(xs) * (1.0 + mrow(1)) + mrow(0)

    mem_cp = pltpu.make_async_copy(mem0_hbm, mem0_ref, sem_x.at[3])
    x_cp = pltpu.make_async_copy(x_hbm, xb, sem_x.at[1])
    wo_cp = [pltpu.make_async_copy(wo_hbm.at[:, pl.ds(j * LANE, LANE)], wo.at[j],
                                   sem_wo.at[j]) for j in range(n_ct)]

    def raw_cp(kp, slot):
        rows = pl.ds(pl.multiple_of(kp * 16, 16), 16)
        cps = [pltpu.make_async_copy(w.at[:, rows, :], ru.at[slot, j],
                                     sem_raw.at[slot, j])
               for j, w in enumerate((w1_hbm, w3_hbm))]
        rows = pl.ds(pl.multiple_of(jnp.minimum(kp, n_dr // 2 - 1) * 2 * DR, 2 * DR), 2 * DR)
        cps.append(pltpu.make_async_copy(w2_hbm.at[:, rows, :], rd.at[slot], sem_raw.at[slot, 2]))
        rows = pl.ds(pl.multiple_of(kp * 2 * mr, 2 * mr), 2 * mr)
        return cps + [pltpu.make_async_copy(wmod_hbm.at[rows, pl.ds(2 * D, 4 * D)], rm.at[slot],
                                            sem_raw.at[slot, 3])]

    def warmup(xp, wm0, wm1, stg, tmp, hp, c_ref):
        hw, hr = HC // 2, n_seg * PRE // 2
        mod_cp = [pltpu.make_async_copy(wmod_hbm.at[:, pl.ds(i * D, w.shape[1])],
                                        w, sem_mod.at[i])
                  for i, w in enumerate((wm0, wm1))]
        c_cp = pltpu.make_async_copy(c_hbm, c_ref, sem_x.at[2])
        xp_cp = pltpu.make_async_copy(x_hbm.at[:, pl.ds(seg - PRE, PRE), :], xp, sem_x.at[0])

        def stg_cp(t, hc, slot):
            src = (wq_hbm, wk_hbm, wv_hbm)[t]
            return pltpu.make_async_copy(src.at[:, pl.ds(pl.multiple_of(hc * HC, HC), HC), :],
                                         stg.at[slot], sem_stg.at[slot])

        c_cp.start()
        xp_cp.start()
        mod_cp[1].start()
        mod_cp[0].start()
        c_cp.wait()
        cv = c_ref[...].astype(F32)
        sc = jnp.broadcast_to(_rnd(cv * jax.nn.sigmoid(cv)), (8, D))
        for j in range(n_ct):
            scb[j * LANE:(j + 1) * LANE, :] = jnp.broadcast_to(
                sc[0:1, j * LANE:(j + 1) * LANE], (LANE, LANE)).T
        for j in range(2, 6):
            mod[j] = jnp.zeros((8, D), F32)
        xp_cp.wait()
        xn = _norm(xp[...].astype(F32).reshape(2 * hr, D))
        mod_cp[1].wait()
        stg_cp(0, 0, 0).start()
        mod[1] = _mm(sc, wm1[...])
        h = xn * (1.0 + mrow(1))
        scaled = _ops7(_LHS, (h[:hr, :hd], h[:hr, hd:], h[hr:, :hd], h[hr:, hd:]))
        mod_cp[0].wait()
        for i in range(1, NSTG):
            stg_cp(i // n_hc, i % n_hc, i).start()
        mod[0] = _mm(sc, wm0[...])
        shift = _ops7(_LHS, (mrow(0)[:, :hd], mrow(0)[:, hd:]) * 2)
        for i in range(7):
            hp[i] = _pack(scaled[i] + shift[i])

        def warm(i, carry):
            slot = lax.rem(i, NSTG)
            stg_cp(0, 0, slot).wait()
            for r in range(D // RP):
                v = stg[slot, pl.ds(r * RP, RP)].reshape(RP * HC, LANE)
                tmp[pl.ds(r * RP * hw, RP * hw), :] = pltpu.bitcast(v, U32)
            ops = []
            for j in range(hw):
                quad = []
                for half in range(2):
                    a = tmp[pl.ds(half * hd * hw + j, hd, stride=hw), :]
                    pair = [pltpu.bitcast(w, F32) for w in (a << 16, a & jnp.uint32(0xFFFF0000))]
                    for k, w in enumerate(_pack_all(pair)):
                        wqkv[i * HC + 2 * j + k, pl.ds(half * hd // 2, hd // 2), :] = w
                    quad += pair
                ops.append(_ops7(_RHS, quad))
            prod = {}
            for n in (1, 5, 0, 2, 3, 4, 6):
                w = jnp.concatenate([o[n] for o in ops], axis=1)
                cuts = (0, hd) if prod else (0, LANE, hd)
                for k0, k1 in zip(cuts, cuts[1:]):
                    v = _mm(_unpack(hp[n, :, k0:k1]), w[k0:k1].astype(BF16))
                    prod[n] = v + prod[n] if k0 else v
            for n, cq in enumerate(_out4(prod)):
                cq = _pack(cq)
                for j in range(hw):
                    pre[i * HC + 2 * j + n % 2, pl.ds((n // 2) * hr // 2, hr // 2), :] = (
                        cq[:, j * LANE:(j + 1) * LANE])
            nx = i + NSTG
            for t in range(3):
                @pl.when(lax.div(nx, n_hc) == t)
                def _(t=t):
                    stg_cp(t, lax.rem(nx, n_hc), slot).start()

            for at, cps in ((0, [x_cp, mem_cp]), (2, wo_cp[:n_ct // 2]), (4, wo_cp[n_ct // 2:]),
                            (3 * n_hc - NSTG - 1, raw_cp(0, 0))):
                @pl.when(i == at)
                def _(cps=cps):
                    for cp in cps:
                        cp.start()

            return carry

        lax.fori_loop(0, 3 * n_hc, warm, 0)

    pl.run_scoped(warmup,
                  pltpu.VMEM((n_seg, PRE, D), BF16),
                  pltpu.VMEM((D, D), BF16),
                  pltpu.VMEM((D, D), BF16),
                  pltpu.VMEM((NSTG, D, HC, LANE), BF16),
                  pltpu.VMEM((D * HC // 2 + 8, LANE), U32),
                  pltpu.VMEM((7, n_seg * PRE // 4, hd), U32),
                  pltpu.VMEM((1, D), BF16))
    for cp in [x_cp, mem_cp] + wo_cp:
        cp.wait()
    hin[...] = _pack(jnp.concatenate([mem0_ref[...].astype(F32), pre_attn(0)], axis=0))

    def step(k, u, side):
        s = k * UNR + u
        h = _unpack(hin[...])
        ri = lax.broadcasted_iota(jnp.int32, (L, L), 0)
        ci = lax.broadcasted_iota(jnp.int32, (L, L), 1)
        mask = (ri < M) | (ri >= ci)
        prow = pl.ds(pl.multiple_of(k * PRE, PRE), PRE)
        qkv, prob, att = {}, {}, {}

        def proj(g, ts):
            heads = [(t, g * HG + j) for t in ts for j in range(HG)]
            r = _mm(h, jnp.concatenate([_unpack(wqkv[t * H + n]) for t, n in heads], axis=1))
            for i, (t, n) in enumerate(heads):
                early = pre[t * H + n, prow, :]
                if (t, n) in side:
                    early = side[t, n](early)
                early = _unpack(early).astype(F32)[u * PRE:(u + 1) * PRE]
                qkv[t, n] = jnp.concatenate([r[:, i * LANE:(i + 1) * LANE], early], axis=0)

        def scores(g):
            for n in range(g * HG, (g + 1) * HG):
                sv = _mm_nt(_rnd(qkv[0, n]), qkv[1, n].astype(BF16)) * (scale * LOG2E)
                sv = jnp.where(mask, sv, -1e9 * LOG2E)
                e = jnp.exp2(sv - jnp.max(sv, axis=-1, keepdims=True))
                den = jnp.sum(e, axis=-1, keepdims=True)
                inv = pl.reciprocal(den, approx=True)
                prob[n] = _rnd(e * (inv * (2.0 - den * inv)))

        def values(g):
            for n in range(g * HG, (g + 1) * HG):
                att[n] = _rnd(_mm(prob[n], qkv[2, n].astype(BF16)))

        nxt = pre_attn(jnp.minimum(s + 1, n_seg - 1))
        for g in range(n_grp):
            proj(g, (0, 1))
            if g >= 1:
                scores(g - 1)
        for g in range(n_grp):
            proj(g, (2,))
            if g == 0:
                scores(n_grp - 1)
            if g >= VLAG:
                values(g - VLAG)
        for g in range(n_grp - VLAG, n_grp):
            values(g)
        cols = []
        for j in range(n_ct):
            w, per = pltpu.bitcast(wo[j], U32), H // n_ct
            rows = w.shape[0] // per
            parts = []
            for i in range(per):
                blk = w[i * rows:(i + 1) * rows]
                if (3, j * per + i) in side:
                    blk = jnp.concatenate([side[3, j * per + i](blk[:8]), blk[8:]], axis=0)
                parts.append(blk)
            cols.append(_unpack(jnp.concatenate(parts, axis=0)))
        acc = _mm(jnp.concatenate([att[n] for n in range(H)], axis=1),
                  jnp.concatenate(cols, axis=1))
        hin[...] = _pack(jnp.concatenate([acc[0:M], nxt], axis=0))
        ab[s] = acc[M:L].astype(BF16)

    def main(wu, wd):
        def steps(k, carry):
            kp, odd = lax.div(k, 2), lax.rem(k, 2)
            slot = lax.rem(kp, 2)
            kd = jnp.minimum(kp, n_dr // 2 - 1) * 2 + odd

            @pl.when(odd == 0)
            def _():
                for cp in raw_cp(kp, slot):
                    cp.wait()

            def up_piece(t, i, v):
                cols = pl.ds(t * LANE, LANE)
                ops = _ops49(_RHS, i, lambda r, c: ru[
                    slot, c // 2, r, :,
                    pl.ds(pl.multiple_of((2 * (c % 2) + odd) * qf + t * LANE, LANE), LANE)
                ].astype(F32))
                for j, o in enumerate(_pack_all(ops)):
                    wu[kp, odd, 7 * i + j, :, cols] = o
                return _after(v, wu[kp, jnp.minimum(odd, 1), 7 * i, :, cols], k)

            def down_piece(a, t, i, v):
                rows, cols = pl.ds(a * 8, 8), pl.ds(t * LANE, LANE)
                src = pl.ds(pl.multiple_of(odd * DR + a * 16, 16), 16)
                ops = _ops49(_RHS, i, lambda r, c: rd[
                    slot, r, src, pl.ds(c * qd + t * LANE, LANE)].astype(F32))
                for j, o in enumerate(_pack_all(ops)):
                    wd[kd, 7 * i + j, rows, cols] = o
                return _after(v, wd[jnp.minimum(kd, n_it), 7 * i, rows, cols], k)

            def mod_piece(j, c, v):
                w = rm[slot, pl.ds(pl.multiple_of(odd * mr, mr), mr), pl.ds(j * D + c * hd, hd)]
                sv = scb[pl.ds(pl.multiple_of(k * mr, mr), mr), :]
                t = w.astype(F32) * jnp.concatenate([sv] * (hd // LANE), axis=1)
                cols = pl.ds(c * hd, hd)
                mod[2 + j, :, cols] += sum(t[r:r + 8] for r in range(8, mr, 8)) + t[0:8]
                return _after(v, mod[jnp.minimum(k, 0) + 2 + j, :, pl.ds(c * hd, LANE)], k)

            pieces = [functools.partial(up_piece, t, i)
                      for t in range(qf // LANE) for i in range(7)]
            pieces += [functools.partial(down_piece, a, t, i) for a in range(DR // 16)
                       for t in range(qd // LANE) for i in range(7)]
            spots = [(u, t, n) for u in range(UNR) for t, m in SPOT for n in range(H) if n % 4 < m]
            assert len(pieces) <= len(spots)
            side = dict(zip(spots, pieces))
            for j in range(4):
                for c in range(2):
                    side[c, 3, 3 + 8 * j] = functools.partial(mod_piece, j, c)
            for u in range(UNR):
                step(k, u, {sp[1:]: f for sp, f in side.items() if sp[0] == u})

            @pl.when((odd == 0) & (k + 2 < n_it))
            def _():
                for cp in raw_cp(kp + 1, 1 - slot):
                    cp.start()

            return carry

        lax.fori_loop(0, n_it, steps, 0)
        for j in range(2, 6):
            mod[j] = jnp.broadcast_to(jnp.sum(mod[j], axis=0, keepdims=True), (8, D))

        def resid(sg, rows):
            return xb[sg, rows, :].astype(F32) + mrow(2) * ab[sg, rows, :].astype(F32)

        def norm_piece(b, r, a):
            rows = pl.ds(a * 16, 16)
            h2f[r, rows, :] = _norm(resid(b * 4 + r, rows)) * (1.0 + mrow(4)) + mrow(3)
            return h2f[jnp.minimum(b, 0) + r, pl.ds(a * 16, 8), 0:qd]

        def lhs_piece(b, a, i):
            ops = _ops49(_LHS, i, lambda r, c: h2f[r, pl.ds(a * 16, 16), pl.ds(c * qd, qd)])
            for j, o in enumerate(ops):
                h2b[7 * i + j, pl.ds(a * 8, 8), :] = _pack(o)
            return h2b[jnp.minimum(b, 0) + 7 * i, pl.ds(a * 8, 8), :]

        ffn_in = [functools.partial(norm_piece, r=r, a=a)
                  for r in range(4) for a in range(seg // 16)]
        ffn_in += [functools.partial(lhs_piece, a=a, i=i)
                   for a in range(seg // 16) for i in range(7)]

        def out_cp(b):
            return pltpu.make_async_copy(ob.at[b % 2], out_hbm.at[pl.ds(b * fm, fm), :],
                                         sem_out.at[b % 2])

        def ffn(b, carry):
            @pl.when(b >= 2)
            def _():
                out_cp(b - 2).wait()

            slot = lax.rem(b, 2)
            lhs = []
            for f in range(qf // LANE):
                cols = pl.ds(f * LANE, LANE)
                gu = _out16([_mm(_unpack(h2b[n]), jnp.concatenate(
                    [_unpack(wu[:, c, n, :, cols].reshape(qd // 2, LANE)) for c in range(2)],
                    axis=1)) for n in range(49)])
                act = {}
                for r in range(4):
                    for c in range(2):
                        v = _silu(gu[r, c]) * gu[r, 2 + c]
                        act[r, 2 * c], act[r, 2 * c + 1] = v[:, :LANE], v[:, LANE:]
                lhs.append([o for i in range(7)
                            for o in _ops49(_LHS, i, lambda r, c: act[r, c])])
            prod, late = [], []
            for n in range(49):
                w = wd[:, n].reshape(qf // 2, qd)
                if 0 <= n - TIE0 < len(ffn_in):
                    token = ffn_in[n - TIE0](jnp.minimum(b + 1, n_blk - 1))
                    w = jnp.concatenate([_after(w[:8], token, b), w[8:]], axis=0)
                a = [l[n] for l in lhs]
                if n < NSPLIT:
                    ks = (qf - LANE) // 2
                    late.append((a.pop().astype(BF16), _unpack(w[ks:])))
                    w = w[:ks]
                prod.append(_mm(jnp.concatenate(a, axis=1).astype(BF16), _unpack(w)))
                if n == NSPLIT - 1:
                    prod = [_mm(*t) + v for t, v in zip(late, prod)]
            y = _out16(prod)
            for r in range(4):
                yr = jnp.concatenate([y[r, c] for c in range(4)], axis=1)
                ob[slot, pl.ds(r * seg, seg), :] = (
                    resid(b * 4 + r, slice(None)) + mrow(5) * yr).astype(ob.dtype)
            out_cp(b).start()
            return carry

        for piece in ffn_in:
            piece(0)
        lax.fori_loop(0, n_blk, ffn, 0)
        for b in range(n_blk - 2, n_blk):
            out_cp(b).wait()

    pl.run_scoped(main, pltpu.VMEM((n_it // 2, 2, 49, 8, qf), U32),
                  pltpu.VMEM((n_dr, 49, DR // 2, qd), U32))


@functools.partial(jax.jit, static_argnames=("A_seg_len",))
def pallas_adaLN_cond__memory_aug_recurrent_mem_tr__glu_gated_swiglu__prompt_kernel(
    A_x, A_mem0, A_Wq, A_Wk, A_Wv, A_Wo, A_seg_len, B_x, B_w1, B_w3, B_w2, c, w_mod,
):
    del B_x
    B, S, D = A_x.shape
    H, Dh = A_Wq.shape[1], A_Wq.shape[2]
    M = A_mem0.shape[1]
    F = B_w1.shape[1]
    seg = int(A_seg_len)
    n_seg = S // seg
    assert B == 1 and Dh == LANE and H == 32 and (M, seg) == (8, 32) and S == n_seg * seg
    assert D == 16 * n_seg and F % (4 * LANE) == 0 and F // 4 <= DR * n_seg // UNR
    hbm = pl.BlockSpec(memory_space=pl.ANY)
    dma = pltpu.SemaphoreType.DMA
    out = pl.pallas_call(
        _kernel,
        out_shape=jax.ShapeDtypeStruct((S, D), A_x.dtype),
        in_specs=[hbm] * 11,
        out_specs=hbm,
        scratch_shapes=[
            pltpu.VMEM((n_seg, seg, D), BF16),
            pltpu.VMEM((n_seg, seg, D), BF16),
            pltpu.VMEM((3 * H, D // 2, LANE), U32),
            pltpu.VMEM((3 * H, n_seg * PRE // 2, LANE), U32),
            pltpu.VMEM((D // LANE, H * Dh, LANE), BF16),
            pltpu.VMEM((6, 8, D), F32),
            pltpu.VMEM(((M + seg - PRE) // 2, D), U32),
            pltpu.VMEM((2, 2, 4, 16, F), BF16),
            pltpu.VMEM((2, 4, 2 * DR, D), BF16),
            pltpu.VMEM((2, 2 * D * UNR // n_seg, 4 * D), BF16),
            pltpu.VMEM((D, LANE), F32),
            pltpu.VMEM((4, seg, D), F32),
            pltpu.VMEM((49, seg // 2, D // 4), U32),
            pltpu.VMEM((2, 4 * seg, D), A_x.dtype),
            pltpu.VMEM((M, D), BF16),
            dma((4,)), dma((2,)), dma((NSTG,)), dma((D // LANE,)), dma((2, 4)), dma((2,)),
        ],
        compiler_params=pltpu.CompilerParams(disable_bounds_checks=True,
                                             vmem_limit_bytes=127 * 2**20),
    )(c, A_mem0.reshape(M, D), A_x.reshape(n_seg, seg, D), A_Wq, A_Wk, A_Wv,
      A_Wo.reshape(H * Dh, D), B_w1.reshape(4, D // 4, F), B_w3.reshape(4, D // 4, F),
      B_w2.reshape(4, F // 4, D), w_mod)
    return out.reshape(B, S, D)
```
